```python
import jax
import jax.numpy as jnp

def _softmax(x, axis=-1):
    return jax.nn.softmax(x, axis=axis)

def _gelu(x):
    return jax.nn.gelu(x, approximate=True)

def _silu(x):
    return jax.nn.silu(x)

def _sigmoid(x):
    return jax.nn.sigmoid(x)

def _layernorm(x, axis=-1, eps=1e-05):
    m = jnp.mean(x, axis=axis, keepdims=True)
    v = jnp.var(x, axis=axis, keepdims=True)
    return (x - m) / jnp.sqrt(v + eps)

def _scatter_add(tgt, idx, src, axis=0):
    return tgt.at[idx].add(src)

def _segment_sum(src, seg, n):
    return jax.ops.segment_sum(src, seg, n)

class _Rng:

    def __init__(self, key):
        self._k = key

    def _next(self):
        self._k, sub = jax.random.split(self._k)
        return sub

    def normal(self, shape):
        return jax.random.normal(self._next(), shape, dtype=jnp.bfloat16)

    def randint(self, lo, hi, shape):
        return jax.random.randint(self._next(), shape, lo, hi, dtype=jnp.int32)

    def uniform(self, shape, lo=0.0, hi=1.0):
        return jax.random.uniform(self._next(), shape, jnp.bfloat16, lo, hi)

    def permutation(self, n):
        return jax.random.permutation(self._next(), n)
kernel_name = 'recurrent_scan__memory_aug_recurrent_mem_tr__mixer_s_mlp__prompt'

def setup_inputs():
    _rng = _Rng(jax.random.key(int.from_bytes(__import__("os").urandom(4), "little")))
    _w = lambda a: (lambda t: t.astype(jnp.bfloat16) if jnp.issubdtype(t.dtype, jnp.floating) else t)(jnp.asarray(a))

    def _A_setup():
        B, S, Dm = (1, 2048, 1024)
        H, Dh = (32, 128)
        M, seg = (8, 32)
        seg = min(seg, S)
        S = S // seg * seg
        return {'x': _w((lambda *s: _rng.normal(s) * 0.05)(B, S, Dm)), 'mem0': _w((lambda *s: _rng.normal(s) * 0.05)(B, M, Dm)), 'Wq': _w((lambda *s: _rng.normal(s) * 0.05)(Dm, H, Dh) * Dm ** (-0.5)), 'Wk': _w((lambda *s: _rng.normal(s) * 0.05)(Dm, H, Dh) * Dm ** (-0.5)), 'Wv': _w((lambda *s: _rng.normal(s) * 0.05)(Dm, H, Dh) * Dm ** (-0.5)), 'Wo': _w((lambda *s: _rng.normal(s) * 0.05)(H, Dh, Dm) * (H * Dh) ** (-0.5)), 'seg_len': seg}
    _A_in = _A_setup()

    def _B_setup():
        B, S, D, F = (1, 2048, 1024, 3584)
        return {'x': _w((lambda *s: _rng.normal(s) * 0.05)(B, S, D)), 'w1': _w((lambda *s: _rng.normal(s) * 0.05)(D, D) * D ** (-0.5)), 'w2': _w((lambda *s: _rng.normal(s) * 0.05)(D, D) * D ** (-0.5)), 'w3': _w((lambda *s: _rng.normal(s) * 0.05)(D, F) * D ** (-0.5)), 'w4': _w((lambda *s: _rng.normal(s) * 0.05)(F, D) * F ** (-0.5))}
    _B_in = _B_setup()
    return {'A_x': _A_in['x'], 'A_mem0': _A_in['mem0'], 'A_Wq': _A_in['Wq'], 'A_Wk': _A_in['Wk'], 'A_Wv': _A_in['Wv'], 'A_Wo': _A_in['Wo'], 'A_seg_len': _A_in['seg_len'], 'B_x': _B_in['x'], 'B_w1': _B_in['w1'], 'B_w2': _B_in['w2'], 'B_w3': _B_in['w3'], 'B_w4': _B_in['w4']}

def reference(A_x, A_mem0, A_Wq, A_Wk, A_Wv, A_Wo, A_seg_len, B_x, B_w1, B_w2, B_w3, B_w4):

    def _A_ref(x, mem0, Wq, Wk, Wv, Wo, seg_len):
        B, S, Dm = x.shape
        H, Dh = (Wq.shape[1], Wq.shape[2])
        M = mem0.shape[1]
        scale = Dh ** (-0.5)
        n_seg = S // seg_len
        L = M + seg_len
        idx = jnp.arange(L)
        mask = (idx[:, None] < M) | (idx[:, None] >= idx[None, :])
        mem = mem0
        outs = []
        for s in range(n_seg):
            xs = x[:, s * seg_len:(s + 1) * seg_len, :].copy()
            h = jnp.concatenate([mem, xs], axis=1)
            q = jnp.einsum('btd,dhe->bhte', h, Wq)
            k = jnp.einsum('btd,dhe->bhte', h, Wk)
            v = jnp.einsum('btd,dhe->bhte', h, Wv)
            scores = jnp.einsum('bhqe,bhke->bhqk', q, k) * scale
            scores = jnp.where(mask[None, None], scores, -1000000000.0)
            p = _softmax(scores, axis=-1)
            o = jnp.einsum('bhqk,bhke->bhqe', p, v)
            o = jnp.einsum('bhte,hed->btd', o, Wo)
            mem = o[:, :M, :].copy()
            outs.append(o[:, M:, :])
        return jnp.concatenate(outs, axis=1)

    def _B_ref(x, w1, w2, w3, w4):
        B, S, D = x.shape
        h = _gelu(_layernorm(x, axis=-1) @ w1)
        c = D // 4
        g0 = jnp.pad(h[:, :, 0 * c:1 * c], ((0, 0), (1, 0), (0, 0)))[:, :S, :]
        g1 = jnp.pad(h[:, :, 1 * c:2 * c], ((0, 0), (0, 1), (0, 0)))[:, 1:, :]
        g2 = jnp.pad(h[:, :, 2 * c:3 * c], ((0, 0), (2, 0), (0, 0)))[:, :S, :]
        g3 = jnp.pad(h[:, :, 3 * c:], ((0, 0), (0, 2), (0, 0)))[:, 2:, :]
        hs = jnp.concatenate([g0, g1, g2, g3], axis=-1) @ w2
        x1 = x + hs
        h2 = _gelu(_layernorm(x1, axis=-1) @ w3) @ w4
        return x1 + h2
    x = A_x
    xn = _layernorm(x, axis=-1)
    s = _A_ref(xn, A_mem0, A_Wq, A_Wk, A_Wv, A_Wo, A_seg_len)
    g = _silu(_B_ref(xn, B_w1, B_w2, B_w3, B_w4))
    return x + s * g
```

```python
import functools
import jax
import jax.numpy as jnp
from jax import lax
import jax.experimental.pallas as pl
import jax.experimental.pallas.tpu as pltpu

F32 = jnp.float32
BF16 = jnp.bfloat16
U32 = jnp.uint32
EPS = 1e-5
LOG2E = 1.4426950408889634


def _ln(x):
    m = jnp.mean(x, axis=-1, keepdims=True)
    xc = x - m
    v = jnp.mean(xc * xc, axis=-1, keepdims=True)
    return xc * lax.rsqrt(v + EPS)


def _gelu(x):
    c = 0.7978845608028654
    return 0.5 * x * (1.0 + jnp.tanh(c * (x + 0.044715 * (x * x * x))))


def _dot(a, w_u32):
    return jnp.dot(a, pltpu.bitcast(w_u32, BF16), preferred_element_type=F32)


def _kernel(x_hbm, mem0_ref, wq_hbm, wk_hbm, wv_hbm, wo_hbm, w1_hbm, w2_hbm, w3_hbm, w4_hbm, out_ref,
            x_ref, stage, wqkv_ref, wo_ref, w1_ref, w2_ref, w3_ref, w4_ref,
            h_ref, x1_ref, mem_ref, sems, *, S, D, H, DH, M, SEG, FF):
    L = M + SEG
    R = 2 * L
    NP = H // 2
    ND = D // 128
    NF = FF // 128
    RB = 256
    C4 = D // 4

    def col_copies(src, dst, n, sem):
        s32 = src.bitcast(U32)
        return [pltpu.make_async_copy(s32.at[:, pl.ds(j * 128, 128)], dst.at[j], sem) for j in range(n)]

    def head_copies(src, m, sem):
        s32 = src.bitcast(U32)
        return [pltpu.make_async_copy(s32.at[:, j, :], stage.at[m, j], sem) for j in range(NP)]

    groups = [
        col_copies(w1_hbm, w1_ref, ND, sems.at[0]),
        [pltpu.make_async_copy(x_hbm, x_ref, sems.at[1])],
        col_copies(w2_hbm, w2_ref, ND, sems.at[2]),
        head_copies(wq_hbm, 0, sems.at[3]),
        head_copies(wk_hbm, 1, sems.at[4]),
        head_copies(wv_hbm, 2, sems.at[5]),
        col_copies(wo_hbm, wo_ref, ND, sems.at[6]),
        col_copies(w3_hbm, w3_ref, NF, sems.at[7]),
        col_copies(w4_hbm, w4_ref, ND, sems.at[8]),
    ]
    for g in groups:
        for cp in g:
            cp.start()

    def wait(i):
        for cp in groups[i]:
            cp.wait()

    h_ref[0:8, :] = jnp.zeros((8, D), F32)
    h_ref[S + 8:S + 16, :] = jnp.zeros((8, D), F32)
    wait(0)
    wait(1)

    def p1(i, c):
        r0 = pl.multiple_of(i * RB, RB)
        xn = _ln(x_ref[pl.ds(r0, RB), :].astype(F32))
        a = _ln(xn).astype(BF16)
        for j in range(ND):
            h_ref[pl.ds(r0 + 8, RB), j * 128:(j + 1) * 128] = _gelu(_dot(a, w1_ref[j]))
        return c
    lax.fori_loop(0, S // RB, p1, 0)
    wait(2)

    def p2(i, c):
        r0 = pl.multiple_of(i * RB, RB)
        xn = _ln(x_ref[pl.ds(r0, RB), :].astype(F32))
        win = h_ref[pl.ds(r0, RB + 16), :]
        g = jnp.concatenate([
            win[7:7 + RB, 0:C4], win[9:9 + RB, C4:2 * C4],
            win[6:6 + RB, 2 * C4:3 * C4], win[10:10 + RB, 3 * C4:]], axis=1).astype(BF16)
        for j in range(ND):
            x1_ref[pl.ds(r0, RB), j * 128:(j + 1) * 128] = xn[:, j * 128:(j + 1) * 128] + _dot(g, w2_ref[j])
        return c
    lax.fori_loop(0, S // RB, p2, 0)

    for m in range(3):
        wait(3 + m)

        def rp(i, c, m=m):
            base = pl.multiple_of(i * 16, 16)
            r = pl.multiple_of(i * 8, 8)
            for j in range(NP):
                a = stage[m, j, pl.ds(base, 8, stride=2), :]
                b = stage[m, j, pl.ds(base + 1, 8, stride=2), :]
                wqkv_ref[m, 2 * j, pl.ds(r, 8), :] = (a & U32(0xFFFF)) | (b << 16)
                wqkv_ref[m, 2 * j + 1, pl.ds(r, 8), :] = (a >> 16) | (b & U32(0xFFFF0000))
            return c
        lax.fori_loop(0, D // 16, rp, 0)
    wait(6); wait(7); wait(8)

    mem_ref[...] = mem0_ref[...].astype(F32)

    row = lax.broadcasted_iota(jnp.int32, (R, R), 0)
    col = lax.broadcasted_iota(jnp.int32, (R, R), 1)
    same = (row >= L) == (col >= L)
    rr = jnp.where(row >= L, row - L, row)
    cc = jnp.where(col >= L, col - L, col)
    ok = same & ((rr < M) | (rr >= cc))
    scale = DH ** -0.5
    fill = jnp.where(same, -1e9 / scale, -jnp.inf).astype(F32)
    cexp = scale * LOG2E

    def qk(q2, k2):
        s = lax.dot_general(q2, k2, (((1,), (1,)), ((), ())), preferred_element_type=F32)
        s = jnp.where(ok, s, fill)
        m = jnp.max(s, axis=-1, keepdims=True)
        e = jnp.exp2((s - m) * cexp)
        l = jnp.sum(e, axis=-1, keepdims=True)
        r = pl.reciprocal(l, approx=True)
        r = r * (2.0 - l * r)
        return (e * r).astype(BF16)

    def pv(p, v2):
        return jnp.dot(p, v2, preferred_element_type=F32)

    def step(j, c):
        r0 = pl.multiple_of(j * 64, 64)
        x = x_ref[pl.ds(r0, 64), :].astype(F32)
        xn = _ln(x)
        mem = mem_ref[...]
        lhs_a = jnp.concatenate([mem, xn[0:40]], axis=0).astype(BF16)
        x1 = x1_ref[pl.ds(r0, 64), :]
        a3 = _ln(x1).astype(BF16)

        u = [None] * NF
        h2 = [None] * ND

        def mlp_up(fs):
            for f in fs:
                u[f] = _gelu(_dot(a3, w3_ref[f])).astype(BF16)

        def mlp_down(ns):
            uu = jnp.concatenate(u, axis=1)
            for n in ns:
                h2[n] = _dot(uu, w4_ref[n])

        def segment(lhs, build_qkv, build_o, fillers):
            qkv = [None] * NP
            er = [None] * NP
            o = [None] * H
            KSPLIT = NP - 2
            KS = KSPLIT * 128

            def do_qkv(p):
                y = [[_dot(lhs, wqkv_ref[m, 2 * p + hh]) for m in range(3)] for hh in range(2)]
                qkv[p] = [t.astype(BF16) for t in build_qkv(p, y)]

            def do_qk(p):
                er[p] = qk(qkv[p][0], qkv[p][1])

            def do_pv(p):
                o2 = pv(er[p], qkv[p][2])
                o[2 * p], o[2 * p + 1] = build_o(p, o2)

            for p in range(NP):
                do_qkv(p)
                if p >= 1:
                    do_qk(p - 1)
                if p >= 2:
                    do_pv(p - 2)
            fillers[0]()
            do_qk(NP - 1)
            do_pv(NP - 2)
            olo = jnp.concatenate(o[:2 * KSPLIT], axis=1)
            acc = [_dot(olo, wo_ref[n, 0:KS, :]) for n in range(ND // 2)]
            do_pv(NP - 1)
            acc += [_dot(olo, wo_ref[n, 0:KS, :]) for n in range(ND // 2, ND)]
            ohi = jnp.concatenate(o[2 * KSPLIT:], axis=1)
            res = jnp.concatenate(
                [acc[n] + _dot(ohi, wo_ref[n, KS:, :]) for n in range(ND)], axis=1)
            fillers[1]()
            return res

        saved = [None] * NP
        o_saved = [None] * H

        def build_qkv_a(p, y):
            saved[p] = [[y[hh][m][40:48] for m in range(3)] for hh in range(2)]
            return [jnp.concatenate([y[0][m][0:40], y[1][m][0:40]], axis=0) for m in range(3)]

        def build_o_a(p, o2):
            o_saved[2 * p] = o2[32:40]
            o_saved[2 * p + 1] = o2[72:80]
            return o2[0:32].astype(BF16), o2[40:72].astype(BF16)

        def build_qkv_b(p, y):
            return [jnp.concatenate([y[0][m][0:8], saved[p][0][m], y[0][m][8:32],
                                     y[1][m][0:8], saved[p][1][m], y[1][m][8:32]], axis=0)
                    for m in range(3)]

        def build_o_b(p, o2):
            return (jnp.concatenate([o2[0:8], o_saved[2 * p], o2[8:40]], axis=0).astype(BF16),
                    jnp.concatenate([o2[40:48], o_saved[2 * p + 1], o2[48:80]], axis=0).astype(BF16))

        sa = segment(lhs_a, build_qkv_a, build_o_a,
                     [lambda: mlp_up(range(0, 8)), lambda: mlp_up(range(8, NF))])
        mem_ref[...] = sa[0:8]
        lhs_b = jnp.concatenate([sa[0:8], xn[40:64]], axis=0).astype(BF16)
        sb = segment(lhs_b, build_qkv_b, build_o_b,
                     [lambda: mlp_down(range(0, 4)), lambda: mlp_down(range(4, ND))])
        mem_ref[...] = sb[0:8]
        s = jnp.concatenate([sa[8:32], sb[8:48]], axis=0)
        b = x1 + jnp.concatenate(h2, axis=1)
        g = b * jax.nn.sigmoid(b)
        out_ref[pl.ds(r0, 64), :] = (x + s * g).astype(out_ref.dtype)
        return c
    lax.fori_loop(0, S // 64, step, 0)


@functools.partial(jax.jit, static_argnames=("A_seg_len",))
def pallas_recurrent_scan__memory_aug_recurrent_mem_tr__mixer_s_mlp__prompt_kernel(
        A_x, A_mem0, A_Wq, A_Wk, A_Wv, A_Wo, A_seg_len, B_x, B_w1, B_w2, B_w3, B_w4):
    _, S, D = A_x.shape
    _, H, DH = A_Wq.shape
    M = A_mem0.shape[1]
    FF = B_w3.shape[1]
    kern = functools.partial(_kernel, S=S, D=D, H=H, DH=DH, M=M, SEG=A_seg_len, FF=FF)
    any_spec = pl.BlockSpec(memory_space=pl.ANY)
    vmem_spec = pl.BlockSpec(memory_space=pltpu.VMEM)
    out = pl.pallas_call(
        kern,
        out_shape=jax.ShapeDtypeStruct((S, D), A_x.dtype),
        in_specs=[any_spec, vmem_spec] + [any_spec] * 8,
        out_specs=vmem_spec,
        scratch_shapes=[
            pltpu.VMEM((S, D), BF16),
            pltpu.VMEM((3, H // 2, D, 128), U32),
            pltpu.VMEM((3, H, D // 2, 128), U32),
            pltpu.VMEM((D // 128, H * DH // 2, 128), U32),
            pltpu.VMEM((D // 128, D // 2, 128), U32),
            pltpu.VMEM((D // 128, D // 2, 128), U32),
            pltpu.VMEM((FF // 128, D // 2, 128), U32),
            pltpu.VMEM((D // 128, FF // 2, 128), U32),
            pltpu.VMEM((S + 16, D), F32),
            pltpu.VMEM((S, D), F32),
            pltpu.VMEM((M, D), F32),
            pltpu.SemaphoreType.DMA((9,)),
        ],
        compiler_params=pltpu.CompilerParams(vmem_limit_bytes=120 * 1024 * 1024),
    )(A_x[0], A_mem0[0], A_Wq, A_Wk, A_Wv, A_Wo.reshape(H * DH, D), B_w1, B_w2, B_w3, B_w4)
    return out[None]
```

```python
import functools
import jax
import jax.numpy as jnp
from jax import lax
import jax.experimental.pallas as pl
import jax.experimental.pallas.tpu as pltpu

F32 = jnp.float32
BF16 = jnp.bfloat16
U32 = jnp.uint32
EPS = 1e-5
LOG2E = 1.4426950408889634

SUB = 128
NSUB = 4
CPRE = 5
STEP = 64


def _ln(x):
    m = jnp.mean(x, axis=-1, keepdims=True)
    xc = x - m
    v = jnp.mean(xc * xc, axis=-1, keepdims=True)
    return xc * lax.rsqrt(v + EPS)


def _gelu(x):
    c = 0.7978845608028654
    return 0.5 * x * (1.0 + jnp.tanh(c * (x + 0.044715 * (x * x * x))))


def _bf(w_u32):
    return pltpu.bitcast(w_u32, BF16)


def _pk(x):
    return pltpu.bitcast(x.astype(BF16), U32)


def _dot(a, w_u32):
    return jnp.dot(a, _bf(w_u32), preferred_element_type=F32)


def _kernel(x_hbm, mem0_ref, wq_hbm, wk_hbm, wv_hbm, wo_hbm, w1_hbm, w2_hbm, w3_hbm, w4_hbm, out_hbm,
            x_ref, stage, wqkv_ref, wo_ref, w1_ref, w2_ref, w3_ref, w4_ref,
            h_ref, b_ref, a3_ref, pre_ref, s_ref, mem_ref, sems, *, S, D, H, DH, M, SEG, FF):
    L = M + SEG
    R = 2 * L
    NP = H // 2
    ND = D // 128
    NF = FF // 128
    C4 = D // 4
    RB = SUB * NSUB
    NIT = S // RB
    NSLAB = 3 * NP
    SLAB_IT = NSLAB // NIT

    SEM_W1, SEM_W2, SEM_W3A, SEM_W4A, SEM_WO, SEM_W3B, SEM_W4B, SEM_OUT, SEM_X0 = range(9)
    SEM_X = 9
    SEM_SLAB = SEM_X + NIT

    def col_copies(src, dst, js, sem, rows=None):
        s32 = src.bitcast(U32)
        if rows is None:
            return [pltpu.make_async_copy(s32.at[:, pl.ds(j * 128, 128)], dst.at[j], sem) for j in js]
        lo, n = rows
        return [pltpu.make_async_copy(s32.at[pl.ds(lo, n), pl.ds(j * 128, 128)],
                                      dst.at[j, pl.ds(lo, n)], sem) for j in js]

    def x_copy(lo, n, sem):
        return pltpu.make_async_copy(x_hbm.at[pl.ds(lo, n)], x_ref.at[pl.ds(lo, n)], sem)

    def x_chunk(i):
        lo = SUB + i * RB
        return lo, min(RB, S - lo)

    wsrc = [wq_hbm.bitcast(U32), wk_hbm.bitcast(U32), wv_hbm.bitcast(U32)]
    slab_copies = [pltpu.make_async_copy(wsrc[s // NP].at[:, s % NP, :], stage.at[s],
                                         sems.at[SEM_SLAB + s // SLAB_IT]) for s in range(NSLAB)]
    g_x0 = [x_copy(0, SUB, sems.at[SEM_X0])]
    g_w1 = col_copies(w1_hbm, w1_ref, range(ND), sems.at[SEM_W1])
    g_x = [x_copy(*x_chunk(i), sems.at[SEM_X + i]) for i in range(NIT)]
    g_w2 = col_copies(w2_hbm, w2_ref, range(ND), sems.at[SEM_W2])
    g_w3a = col_copies(w3_hbm, w3_ref, range(CPRE), sems.at[SEM_W3A])
    g_w4a = col_copies(w4_hbm, w4_ref, range(ND), sems.at[SEM_W4A], rows=(0, CPRE * 64))
    g_wo = col_copies(wo_hbm, wo_ref, range(ND), sems.at[SEM_WO])
    g_w3b = col_copies(w3_hbm, w3_ref, range(CPRE, NF), sems.at[SEM_W3B])
    g_w4b = col_copies(w4_hbm, w4_ref, range(ND), sems.at[SEM_W4B], rows=(CPRE * 64, (NF - CPRE) * 64))
    def start(*gs):
        for g in gs:
            for cp in g:
                cp.start()

    start(g_x0, g_x[:1], g_w1, g_x[1:], g_w2, g_w3a, g_w4a)

    def wait(g):
        for cp in g:
            cp.wait()

    h_ref[:, 0:8, :] = jnp.zeros((ND, 8, 128), F32)
    h_ref[:, S + 8:S + 16, :] = jnp.zeros((ND, 8, 128), F32)
    s_ref[...] = jnp.zeros(s_ref.shape, F32)
    mem_ref[...] = mem0_ref[...].astype(F32)

    def ln2(r):
        xn = _ln(x_ref[pl.ds(r, SUB), :].astype(F32))
        b_ref[pl.ds(r, SUB), :] = xn
        return _ln(xn)

    wait(g_x0)
    pre_ref[...] = _pk(ln2(0))
    wait(g_w1)

    def p1_body(base):
        a = _bf(pre_ref[...])
        for s in range(NSUB):
            if s + 1 < NSUB:
                a_next = ln2(base + (s + 1) * SUB).astype(BF16)
            for j in range(ND):
                h_ref[j, pl.ds(base + s * SUB + 8, SUB), :] = _gelu(_dot(a, w1_ref[j]))
            if s + 1 < NSUB:
                a = a_next
        nxt = pl.multiple_of(jnp.minimum(base + RB, S - SUB), SUB)
        pre_ref[...] = _pk(ln2(nxt))

    def p1(i, c):
        base = pl.multiple_of(i * RB, RB)
        lo = pl.multiple_of(base + SUB, SUB)
        for k in range(NIT - 1):
            pl.when(i == k)(functools.partial(start, slab_copies[k * SLAB_IT:(k + 1) * SLAB_IT]))
        x_copy(lo, RB, sems.at[SEM_X + i]).wait()
        p1_body(base)
        return c
    lax.fori_loop(0, NIT - 1, p1, 0)
    start(slab_copies[(NIT - 1) * SLAB_IT:])
    wait(g_x[NIT - 1:])
    p1_body((NIT - 1) * RB)

    def build_g(r):
        offs = (7, 9, 6, 10)
        return jnp.concatenate(
            [h_ref[j, pl.ds(r + offs[j * 128 // C4], SUB), :] for j in range(ND)], axis=1)

    pre_ref[...] = _pk(build_g(0))
    wait(g_w2); wait(g_w3a); wait(g_w4a)

    def p23(it, c):
        base = pl.multiple_of(it * RB, RB)
        for k, gs in enumerate(((g_wo,), (g_w3b,), (g_w4b,))):
            pl.when(it == k)(functools.partial(start, *gs))
        sl = stage.at[pl.ds(it * SLAB_IT, SLAB_IT)]
        pltpu.make_async_copy(sl, sl, sems.at[SEM_SLAB + it]).wait()

        g = [None] * NSUB
        x1 = [None] * NSUB
        a3 = [None] * NSUB
        u = [None] * NSUB
        g[0] = _bf(pre_ref[...])

        items = [(k, i) for k in range(SLAB_IT) for i in range(D // 16)]
        nties = NSUB * (2 * ND + CPRE) - ND
        per = -(-len(items) // nties)

        def tie(y):
            z = (pltpu.bitcast(y[0:8, :], U32) >> 31) >> 1
            mlo = z + U32(0xFFFF)
            mhi = z + U32(0xFFFF0000)
            for _ in range(per):
                if not items:
                    break
                k, i = items.pop(0)
                slab = it * SLAB_IT + k
                a = stage[slab, pl.ds(i * 16, 8, stride=2), :]
                b = stage[slab, pl.ds(i * 16 + 1, 8, stride=2), :]
                wqkv_ref[2 * slab, i * 8:(i + 1) * 8, :] = (a & mlo) | (b << 16)
                wqkv_ref[2 * slab + 1, i * 8:(i + 1) * 8, :] = (a >> 16) | (b & mhi)

        def m2(s):
            if s + 1 < NSUB:
                g[s + 1] = build_g(base + (s + 1) * SUB).astype(BF16)
            ys = []
            for j in range(ND):
                ys.append(_dot(g[s], w2_ref[j]))
                tie(ys[-1])
            x1[s] = jnp.concatenate(ys, axis=1) + b_ref[pl.ds(base + s * SUB, SUB), :]
            a3[s] = _ln(x1[s]).astype(BF16)
            r2 = pl.multiple_of(it * (RB // 2) + s * (SUB // 2), SUB // 2)
            a3_ref[pl.ds(r2, SUB // 2), :] = pltpu.bitcast(a3[s], U32)

        def up(s):
            us = []
            for f in range(CPRE):
                y = _dot(a3[s], w3_ref[f])
                tie(y)
                us.append(_gelu(y).astype(BF16))
            u[s] = jnp.concatenate(us, axis=1)

        def down(s):
            for n in range(ND):
                y = _dot(u[s], w4_ref[n, 0:CPRE * 64, :]) + x1[s][:, n * 128:(n + 1) * 128]
                tie(y)
                b_ref[pl.ds(base + s * SUB, SUB), n * 128:(n + 1) * 128] = y

        q = SLAB_IT // NSUB
        m2(0)
        m2(1); up(0)
        m2(2); up(1); down(0)
        m2(3); up(2); down(1)
        nxt = pl.multiple_of(jnp.minimum(base + RB, S - SUB), SUB)
        pre_ref[...] = _pk(build_g(nxt))
        down(2); up(3); down(3)
        assert not items
        return c
    lax.fori_loop(0, NIT, p23, 0)
    wait(g_wo); wait(g_w3b); wait(g_w4b)

    row = lax.broadcasted_iota(jnp.int32, (R, R), 0)
    col = lax.broadcasted_iota(jnp.int32, (R, R), 1)
    same = (row >= L) == (col >= L)
    rr = jnp.where(row >= L, row - L, row)
    cc = jnp.where(col >= L, col - L, col)
    ok = same & ((rr < M) | (rr >= cc))
    scale = DH ** -0.5
    fill = jnp.where(same, -1e9 / scale, -jnp.inf).astype(F32)
    cexp = scale * LOG2E

    def qk(q2, k2):
        s = lax.dot_general(q2, k2, (((1,), (1,)), ((), ())), preferred_element_type=F32)
        s = jnp.where(ok, s, fill)
        m = jnp.max(s, axis=-1, keepdims=True)
        e = jnp.exp2((s - m) * cexp)
        l = jnp.sum(e, axis=-1, keepdims=True)
        r = pl.reciprocal(l, approx=True)
        r = r * (2.0 - l * r)
        return (e * r).astype(BF16)

    def pv(p, v2):
        return jnp.dot(p, v2, preferred_element_type=F32)

    def combine(r):
        b = b_ref[pl.ds(r, STEP), :]
        g = b * jax.nn.sigmoid(b)
        x = x_ref[pl.ds(r, STEP), :].astype(F32)
        x_ref[pl.ds(r, STEP), :] = (x + s_ref[...] * g).astype(x_ref.dtype)

    def out_copy(r):
        return pltpu.make_async_copy(x_ref.at[pl.ds(r, STEP)], out_hbm.at[pl.ds(r, STEP)], sems.at[SEM_OUT])

    def step(j, c):
        r0 = pl.multiple_of(j * STEP, STEP)
        rprev = pl.multiple_of(jnp.maximum(r0 - STEP, 0), STEP)
        a3 = _bf(a3_ref[pl.ds(pl.multiple_of(j * (STEP // 2), STEP // 2), STEP // 2), :])
        xn = _ln(x_ref[pl.ds(r0, STEP), :].astype(F32))
        mem = mem_ref[...]
        lhs_a = jnp.concatenate([mem, xn[0:40]], axis=0).astype(BF16)

        u = [None] * NF

        def mlp_up(fs):
            for f in fs:
                u[f] = _gelu(_dot(a3, w3_ref[f])).astype(BF16)

        def mlp_down(ns):
            uu = jnp.concatenate(u[CPRE:], axis=1)
            for n in ns:
                b_ref[pl.ds(r0, STEP), n * 128:(n + 1) * 128] = (
                    _dot(uu, w4_ref[n, CPRE * 64:, :]) + b_ref[pl.ds(r0, STEP), n * 128:(n + 1) * 128])

        def segment(lhs, build_qkv, build_o, fillers):
            qkv = [None] * NP
            er = [None] * NP
            o = [None] * H
            KSPLIT = NP - 3
            KS = KSPLIT * 128

            def do_qkv(p):
                y = [[_dot(lhs, wqkv_ref[m * H + 2 * p + hh]) for m in range(3)] for hh in range(2)]
                qkv[p] = [t.astype(BF16) for t in build_qkv(p, y)]

            def do_qk(p):
                er[p] = qk(qkv[p][0], qkv[p][1])

            def do_pv(p):
                o2 = pv(er[p], qkv[p][2])
                o[2 * p], o[2 * p + 1] = build_o(p, o2)

            for p in range(NP):
                do_qkv(p)
                if p >= 1:
                    do_qk(p - 1)
                if p >= 3:
                    do_pv(p - 3)
            fillers[0]()
            do_qk(NP - 1)
            do_pv(NP - 3)
            do_pv(NP - 2)
            olo = jnp.concatenate(o[:2 * KSPLIT], axis=1)
            acc = [_dot(olo, wo_ref[n, 0:KS, :]) for n in range(ND // 2)]
            do_pv(NP - 1)
            acc += [_dot(olo, wo_ref[n, 0:KS, :]) for n in range(ND // 2, ND)]
            ohi = jnp.concatenate(o[2 * KSPLIT:], axis=1)
            res = jnp.concatenate(
                [_dot(ohi, wo_ref[n, KS:, :]) + acc[n] for n in range(ND)], axis=1)
            fillers[1]()
            return res

        saved = [None] * NP
        o_saved = [None] * H

        def build_qkv_a(p, y):
            saved[p] = [[y[hh][m][40:48] for m in range(3)] for hh in range(2)]
            return [jnp.concatenate([y[0][m][0:40], y[1][m][0:40]], axis=0) for m in range(3)]

        def build_o_a(p, o2):
            o_saved[2 * p] = o2[32:40]
            o_saved[2 * p + 1] = o2[72:80]
            return o2[0:32].astype(BF16), o2[40:72].astype(BF16)

        def build_qkv_b(p, y):
            return [jnp.concatenate([y[0][m][0:8], saved[p][0][m], y[0][m][8:32],
                                     y[1][m][0:8], saved[p][1][m], y[1][m][8:32]], axis=0)
                    for m in range(3)]

        def build_o_b(p, o2):
            return (jnp.concatenate([o2[0:8], o_saved[2 * p], o2[8:40]], axis=0).astype(BF16),
                    jnp.concatenate([o2[40:48], o_saved[2 * p + 1], o2[48:80]], axis=0).astype(BF16))

        mlp_up(range(CPRE, CPRE + 4))
        combine(rprev)
        sa = segment(lhs_a, build_qkv_a, build_o_a,
                     [lambda: mlp_up(range(CPRE + 4, CPRE + 12)), lambda: mlp_up(range(CPRE + 12, NF))])
        mem_ref[...] = sa[0:8]
        s_ref[0:24, :] = sa[8:32]
        lhs_b = jnp.concatenate([sa[0:8], xn[40:64]], axis=0).astype(BF16)
        sb = segment(lhs_b, build_qkv_b, build_o_b,
                     [lambda: mlp_down(range(0, 4)), lambda: mlp_down(range(4, ND))])
        mem_ref[...] = sb[0:8]
        s_ref[24:64, :] = sb[8:48]

        @pl.when(j > 0)
        def _():
            out_copy(rprev).start()
        return c
    lax.fori_loop(0, S // STEP, step, 0)
    combine(S - STEP)
    out_copy(S - STEP).start()
    pltpu.make_async_copy(x_ref, out_hbm, sems.at[SEM_OUT]).wait()


@functools.partial(jax.jit, static_argnames=("A_seg_len",))
def pallas_recurrent_scan__memory_aug_recurrent_mem_tr__mixer_s_mlp__prompt_kernel(
        A_x, A_mem0, A_Wq, A_Wk, A_Wv, A_Wo, A_seg_len, B_x, B_w1, B_w2, B_w3, B_w4):
    _, S, D = A_x.shape
    _, H, DH = A_Wq.shape
    M = A_mem0.shape[1]
    FF = B_w3.shape[1]
    kern = functools.partial(_kernel, S=S, D=D, H=H, DH=DH, M=M, SEG=A_seg_len, FF=FF)
    any_spec = pl.BlockSpec(memory_space=pl.ANY)
    vmem_spec = pl.BlockSpec(memory_space=pltpu.VMEM)
    nit = S // (SUB * NSUB)
    out = pl.pallas_call(
        kern,
        out_shape=jax.ShapeDtypeStruct((S, D), A_x.dtype),
        in_specs=[any_spec, vmem_spec] + [any_spec] * 8,
        out_specs=any_spec,
        scratch_shapes=[
            pltpu.VMEM((S, D), BF16),
            pltpu.VMEM((3 * H // 2, D, 128), U32),
            pltpu.VMEM((3 * H, D // 2, 128), U32),
            pltpu.VMEM((D // 128, H * DH // 2, 128), U32),
            pltpu.VMEM((D // 128, D // 2, 128), U32),
            pltpu.VMEM((D // 128, D // 2, 128), U32),
            pltpu.VMEM((FF // 128, D // 2, 128), U32),
            pltpu.VMEM((D // 128, FF // 2, 128), U32),
            pltpu.VMEM((D // 128, S + 16, 128), F32),
            pltpu.VMEM((S, D), F32),
            pltpu.VMEM((S // 2, D), U32),
            pltpu.VMEM((SUB // 2, D), U32),
            pltpu.VMEM((STEP, D), F32),
            pltpu.VMEM((M, D), F32),
            pltpu.SemaphoreType.DMA((9 + 2 * nit,)),
        ],
        compiler_params=pltpu.CompilerParams(vmem_limit_bytes=120 * 1024 * 1024),
    )(A_x[0], A_mem0[0], A_Wq, A_Wk, A_Wv, A_Wo.reshape(H * DH, D), B_w1, B_w2, B_w3, B_w4)
    return out[None]
```

```python
import functools
import jax
import jax.numpy as jnp
from jax import lax
import jax.experimental.pallas as pl
import jax.experimental.pallas.tpu as pltpu

F32 = jnp.float32
BF16 = jnp.bfloat16
U32 = jnp.uint32
EPS = 1e-5
LOG2E = 1.4426950408889634

SUB = 64
NSUB = 512 // SUB
CPRE = 6
XK = 448
NPRE = 2
W1G = ((0, 2), (2, 5), (5, 8))
XCH = ((0, 256), (256, 320), (320, 704), (704, 1152), (1152, 1600), (1600, 2048))
STEP = 64


def _ln(x):
    m = jnp.mean(x, axis=-1, keepdims=True)
    xc = x - m
    v = jnp.mean(xc * xc, axis=-1, keepdims=True)
    return xc * lax.rsqrt(v + EPS)


def _gelu(x):
    c = 0.7978845608028654
    return 0.5 * x * (1.0 + jnp.tanh(c * (x + 0.044715 * (x * x * x))))


def _bf(w_u32):
    return pltpu.bitcast(w_u32, BF16)


def _pk(x):
    return pltpu.bitcast(x.astype(BF16), U32)


def _dot(a, w_u32):
    return jnp.dot(a, _bf(w_u32), preferred_element_type=F32)


def _kernel(x_hbm, mem0_hbm, wq_hbm, wk_hbm, wv_hbm, wo_hbm, w1_hbm, w2_hbm, w3_hbm, w4_hbm, out_hbm,
            x_ref, stage, wqkv_ref, wo_ref, w1_ref, w2_ref, w3_ref, w4_ref,
            h_ref, b_ref, a3_ref, pre_ref, s_ref, mem0_ref, mem_ref, sems, *, S, D, H, DH, M, SEG, FF):
    L = M + SEG
    R = 2 * L
    NP = H // 2
    ND = D // 128
    NF = FF // 128
    C4 = D // 4
    RB = SUB * NSUB
    NIT = S // RB
    NSLAB = 3 * NP
    SLAB_IT = NSLAB // NIT

    SEM_W2, SEM_W3A, SEM_W4A, SEM_WO, SEM_W3B, SEM_W4B, SEM_OUT, SEM_MEM = range(8)
    SEM_W1 = 8
    SEM_X = SEM_W1 + ND
    SEM_SLAB = SEM_X + len(XCH)
    JG = NP // NIT
    W3X = (NF - CPRE) % NIT
    W3G = (NF - CPRE) // NIT
    NG = ND // NIT

    def col_copy(src, dst, j, sem, rows=None):
        s32 = src.bitcast(U32)
        cols = pl.ds(pl.multiple_of(j * 128, 128), 128)
        if rows is None:
            return pltpu.make_async_copy(s32.at[:, cols], dst.at[j], sem)
        return pltpu.make_async_copy(s32.at[pl.ds(*rows), cols], dst.at[j, pl.ds(*rows)], sem)

    def slab_group(i):
        return [pltpu.make_async_copy(w.bitcast(U32).at[:, i * JG + k, :], stage.at[m * NP + i * JG + k],
                                      sems.at[SEM_SLAB + i])
                for m, w in enumerate((wq_hbm, wk_hbm, wv_hbm)) for k in range(JG)]

    w4a_rows = (0, CPRE * 64)
    w4b_rows = (CPRE * 64, (NF - CPRE) * 64)

    def late_group(i):
        return ([col_copy(wo_hbm, wo_ref, i * NG + k, sems.at[SEM_WO]) for k in range(NG)]
                + [col_copy(w3_hbm, w3_ref, CPRE + W3X + i * W3G + k, sems.at[SEM_W3B]) for k in range(W3G)]
                + [col_copy(w4_hbm, w4_ref, i * NG + k, sems.at[SEM_W4B], w4b_rows) for k in range(NG)])

    g_mem = [pltpu.make_async_copy(mem0_hbm, mem0_ref, sems.at[SEM_MEM])]
    g_x = [pltpu.make_async_copy(x_hbm.at[pl.ds(lo, hi - lo)], x_ref.at[pl.ds(lo, hi - lo)], sems.at[SEM_X + i])
           for i, (lo, hi) in enumerate(XCH)]
    g_w1 = [col_copy(w1_hbm, w1_ref, j, sems.at[SEM_W1 + j]) for j in range(ND)]
    g_w2 = [col_copy(w2_hbm, w2_ref, j, sems.at[SEM_W2]) for j in range(ND)]
    g_w3a = [col_copy(w3_hbm, w3_ref, j, sems.at[SEM_W3A]) for j in range(CPRE)]
    g_w4a = [col_copy(w4_hbm, w4_ref, j, sems.at[SEM_W4A], w4a_rows) for j in range(ND)]
    g_w3x = [col_copy(w3_hbm, w3_ref, j, sems.at[SEM_W3B]) for j in range(CPRE, CPRE + W3X)]

    def start(*gs):
        for g in gs:
            for cp in g:
                cp.start()

    def wait(*gs):
        for g in gs:
            for cp in g:
                cp.wait()

    start(g_x[0:1], g_w1[0:5], g_x[1:2], g_w1[5:], g_x[2:], g_w2, g_w3a, g_w4a, g_mem, slab_group(0))

    h_ref[:, 0:8, :] = jnp.zeros((ND, 8, 128), F32)
    h_ref[:, S + 8:S + 16, :] = jnp.zeros((ND, 8, 128), F32)
    s_ref[...] = jnp.zeros(s_ref.shape, F32)

    def ln2(r):
        xn = _ln(x_ref[pl.ds(r, SUB), :].astype(F32))
        b_ref[pl.ds(r, SUB), :] = xn
        return _ln(xn)

    def h_dot(a, r, j):
        h_ref[j, pl.ds(r + 8, SUB), :] = _gelu(_dot(a, w1_ref[j]))

    def p1_rows(base, a, s0):
        for s in range(s0, NSUB):
            if s + 1 < NSUB:
                a_next = ln2(base + (s + 1) * SUB).astype(BF16)
            for j in range(ND):
                h_dot(a, base + s * SUB, j)
            if s + 1 < NSUB:
                a = a_next
        nxt = pl.multiple_of(jnp.minimum(base + RB, S - SUB), SUB)
        pre_ref[...] = _pk(ln2(nxt))

    NA = XCH[0][1] // SUB
    wait(g_x[0:1])
    a0 = [ln2(s * SUB).astype(BF16) for s in range(NPRE)]
    for gi, (j0, j1) in enumerate(W1G):
        wait(g_w1[j0:j1])
        if gi == len(W1G) - 1:
            wait(g_x[1:2])
            a_n = ln2(NA * SUB).astype(BF16)
        for s in range(NA):
            if s == len(a0):
                a0.append(ln2(s * SUB).astype(BF16))
            for j in range(j0, j1):
                h_dot(a0[s], s * SUB, j)
    wait(g_x[2:3])
    p1_rows(0, a_n, NA)

    def p1(i, c):
        lo = pl.multiple_of(XCH[2][1] + (i - 1) * XK, 64)
        pltpu.make_async_copy(x_hbm.at[pl.ds(lo, XK)], x_ref.at[pl.ds(lo, XK)], sems.at[SEM_X + 2 + i]).wait()
        start(slab_group(i))
        p1_rows(pl.multiple_of(i * RB, RB), _bf(pre_ref[...]), 0)
        return c
    lax.fori_loop(1, NIT, p1, 0)

    def build_g(r):
        offs = (7, 9, 6, 10)
        return jnp.concatenate(
            [h_ref[j, pl.ds(r + offs[j * 128 // C4], SUB), :] for j in range(ND)], axis=1)

    pre_ref[...] = _pk(build_g(0))
    start(g_w3x)
    wait(g_w2, g_w3a, g_w4a, g_mem)
    mem_ref[...] = mem0_ref[...].astype(F32)

    def p23(it, c):
        base = pl.multiple_of(it * RB, RB)
        wait(slab_group(it))
        start(late_group(it))

        g = [None] * NSUB
        x1 = [None] * NSUB
        a3 = [None] * NSUB
        u = [None] * NSUB
        g[0] = _bf(pre_ref[...])

        items = [(k, i) for k in range(SLAB_IT) for i in range(D // 16)]
        nties = NSUB * (2 * ND + CPRE) - ND
        per = -(-len(items) // nties)

        def tie(y):
            z = (pltpu.bitcast(y[0:8, :], U32) >> 31) >> 1
            mlo = z + U32(0xFFFF)
            mhi = z + U32(0xFFFF0000)
            for _ in range(per):
                if not items:
                    break
                k, i = items.pop(0)
                slab = (k // JG) * NP + it * JG + k % JG
                a = stage[slab, pl.ds(i * 16, 8, stride=2), :]
                b = stage[slab, pl.ds(i * 16 + 1, 8, stride=2), :]
                wqkv_ref[2 * slab, i * 8:(i + 1) * 8, :] = (a & mlo) | (b << 16)
                wqkv_ref[2 * slab + 1, i * 8:(i + 1) * 8, :] = (a >> 16) | (b & mhi)

        def m2(s):
            if s + 1 < NSUB:
                g[s + 1] = build_g(base + (s + 1) * SUB).astype(BF16)
            ys = []
            for j in range(ND):
                ys.append(_dot(g[s], w2_ref[j]))
                tie(ys[-1])
            x1[s] = jnp.concatenate(ys, axis=1) + b_ref[pl.ds(base + s * SUB, SUB), :]
            a3[s] = _ln(x1[s]).astype(BF16)
            r2 = pl.multiple_of(it * (RB // 2) + s * (SUB // 2), SUB // 2)
            a3_ref[pl.ds(r2, SUB // 2), :] = pltpu.bitcast(a3[s], U32)

        def up(s):
            us = []
            for f in range(CPRE):
                y = _dot(a3[s], w3_ref[f])
                tie(y)
                us.append(_gelu(y).astype(BF16))
            u[s] = jnp.concatenate(us, axis=1)

        def down(s):
            for n in range(ND):
                y = _dot(u[s], w4_ref[n, 0:CPRE * 64, :]) + x1[s][:, n * 128:(n + 1) * 128]
                tie(y)
                b_ref[pl.ds(base + s * SUB, SUB), n * 128:(n + 1) * 128] = y

        for s in range(NSUB):
            m2(s)
            if s >= 1:
                up(s - 1)
            if s >= 2:
                down(s - 2)
        nxt = pl.multiple_of(jnp.minimum(base + RB, S - SUB), SUB)
        pre_ref[...] = _pk(build_g(nxt))
        down(NSUB - 2); up(NSUB - 1); down(NSUB - 1)
        assert not items
        return c
    lax.fori_loop(0, NIT, p23, 0)
    wait(g_w3x)
    for i in range(NIT):
        wait(late_group(i))

    row = lax.broadcasted_iota(jnp.int32, (R, R), 0)
    col = lax.broadcasted_iota(jnp.int32, (R, R), 1)
    same = (row >= L) == (col >= L)
    rr = jnp.where(row >= L, row - L, row)
    cc = jnp.where(col >= L, col - L, col)
    ok = same & ((rr < M) | (rr >= cc))
    scale = DH ** -0.5
    fill = jnp.where(same, -1e9 / scale, -jnp.inf).astype(F32)
    cexp = scale * LOG2E

    def qk(q2, k2):
        s = lax.dot_general(q2, k2, (((1,), (1,)), ((), ())), preferred_element_type=F32)
        s = jnp.where(ok, s, fill)
        m = jnp.max(s, axis=-1, keepdims=True)
        e = jnp.exp2((s - m) * cexp)
        l = jnp.sum(e, axis=-1, keepdims=True)
        r = pl.reciprocal(l, approx=True)
        r = r * (2.0 - l * r)
        return (e * r).astype(BF16)

    def pv(p, v2):
        return jnp.dot(p, v2, preferred_element_type=F32)

    def combine(r):
        b = b_ref[pl.ds(r, STEP), :]
        g = b * jax.nn.sigmoid(b)
        x = x_ref[pl.ds(r, STEP), :].astype(F32)
        x_ref[pl.ds(r, STEP), :] = (x + s_ref[...] * g).astype(x_ref.dtype)

    def out_copy(r):
        return pltpu.make_async_copy(x_ref.at[pl.ds(r, STEP)], out_hbm.at[pl.ds(r, STEP)], sems.at[SEM_OUT])

    def step(j, c):
        r0 = pl.multiple_of(j * STEP, STEP)
        rprev = pl.multiple_of(jnp.maximum(r0 - STEP, 0), STEP)
        a3 = _bf(a3_ref[pl.ds(pl.multiple_of(j * (STEP // 2), STEP // 2), STEP // 2), :])
        xn = _ln(x_ref[pl.ds(r0, STEP), :].astype(F32))
        mem = mem_ref[...]
        lhs_a = jnp.concatenate([mem, xn[0:40]], axis=0).astype(BF16)

        u = [None] * NF

        def mlp_up(fs):
            for f in fs:
                u[f] = _gelu(_dot(a3, w3_ref[f])).astype(BF16)

        half = {}

        def mlp_up_half(f, hi):
            if not hi:
                half[f] = _dot(a3[:, 0:D // 2], w3_ref[f, 0:D // 4, :])
            else:
                u[f] = _gelu(_dot(a3[:, D // 2:], w3_ref[f, D // 4:, :]) + half[f]).astype(BF16)

        def mlp_down(ns):
            uu = jnp.concatenate(u[CPRE:], axis=1)
            for n in ns:
                b_ref[pl.ds(r0, STEP), n * 128:(n + 1) * 128] = (
                    _dot(uu, w4_ref[n, CPRE * 64:, :]) + b_ref[pl.ds(r0, STEP), n * 128:(n + 1) * 128])

        def segment(lhs, build_qkv, build_o, fillers, inter=None):
            qkv = [None] * NP
            er = [None] * NP
            o = [None] * H
            KSPLIT = NP - 3
            KS = KSPLIT * 128

            def do_qkv(p):
                y = [[_dot(lhs, wqkv_ref[m * H + 2 * p + hh]) for m in range(3)] for hh in range(2)]
                qkv[p] = [t.astype(BF16) for t in build_qkv(p, y)]

            def do_qk(p):
                er[p] = qk(qkv[p][0], qkv[p][1])

            def do_pv(p):
                o2 = pv(er[p], qkv[p][2])
                o[2 * p], o[2 * p + 1] = build_o(p, o2)

            for p in range(NP):
                do_qkv(p)
                if inter is not None:
                    inter(p)
                if p >= 1:
                    do_qk(p - 1)
                if p >= 3:
                    do_pv(p - 3)
            fillers[0]()
            do_qk(NP - 1)
            do_pv(NP - 3)
            do_pv(NP - 2)
            olo = jnp.concatenate(o[:2 * KSPLIT], axis=1)
            acc = [_dot(olo, wo_ref[n, 0:KS, :]) for n in range(ND // 2)]
            do_pv(NP - 1)
            acc += [_dot(olo, wo_ref[n, 0:KS, :]) for n in range(ND // 2, ND)]
            ohi = jnp.concatenate(o[2 * KSPLIT:], axis=1)
            res = jnp.concatenate(
                [_dot(ohi, wo_ref[n, KS:, :]) + acc[n] for n in range(ND)], axis=1)
            fillers[1]()
            return res

        saved = [None] * NP
        o_saved = [None] * H

        def build_qkv_a(p, y):
            saved[p] = [[y[hh][m][40:48] for m in range(3)] for hh in range(2)]
            return [jnp.concatenate([y[0][m][0:40], y[1][m][0:40]], axis=0) for m in range(3)]

        def build_o_a(p, o2):
            o_saved[2 * p] = o2[32:40]
            o_saved[2 * p + 1] = o2[72:80]
            return o2[0:32].astype(BF16), o2[40:72].astype(BF16)

        def build_qkv_b(p, y):
            return [jnp.concatenate([y[0][m][0:8], saved[p][0][m], y[0][m][8:32],
                                     y[1][m][0:8], saved[p][1][m], y[1][m][8:32]], axis=0)
                    for m in range(3)]

        def build_o_b(p, o2):
            return (jnp.concatenate([o2[0:8], o_saved[2 * p], o2[8:40]], axis=0).astype(BF16),
                    jnp.concatenate([o2[40:48], o_saved[2 * p + 1], o2[48:80]], axis=0).astype(BF16))

        mlp_up(range(CPRE, CPRE + 4))
        combine(rprev)
        sa = segment(lhs_a, build_qkv_a, build_o_a,
                     [lambda: mlp_up(range(CPRE + 4, CPRE + 8)), lambda: mlp_up(range(CPRE + 8, NF - 8))])
        mem_ref[...] = sa[0:8]
        s_ref[0:24, :] = sa[8:32]
        lhs_b = jnp.concatenate([sa[0:8], xn[40:64]], axis=0).astype(BF16)
        sb = segment(lhs_b, build_qkv_b, build_o_b,
                     [lambda: mlp_down(range(0, 4)), lambda: mlp_down(range(4, ND))],
                     inter=lambda p: mlp_up_half(NF - 8 + p // 2, p % 2))
        mem_ref[...] = sb[0:8]
        s_ref[24:64, :] = sb[8:48]

        @pl.when(j > 0)
        def _():
            out_copy(rprev).start()
        return c
    lax.fori_loop(0, S // STEP, step, 0)
    combine(S - STEP)
    out_copy(S - STEP).start()
    pltpu.make_async_copy(x_ref, out_hbm, sems.at[SEM_OUT]).wait()


@functools.partial(jax.jit, static_argnames=("A_seg_len",))
def pallas_recurrent_scan__memory_aug_recurrent_mem_tr__mixer_s_mlp__prompt_kernel(
        A_x, A_mem0, A_Wq, A_Wk, A_Wv, A_Wo, A_seg_len, B_x, B_w1, B_w2, B_w3, B_w4):
    _, S, D = A_x.shape
    _, H, DH = A_Wq.shape
    M = A_mem0.shape[1]
    FF = B_w3.shape[1]
    kern = functools.partial(_kernel, S=S, D=D, H=H, DH=DH, M=M, SEG=A_seg_len, FF=FF)
    any_spec = pl.BlockSpec(memory_space=pl.ANY)
    vmem_spec = pl.BlockSpec(memory_space=pltpu.VMEM)
    nit = S // (SUB * NSUB)
    out = pl.pallas_call(
        kern,
        out_shape=jax.ShapeDtypeStruct((S, D), A_x.dtype),
        in_specs=[any_spec] * 10,
        out_specs=any_spec,
        scratch_shapes=[
            pltpu.VMEM((S, D), BF16),
            pltpu.VMEM((3 * H // 2, D, 128), U32),
            pltpu.VMEM((3 * H, D // 2, 128), U32),
            pltpu.VMEM((D // 128, H * DH // 2, 128), U32),
            pltpu.VMEM((D // 128, D // 2, 128), U32),
            pltpu.VMEM((D // 128, D // 2, 128), U32),
            pltpu.VMEM((FF // 128, D // 2, 128), U32),
            pltpu.VMEM((D // 128, FF // 2, 128), U32),
            pltpu.VMEM((D // 128, S + 16, 128), F32),
            pltpu.VMEM((S, D), F32),
            pltpu.VMEM((S // 2, D), U32),
            pltpu.VMEM((SUB // 2, D), U32),
            pltpu.VMEM((STEP, D), F32),
            pltpu.VMEM((M, D), BF16),
            pltpu.VMEM((M, D), F32),
            pltpu.SemaphoreType.DMA((8 + D // 128 + len(XCH) + nit,)),
        ],
        compiler_params=pltpu.CompilerParams(vmem_limit_bytes=120 * 1024 * 1024, disable_bounds_checks=True),
    )(A_x[0], A_mem0[0], A_Wq, A_Wk, A_Wv, A_Wo.reshape(H * DH, D), B_w1, B_w2, B_w3, B_w4)
    return out[None]
```

```python
import functools

import jax
import jax.numpy as jnp
from jax import lax
import jax.experimental.pallas as pl
import jax.experimental.pallas.tpu as pltpu

F32 = jnp.float32
BF16 = jnp.bfloat16
U32 = jnp.uint32
EPS = 1e-5
LOG2E = 1.4426950408889634

SUB = 64
NSUB = 8
CPRE = 6
STEP = 64
NPRE = 2
W1G = ((0, 2), (2, 5), (5, 8))
XK = 448
XCH = ((0, 256), (256, 320), (320, 704), (704, 1152), (1152, 1600), (1600, 2048))


def _ln(x):
    m = jnp.mean(x, axis=-1, keepdims=True)
    xc = x - m
    v = jnp.mean(xc * xc, axis=-1, keepdims=True)
    return xc * lax.rsqrt(v + EPS)


def _gelu(x):
    c = 0.7978845608028654
    return 0.5 * x * (1.0 + jnp.tanh(c * (x + 0.044715 * (x * x * x))))


def _bf(w_u32):
    return pltpu.bitcast(w_u32, BF16)


def _pk(x):
    return pltpu.bitcast(x.astype(BF16), U32)


def _dot(a, w_u32):
    return jnp.dot(a, _bf(w_u32), preferred_element_type=F32)


def _kernel(x_hbm, mem0_hbm, wq_hbm, wk_hbm, wv_hbm, wo_hbm, w1_hbm, w2_hbm, w3_hbm, w4_hbm, out_hbm,
            x_ref, o_ref, stage, wqkv_ref, wo_ref, w1_ref, w2_ref, w3_ref, w4_ref,
            h_ref, b_ref, a3_ref, pre_ref, s_ref, mem0_ref, mem_ref, sems, *, S, D, H, DH, M, SEG, FF):
    L = M + SEG
    R = 2 * L
    NP = H // 2
    ND = D // 128
    NF = FF // 128
    RB = SUB * NSUB
    NIT = S // RB

    SEM_W2, SEM_W3A, SEM_W4A, SEM_WO, SEM_W3B, SEM_W4B, SEM_OUT, SEM_MEM = range(8)
    SEM_W1 = 8
    SEM_X = SEM_W1 + ND
    SEM_SLAB = SEM_X + len(XCH)
    JG = NP // NIT
    W3X = (NF - CPRE) % NIT
    W3G = (NF - CPRE) // NIT
    NG = ND // NIT

    def col_copy(src, dst, j, sem, rows=None):
        s32 = src.bitcast(U32)
        cols = pl.ds(pl.multiple_of(j * 128, 128), 128)
        if rows is None:
            return pltpu.make_async_copy(s32.at[:, cols], dst.at[j], sem)
        return pltpu.make_async_copy(s32.at[pl.ds(*rows), cols], dst.at[j, pl.ds(*rows)], sem)

    def x_copy(lo, n, sem):
        return pltpu.make_async_copy(x_hbm.at[pl.ds(lo, n)], x_ref.at[pl.ds(lo, n)], sem)

    def slab_group(i):
        return [pltpu.make_async_copy(w.bitcast(U32).at[:, i * JG + k, :], stage.at[m * NP + i * JG + k],
                                      sems.at[SEM_SLAB + i])
                for m, w in enumerate((wq_hbm, wk_hbm, wv_hbm)) for k in range(JG)]

    w4a_rows = (0, CPRE * 64)
    w4b_rows = (CPRE * 64, (NF - CPRE) * 64)

    def late_group(i):
        return ([col_copy(wo_hbm, wo_ref, i * NG + k, sems.at[SEM_WO]) for k in range(NG)]
                + [col_copy(w3_hbm, w3_ref, CPRE + W3X + i * W3G + k, sems.at[SEM_W3B]) for k in range(W3G)]
                + [col_copy(w4_hbm, w4_ref, i * NG + k, sems.at[SEM_W4B], w4b_rows) for k in range(NG)])

    g_mem = [pltpu.make_async_copy(mem0_hbm, mem0_ref, sems.at[SEM_MEM])]
    g_x = [x_copy(lo, hi - lo, sems.at[SEM_X + i]) for i, (lo, hi) in enumerate(XCH)]
    g_w1 = [col_copy(w1_hbm, w1_ref, j, sems.at[SEM_W1 + j]) for j in range(ND)]
    g_w2 = [col_copy(w2_hbm, w2_ref, j, sems.at[SEM_W2]) for j in range(ND)]
    g_w3a = [col_copy(w3_hbm, w3_ref, j, sems.at[SEM_W3A]) for j in range(CPRE)]
    g_w4a = [col_copy(w4_hbm, w4_ref, j, sems.at[SEM_W4A], w4a_rows) for j in range(ND)]
    g_w3x = [col_copy(w3_hbm, w3_ref, j, sems.at[SEM_W3B]) for j in range(CPRE, CPRE + W3X)]

    def start(*gs):
        for g in gs:
            for cp in g:
                cp.start()

    def wait(*gs):
        for g in gs:
            for cp in g:
                cp.wait()

    start(g_x[0:1], g_w1[0:5], g_x[1:2], g_w1[5:], g_x[2:], g_w2, g_w3a, g_w4a, g_mem, slab_group(0))

    h_ref[:, 0:8, :] = jnp.zeros((ND, 8, 128), F32)
    h_ref[:, S + 8:S + 16, :] = jnp.zeros((ND, 8, 128), F32)
    s_ref[...] = jnp.zeros(s_ref.shape, F32)

    def ln2(r):
        xn = _ln(x_ref[pl.ds(r, SUB), :].astype(F32))
        b_ref[pl.ds(r, SUB), :] = xn
        return _ln(xn)

    def h_dot(a, r, j):
        h_ref[j, pl.ds(r + 8, SUB), :] = _gelu(_dot(a, w1_ref[j]))

    def p1_rows(base, a, s0):
        for s in range(s0, NSUB):
            if s + 1 < NSUB:
                a_next = ln2(base + (s + 1) * SUB).astype(BF16)
            for j in range(ND):
                h_dot(a, base + s * SUB, j)
            if s + 1 < NSUB:
                a = a_next
        nxt = pl.multiple_of(jnp.minimum(base + RB, S - SUB), SUB)
        pre_ref[...] = _pk(ln2(nxt))

    NA = XCH[0][1] // SUB
    wait(g_x[0:1])
    a0 = [ln2(s * SUB).astype(BF16) for s in range(NPRE)]
    for gi, (j0, j1) in enumerate(W1G):
        wait(g_w1[j0:j1])
        if gi == len(W1G) - 1:
            wait(g_x[1:2])
            a_n = ln2(NA * SUB).astype(BF16)
        for s in range(NA):
            if s == len(a0):
                a0.append(ln2(s * SUB).astype(BF16))
            for j in range(j0, j1):
                h_dot(a0[s], s * SUB, j)
    wait(g_x[2:3])
    p1_rows(0, a_n, NA)

    def p1(i, c):
        x_copy(pl.multiple_of(XCH[2][1] + (i - 1) * XK, 64), XK, sems.at[SEM_X + 2 + i]).wait()
        start(slab_group(i))
        p1_rows(pl.multiple_of(i * RB, RB), _bf(pre_ref[...]), 0)
        return c
    lax.fori_loop(1, NIT, p1, 0)

    def shifted(r):
        offs = (7, 9, 6, 10)
        return jnp.concatenate(
            [h_ref[j, pl.ds(r + offs[4 * j // ND], SUB), :] for j in range(ND)], axis=1)

    pre_ref[...] = _pk(shifted(0))
    start(g_w3x)
    wait(g_w2, g_w3a, g_w4a, g_mem)
    mem_ref[...] = mem0_ref[...].astype(F32)

    def p23(it, c):
        base = pl.multiple_of(it * RB, RB)
        wait(slab_group(it))
        start(late_group(it))

        g = [None] * NSUB
        x1 = [None] * NSUB
        a3 = [None] * NSUB
        u = [None] * NSUB
        g[0] = _bf(pre_ref[...])

        items = [(k, i) for k in range(3 * JG) for i in range(D // 16)]
        per = -(-len(items) // (NSUB * (2 * ND + CPRE) - ND))

        def repack_after(y):
            z = (pltpu.bitcast(y[0:8, :], U32) >> 31) >> 1
            mlo = z + U32(0xFFFF)
            mhi = z + U32(0xFFFF0000)
            for _ in range(min(per, len(items))):
                k, i = items.pop(0)
                slab = (k // JG) * NP + it * JG + k % JG
                a = stage[slab, pl.ds(i * 16, 8, stride=2), :]
                b = stage[slab, pl.ds(i * 16 + 1, 8, stride=2), :]
                wqkv_ref[2 * slab, i * 8:(i + 1) * 8, :] = (a & mlo) | (b << 16)
                wqkv_ref[2 * slab + 1, i * 8:(i + 1) * 8, :] = (a >> 16) | (b & mhi)

        def mix(s):
            if s + 1 < NSUB:
                g[s + 1] = shifted(base + (s + 1) * SUB).astype(BF16)
            ys = []
            for j in range(ND):
                ys.append(_dot(g[s], w2_ref[j]))
                repack_after(ys[-1])
            x1[s] = jnp.concatenate(ys, axis=1) + b_ref[pl.ds(base + s * SUB, SUB), :]
            a3[s] = _ln(x1[s]).astype(BF16)
            r2 = pl.multiple_of(it * (RB // 2) + s * (SUB // 2), SUB // 2)
            a3_ref[pl.ds(r2, SUB // 2), :] = pltpu.bitcast(a3[s], U32)

        def up(s):
            us = []
            for f in range(CPRE):
                y = _dot(a3[s], w3_ref[f])
                repack_after(y)
                us.append(_gelu(y).astype(BF16))
            u[s] = jnp.concatenate(us, axis=1)

        def down(s):
            for n in range(ND):
                y = _dot(u[s], w4_ref[n, 0:CPRE * 64, :]) + x1[s][:, n * 128:(n + 1) * 128]
                repack_after(y)
                b_ref[pl.ds(base + s * SUB, SUB), n * 128:(n + 1) * 128] = y

        for s in range(NSUB):
            mix(s)
            if s >= 1:
                up(s - 1)
            if s >= 2:
                down(s - 2)
        nxt = pl.multiple_of(jnp.minimum(base + RB, S - SUB), SUB)
        pre_ref[...] = _pk(shifted(nxt))
        down(NSUB - 2)
        up(NSUB - 1)
        down(NSUB - 1)
        assert not items
        return c
    lax.fori_loop(0, NIT, p23, 0)
    wait(g_w3x, *[late_group(i) for i in range(NIT)])

    row = lax.broadcasted_iota(jnp.int32, (R, R), 0)
    col = lax.broadcasted_iota(jnp.int32, (R, R), 1)
    same_head = (row >= L) == (col >= L)
    rr = jnp.where(row >= L, row - L, row)
    cc = jnp.where(col >= L, col - L, col)
    visible = same_head & ((rr < M) | (rr >= cc))
    scale = DH ** -0.5
    fill = jnp.where(same_head, -1e9 / scale, -jnp.inf).astype(F32)

    def softmax_qk(q2, k2):
        s = lax.dot_general(q2, k2, (((1,), (1,)), ((), ())), preferred_element_type=F32)
        s = jnp.where(visible, s, fill)
        m = jnp.max(s, axis=-1, keepdims=True)
        e = jnp.exp2((s - m) * (scale * LOG2E))
        l = jnp.sum(e, axis=-1, keepdims=True)
        r = pl.reciprocal(l, approx=True)
        r = r * (2.0 - l * r)
        return (e * r).astype(BF16)

    def combine(r):
        b = b_ref[pl.ds(r, STEP), :]
        g = b * jax.nn.sigmoid(b)
        x = x_ref[pl.ds(r, STEP), :].astype(F32)
        o_ref[pl.ds(r, STEP), :] = (x + s_ref[...] * g).astype(o_ref.dtype)

    def out_copy(r):
        return pltpu.make_async_copy(o_ref.at[pl.ds(r, STEP)], out_hbm.at[pl.ds(r, STEP)], sems.at[SEM_OUT])

    def step(j, c):
        r0 = pl.multiple_of(j * STEP, STEP)
        rprev = pl.multiple_of(jnp.maximum(r0 - STEP, 0), STEP)
        a3 = _bf(a3_ref[pl.ds(pl.multiple_of(j * (STEP // 2), STEP // 2), STEP // 2), :])
        xn = _ln(x_ref[pl.ds(r0, STEP), :].astype(F32))

        u = [None] * NF
        half = {}

        def mlp_up(fs):
            for f in fs:
                u[f] = _gelu(_dot(a3, w3_ref[f])).astype(BF16)

        def mlp_up_half(f, hi):
            if not hi:
                half[f] = _dot(a3[:, 0:D // 2], w3_ref[f, 0:D // 4, :])
            else:
                u[f] = _gelu(_dot(a3[:, D // 2:], w3_ref[f, D // 4:, :]) + half[f]).astype(BF16)

        def mlp_down(ns):
            uu = jnp.concatenate(u[CPRE:], axis=1)
            for n in ns:
                cols = slice(n * 128, (n + 1) * 128)
                b_ref[pl.ds(r0, STEP), cols] = _dot(uu, w4_ref[n, CPRE * 64:, :]) + b_ref[pl.ds(r0, STEP), cols]

        def segment(lhs, build_qkv, build_o, fillers, inter=None):
            qkv = [None] * NP
            prob = [None] * NP
            o = [None] * H
            ph = NP - 3
            ks = ph * 128

            def do_qkv(p):
                y = [[_dot(lhs, wqkv_ref[m * H + 2 * p + hh]) for m in range(3)] for hh in range(2)]
                qkv[p] = [t.astype(BF16) for t in build_qkv(p, y)]

            def do_qk(p):
                prob[p] = softmax_qk(qkv[p][0], qkv[p][1])

            def do_pv(p):
                o2 = jnp.dot(prob[p], qkv[p][2], preferred_element_type=F32)
                o[2 * p], o[2 * p + 1] = build_o(p, o2)

            for p in range(NP):
                do_qkv(p)
                if inter is not None:
                    inter(p)
                if p >= 1:
                    do_qk(p - 1)
                if p >= 3:
                    do_pv(p - 3)
            fillers[0]()
            do_qk(NP - 1)
            do_pv(NP - 3)
            do_pv(NP - 2)
            olo = jnp.concatenate(o[:2 * ph], axis=1)
            acc = [_dot(olo, wo_ref[n, 0:ks, :]) for n in range(ND // 2)]
            do_pv(NP - 1)
            acc += [_dot(olo, wo_ref[n, 0:ks, :]) for n in range(ND // 2, ND)]
            ohi = jnp.concatenate(o[2 * ph:], axis=1)
            res = jnp.concatenate([_dot(ohi, wo_ref[n, ks:, :]) + acc[n] for n in range(ND)], axis=1)
            fillers[1]()
            return res

        qkv_kept = [None] * NP
        o_kept = [None] * H

        def build_qkv_a(p, y):
            qkv_kept[p] = [[y[hh][m][40:48] for m in range(3)] for hh in range(2)]
            return [jnp.concatenate([y[0][m][0:40], y[1][m][0:40]], axis=0) for m in range(3)]

        def build_o_a(p, o2):
            o_kept[2 * p] = o2[32:40]
            o_kept[2 * p + 1] = o2[72:80]
            return o2[0:32].astype(BF16), o2[40:72].astype(BF16)

        def build_qkv_b(p, y):
            return [jnp.concatenate([y[0][m][0:8], qkv_kept[p][0][m], y[0][m][8:32],
                                     y[1][m][0:8], qkv_kept[p][1][m], y[1][m][8:32]], axis=0)
                    for m in range(3)]

        def build_o_b(p, o2):
            return (jnp.concatenate([o2[0:8], o_kept[2 * p], o2[8:40]], axis=0).astype(BF16),
                    jnp.concatenate([o2[40:48], o_kept[2 * p + 1], o2[48:80]], axis=0).astype(BF16))

        lhs_a = jnp.concatenate([mem_ref[...], xn[0:40]], axis=0).astype(BF16)
        mlp_up(range(CPRE, CPRE + 4))
        combine(rprev)
        sa = segment(lhs_a, build_qkv_a, build_o_a,
                     [lambda: mlp_up(range(CPRE + 4, CPRE + 8)), lambda: mlp_up(range(CPRE + 8, NF - NP // 2))])
        mem_ref[...] = sa[0:8]
        s_ref[0:24, :] = sa[8:32]
        lhs_b = jnp.concatenate([sa[0:8], xn[40:64]], axis=0).astype(BF16)
        sb = segment(lhs_b, build_qkv_b, build_o_b,
                     [lambda: mlp_down(range(0, ND // 2)), lambda: mlp_down(range(ND // 2, ND))],
                     inter=lambda p: mlp_up_half(NF - NP // 2 + p // 2, p % 2))
        mem_ref[...] = sb[0:8]
        s_ref[24:64, :] = sb[8:48]

        @pl.when(j > 0)
        def _():
            out_copy(rprev).start()
        return c
    lax.fori_loop(0, S // STEP, step, 0)
    combine(S - STEP)
    out_copy(S - STEP).start()
    pltpu.make_async_copy(o_ref, out_hbm, sems.at[SEM_OUT]).wait()


@functools.partial(jax.jit, static_argnames=("A_seg_len",))
def pallas_recurrent_scan__memory_aug_recurrent_mem_tr__mixer_s_mlp__prompt_kernel(
        A_x, A_mem0, A_Wq, A_Wk, A_Wv, A_Wo, A_seg_len, B_x, B_w1, B_w2, B_w3, B_w4):
    del B_x
    B, S, D = A_x.shape
    _, H, DH = A_Wq.shape
    M = A_mem0.shape[1]
    FF = B_w3.shape[1]
    assert (B, S, D, H, DH, M, A_seg_len) == (1, XCH[-1][1], 1024, 32, 128, 8, 32) and FF % 128 == 0
    kern = functools.partial(_kernel, S=S, D=D, H=H, DH=DH, M=M, SEG=A_seg_len, FF=FF)
    any_spec = pl.BlockSpec(memory_space=pl.ANY)
    out = pl.pallas_call(
        kern,
        out_shape=jax.ShapeDtypeStruct((S, D), A_x.dtype),
        in_specs=[any_spec] * 10,
        out_specs=any_spec,
        scratch_shapes=[
            pltpu.VMEM((S, D), BF16),
            pltpu.VMEM((S, D), BF16),
            pltpu.VMEM((3 * H // 2, D, 128), U32),
            pltpu.VMEM((3 * H, D // 2, 128), U32),
            pltpu.VMEM((D // 128, H * DH // 2, 128), U32),
            pltpu.VMEM((D // 128, D // 2, 128), U32),
            pltpu.VMEM((D // 128, D // 2, 128), U32),
            pltpu.VMEM((FF // 128, D // 2, 128), U32),
            pltpu.VMEM((D // 128, FF // 2, 128), U32),
            pltpu.VMEM((D // 128, S + 16, 128), F32),
            pltpu.VMEM((S, D), F32),
            pltpu.VMEM((S // 2, D), U32),
            pltpu.VMEM((SUB // 2, D), U32),
            pltpu.VMEM((STEP, D), F32),
            pltpu.VMEM((M, D), BF16),
            pltpu.VMEM((M, D), F32),
            pltpu.SemaphoreType.DMA((8 + D // 128 + len(XCH) + S // (SUB * NSUB),)),
        ],
        compiler_params=pltpu.CompilerParams(vmem_limit_bytes=120 * 1024 * 1024,
                                             disable_bounds_checks=True),
    )(A_x[0], A_mem0[0], A_Wq, A_Wk, A_Wv, A_Wo.reshape(H * DH, D), B_w1, B_w2, B_w3, B_w4)
    return out[None]
```

```python
import functools

import jax
import jax.numpy as jnp
from jax import lax
import jax.experimental.pallas as pl
import jax.experimental.pallas.tpu as pltpu

F32 = jnp.float32
BF16 = jnp.bfloat16
U32 = jnp.uint32
EPS = 1e-5
LOG2E = 1.4426950408889634

HB = 64
BLK = 2 * HB
RB0 = 512
RA = 256
RB1 = 256
RB2 = 512
CPRE = 8
STEP = 64
NPRE = 2
W1G = ((0, 2), (2, 5), (5, 8))
XK = 192
CH = 16


def _ln(x):
    m = jnp.mean(x, axis=-1, keepdims=True)
    xc = x - m
    v = jnp.mean(xc * xc, axis=-1, keepdims=True)
    return xc * lax.rsqrt(v + EPS)


def _gelu(x):
    c = 0.7978845608028654
    return 0.5 * x * (1.0 + jnp.tanh(c * (x + 0.044715 * (x * x * x))))


def _bf(w_u32):
    return pltpu.bitcast(w_u32, BF16)


def _pk(x):
    return pltpu.bitcast(x.astype(BF16), U32)


def _dot(a, w_u32):
    return jnp.dot(a, _bf(w_u32), preferred_element_type=F32)


def _zero_of(y):
    if y.dtype != U32:
        y = pltpu.bitcast(y[0:(8 if y.dtype == F32 else 16), 0:128], U32)
    return (y[0:8, 0:128] >> 31) >> 1


def _after(y, z):
    return jnp.concatenate([y[0:8] + pltpu.bitcast(z, F32), y[8:]], axis=0)


def _left(get, nk):
    rows, zs = [], []
    for r in range(0, HB, CH):
        cols = []
        for t in range(nk):
            a11, a12, a21, a22 = get(r, t), get(r, nk + t), get(HB + r, t), get(HB + r, nk + t)
            p = [y.astype(BF16) for y in (a11 + a22, a21 + a22, a11, a22, a11 + a12, a21 - a11, a12 - a22)]
            zs.append(_zero_of(functools.reduce(jnp.bitwise_or, [pltpu.bitcast(y, U32) for y in p])))
            cols.append(p)
        rows.append(_cat(cols, 1))
    return _cat(rows, 0), zs


def _cat(parts, axis):
    return [jnp.concatenate([p[t] for p in parts], axis=axis) for t in range(7)]


def _right_sums(b11, b21, b12, b22):
    b11, b21, b12, b22 = [_bf(t).astype(F32) for t in (b11, b21, b12, b22)]
    return [_pk(t) for t in (b21 - b11, b12 - b22, b11 + b22, b11 + b12, b21 + b22)]


class _Pace:
    def __init__(self):
        self.items, self.per, self.before = [], 0, []

    def spread(self, items, nslots):
        self.items, self.per, self.credit = list(items), len(items) / nslots, 0.0

    def require(self, zeros, nslots):
        self.before += [None] * (nslots - len(self.before))
        for i, z in enumerate(zeros):
            k = (i + 1) * nslots // len(zeros) - 1
            self.before[k] = z if self.before[k] is None else self.before[k] | z

    def __call__(self, y):
        if self.items:
            self.credit += self.per
            n = min(int(self.credit + 1e-6), len(self.items))
            self.credit -= n
            if n:
                z = _zero_of(y)
                for _ in range(n):
                    self.items.pop(0)(z)
        if self.before:
            z = self.before.pop(0)
            if z is not None:
                y = _after(y, z)
        return y


def _strassen(al, wt, pace=lambda y: y):
    m1 = pace(_dot(al[0], wt(4)))
    yield None
    m4 = pace(_dot(al[3], wt(1)))
    yield None
    m5 = pace(_dot(al[4], wt(3)))
    yield None
    m2 = pace(_dot(al[1], wt(0)))
    yield None
    m3 = pace(_dot(al[2], wt(2)))
    yield None
    c11 = pace(_dot(al[6], wt(6)) + (m1 + m4 - m5))
    yield None
    c22 = pace(_dot(al[5], wt(5)) + (m1 - m2 + m3))
    yield (jnp.concatenate([c11, m2 + m4], axis=0), jnp.concatenate([m3 + m5, c22], axis=0))


def _run(gen):
    for y in gen:
        pass
    return y


def _gelu_left(y0, y1):
    return _left(lambda r, t: _gelu((y0, y1)[t][r:r + CH]), 1)


def _kernel(x_hbm, mem0_hbm, wq_hbm, wk_hbm, wv_hbm, wo_hbm, w1_hbm, w2_hbm, w3_hbm, w4_hbm, out_hbm,
            x_ref, stage, wqkv_ref, wo_ref, w1_ref, q_ref, p_ref, r_ref,
            h_ref, b_ref, a3_ref, pre_ref, s_ref, mem0_ref, mem_ref, sems, *, S, D, H, DH, M, SEG, FF):
    L = M + SEG
    R = 2 * L
    NP = H // 2
    ND = D // 128
    NF = FF // 128
    NQ = ND // 2
    KH = D // 4
    FS = (NF - CPRE) // 2
    FH = FS * 32
    N1 = (S - RB0) // RB1
    N2 = S // RB2
    assert CPRE == ND and FS % 2 == 0
    Q_W2, Q_W3A, Q_W4A = 0, NQ, 2 * NQ
    assert 2 * N1 == 3 * NQ and N2 == NQ == 4 and FS // 2 - 1 == NQ

    SEM_WO, SEM_OUT, SEM_MEM, SEM_P = range(4)
    SEM_W1 = 4
    SEM_X = SEM_W1 + ND
    SEM_Q = SEM_X + 4 + N1
    SEM_G = SEM_Q + N1
    JG = NP // N2

    def tile_copy(src, row0, nrows, col, dst, sem):
        cols = pl.ds(pl.multiple_of(col * 128, 128), 128)
        return pltpu.make_async_copy(src.bitcast(U32).at[pl.ds(row0, nrows), cols], dst, sem)

    def quad_copies(src, row0, kh, col, dst_ref, q, sem, dist=1):
        return [tile_copy(src, row0, 2 * kh, col + t * dist, dst_ref.at[q, pl.ds(2 * kh * t, 2 * kh)], sem)
                for t in range(2)]

    def q_copies(q, sem):
        if q < Q_W3A:
            return quad_copies(w2_hbm, 0, KH, 2 * q, q_ref, q, sem)
        if q < Q_W4A:
            return quad_copies(w3_hbm, 0, KH, q - Q_W3A, q_ref, q, sem, CPRE // 2)
        return quad_copies(w4_hbm, 0, KH, 2 * (q - Q_W4A), q_ref, q, sem)

    def x_copy(lo, n, sem):
        return pltpu.make_async_copy(x_hbm.at[pl.ds(lo, n)], x_ref.at[pl.ds(lo, n)], sem)

    def group(i):
        sem = sems.at[SEM_G + i]
        cps = [pltpu.make_async_copy(w.bitcast(U32).at[:, i * JG + k, :], stage.at[m * NP + i * JG + k], sem)
               for m, w in enumerate((wq_hbm, wk_hbm, wv_hbm)) for k in range(JG)]
        for t in range(2):
            rq = 2 * i + t
            par, pair = rq >> 2, rq & 3
            cps += quad_copies(w3_hbm, 0, KH, CPRE + par * FS + 1 + pair, p_ref, rq, sem, FS // 2)
            row0 = pl.multiple_of(CPRE * 64 + par * 2 * FH, 64)
            cps += quad_copies(w4_hbm, row0, FH, 2 * pair, r_ref, rq, sem)
        return cps

    g_mem = [pltpu.make_async_copy(mem0_hbm, mem0_ref, sems.at[SEM_MEM])]
    X0 = S - N1 * XK
    assert all(X0 + (k + 1) * XK >= min(RB0 + (k + 1) * RB1 + HB, S) for k in range(N1))
    xch = [(0, RA), (RA, RA + HB), (RA + HB, RB0 + HB), (RB0 + HB, X0)]
    xch += [(X0 + k * XK, X0 + (k + 1) * XK) for k in range(N1)]
    g_x = [x_copy(lo, hi - lo, sems.at[SEM_X + i]) for i, (lo, hi) in enumerate(xch)]
    g_w1 = [tile_copy(w1_hbm, 0, 2 * KH, j, w1_ref.at[j], sems.at[SEM_W1 + j]) for j in range(ND)]
    g_q = [q_copies(2 * k, sems.at[SEM_Q + k]) + q_copies(2 * k + 1, sems.at[SEM_Q + k]) for k in range(N1)]
    g_p = [cp for par in range(2)
           for cp in quad_copies(w3_hbm, 0, KH, CPRE + par * FS, p_ref, 2 * NQ + par, sems.at[SEM_P], FS // 2)]
    g_wo = [tile_copy(wo_hbm, 0, H * DH // 2, j, wo_ref.at[j], sems.at[SEM_WO]) for j in range(ND)]

    def start(*gs):
        for g in gs:
            for cp in g:
                cp.start()

    def wait(*gs):
        for g in gs:
            for cp in g:
                cp.wait()

    start(g_x[0:1], g_w1[0:6], g_x[1:2], g_w1[6:], g_x[2:4])
    for k in range(N1):
        start(g_x[4 + k:5 + k], g_q[k])
    start(g_mem, g_p)

    def prep_items(ref, q, kh, r0=0, n=None):
        def item(r, z):
            b = [ref[q, pl.ds(t * kh + r0 + r, 8), :] for t in range(4)]
            for t, y in zip((1, 2, 4, 5, 6), _right_sums(b[0] | z, b[1], b[2], b[3] | z)):
                ref[q, pl.ds(t * kh + r0 + r, 8), :] = y
        return [functools.partial(item, r) for r in range(0, kh if n is None else n, 8)]

    def quad_wt(ref, q, kh):
        return lambda i: ref[q, i * kh:(i + 1) * kh, :]

    def load_left(ref):
        return [_bf(ref[t]) for t in range(7)]

    def store_left(ref, al):
        for t in range(7):
            ref[t] = pltpu.bitcast(al[t], U32)

    h_ref[:, 0:8, :] = jnp.zeros((ND, 8, 128), F32)
    h_ref[:, S + 8:S + 16, :] = jnp.zeros((ND, 8, 128), F32)
    s_ref[...] = jnp.zeros(s_ref.shape, F32)

    def ln2(r):
        xn = _ln(x_ref[pl.ds(r, HB), :].astype(F32))
        b_ref[pl.ds(r, HB), :] = xn
        return _ln(xn).astype(BF16)

    def store_pre(a):
        a32 = pltpu.bitcast(a, U32)
        pre_ref[0] = a32[:, :D // 2]
        pre_ref[1] = a32[:, D // 2:]

    def p1_rows(base, n, a, pace):
        for s in range(n):
            r = base + s * HB
            nxt = r + HB if s + 1 < n else pl.multiple_of(jnp.minimum(r + HB, S - HB), HB)
            a_n = ln2(nxt)
            for j in range(ND):
                h_ref[j, pl.ds(r + 8, HB), :] = pace(_dot(a, w1_ref[j]))
            a = a_n
        store_pre(a)

    NA = RA // HB
    wait(g_x[0:1])
    a0 = [ln2(s * HB) for s in range(NPRE)]
    for gi, (j0, j1) in enumerate(W1G):
        wait(g_w1[j0:j1])
        if gi == len(W1G) - 1:
            wait(g_x[1:2])
            a_n = ln2(RA)
        for s in range(NA):
            if s == len(a0):
                a0.append(ln2(s * HB))
            for j in range(j0, j1):
                h_ref[j, pl.ds(s * HB + 8, HB), :] = _dot(a0[s], w1_ref[j])
    wait(g_x[2:3])
    p1_rows(RA, (RB0 - RA) // HB, a_n, lambda y: y)
    wait(g_x[3:4])

    def p1(k, c):
        base = pl.multiple_of(RB0 + k * RB1, RB1)
        x_copy(pl.multiple_of(X0 + k * XK, HB), XK, sems.at[SEM_X + 4 + k]).wait()
        landed = q_ref.at[pl.ds(2 * k, 2), pl.ds(0, 4 * KH)]
        pltpu.make_async_copy(landed, landed, sems.at[SEM_Q + k]).wait()

        @pl.when((k == 2) | (k == N1 - 1))
        def _():
            start(group(k >> 2))

        pace = _Pace()
        pace.spread(prep_items(q_ref, 2 * k, KH) + prep_items(q_ref, 2 * k + 1, KH), RB1 // HB * ND - 2)
        p1_rows(base, RB1 // HB, _bf(jnp.concatenate([pre_ref[0], pre_ref[1]], axis=1)), pace)
        assert not pace.items
        return c
    lax.fori_loop(0, N1, p1, 0)

    def shifted_left(r0):
        offs = (7, 9, 6, 10)
        return _left(lambda r, t: _gelu(h_ref[t, pl.ds(r0 + r + offs[4 * t // ND], CH), :]), NQ)

    store_left(pre_ref, shifted_left(0)[0])
    wait(g_mem, g_p)
    mem_ref[...] = mem0_ref[...].astype(F32)

    def p2(it, c):
        base = pl.multiple_of(it * RB2, RB2)
        nb = RB2 // BLK
        g = [None] * nb
        u = [None] * nb
        g[0] = load_left(pre_ref)

        masks = {}

        def repack(k, i, z):
            slab = (k // JG) * NP + it * JG + k % JG
            a = stage[slab, pl.ds(i * 16, 8, stride=2), :]
            b = stage[slab, pl.ds(i * 16 + 1, 8, stride=2), :]
            if id(z) not in masks:
                masks[id(z)] = (z, z + U32(0xFFFF), z + U32(0xFFFF0000))
            _, mlo, mhi = masks[id(z)]
            wqkv_ref[2 * slab, i * 8:(i + 1) * 8, :] = (a & mlo) | (b << 16)
            wqkv_ref[2 * slab + 1, i * 8:(i + 1) * 8, :] = (a >> 16) | (b & mhi)

        rp = [functools.partial(repack, k, i) for k in range(3 * JG) for i in range(D // 16)]
        pp = [it_ for t in range(2) for it_ in
              prep_items(p_ref, 2 * it + t, KH) + prep_items(r_ref, 2 * it + t, FH)
              + prep_items(p_ref, 2 * NQ + t, KH, pl.multiple_of(it * (KH // N2), 8), KH // N2)]
        items = []
        while rp or pp:
            items += rp[:5] + pp[:1]
            rp, pp = rp[5:], pp[1:]
        pace = _Pace()
        SL = NQ * 7

        zeros = {}
        carry = {}
        nitems = len(items)

        def make_g(s):
            if s < nb:
                g[s], zeros["g", s] = shifted_left(base + s * BLK)
            else:
                al_n, zeros["g", s] = shifted_left(pl.multiple_of(jnp.minimum(base + RB2, S - BLK), BLK))
                store_left(pre_ref, al_n)

        def mix(s):
            ys = []
            for q in range(NQ):
                ys += _run(_strassen(g[s], quad_wt(q_ref, Q_W2 + q, KH), pace))
            if s == nb - 1:
                wait(group(it))

                @pl.when(it < N2 - 2)
                def _():
                    start(group(it + 2))

                @pl.when(it == N2 - 2)
                def _():
                    start(g_wo)
                pace.spread(items, 1)
            rows = pl.ds(base + s * BLK, BLK)
            x1 = jnp.concatenate(ys, axis=1) + b_ref[rows, :]
            b_ref[rows, :] = x1
            y = [_ln(x1[r:r + CH]) for r in range(0, BLK, CH)]
            al, zeros["a", s] = _left(lambda r, t: y[r // CH][:, t * 128:(t + 1) * 128], NQ)
            store_left(a3_ref.at[it * nb + s], al)

        def up(s):
            al = load_left(a3_ref.at[it * nb + s])
            parts = []
            for q in range(NQ):
                p, carry[0] = _gelu_left(*_run(_strassen(al, quad_wt(q_ref, Q_W3A + q, KH), pace)))
                parts.append(p)
                if q + 1 < NQ:
                    pace.require(carry.pop(0), 7)
            u[s] = _cat(parts, 1)

        def down(s):
            for q in range(NQ):
                ys = _run(_strassen(u[s], quad_wt(q_ref, Q_W4A + q, KH), pace))
                for t in range(2):
                    cols = slice((2 * q + t) * 128, (2 * q + t + 1) * 128)
                    rows = pl.ds(base + s * BLK, BLK)
                    b_ref[rows, cols] = ys[t] + b_ref[rows, cols]

        assert nb == 4
        for s in range(1, nb):
            make_g(s)
        zg = zeros["g", 1] + zeros["g", 2] + zeros["g", 3]
        zeros["g01"], zeros["g12"], zeros["g23"] = zg[:24], zg[24:36], zg[36:]
        plan = [(mix, 0, ["g01"], 0), (mix, 1, [("a", 0), "g12"], 0), (mix, 2, [("a", 1), "g23"], 0),
                (mix, 3, [("a", 2)], 0), (up, 0, [("a", 3)], 0.3), (up, 1, [], 1.0), (down, 0, [], 1.5),
                (up, 2, [], 1.0), (down, 1, [], 1.5), (up, 3, [], 1.0), (down, 2, [], 1.5),
                (down, 3, [("g", 4)], 1.1)]
        wsum = sum(p[3] for p in plan) - plan[-1][3] * 8 / SL
        for fn, s, keys, w in plan:
            for key in keys:
                if key not in zeros:
                    make_g(key[1])
            zs = carry.pop(0, []) + [z for key in keys for z in zeros[key]]
            if zs:
                pace.require(zs, SL - 4 if keys else 7)
            pace.per = nitems * w / wsum / SL
            fn(s)
        assert not pace.items
        return c
    lax.fori_loop(0, N2, p2, 0)
    wait(g_wo)

    row = lax.broadcasted_iota(jnp.int32, (R, R), 0)
    col = lax.broadcasted_iota(jnp.int32, (R, R), 1)
    same_head = (row >= L) == (col >= L)
    rr = jnp.where(row >= L, row - L, row)
    cc = jnp.where(col >= L, col - L, col)
    visible = same_head & ((rr < M) | (rr >= cc))
    scale = DH ** -0.5
    fill = jnp.where(same_head, -1e9 / scale, -jnp.inf).astype(F32)

    def softmax_qk(q2, k2):
        s = lax.dot_general(q2, k2, (((1,), (1,)), ((), ())), preferred_element_type=F32)
        s = jnp.where(visible, s, fill)
        m = jnp.max(s, axis=-1, keepdims=True)
        e = jnp.exp2((s - m) * (scale * LOG2E))
        l = jnp.sum(e, axis=-1, keepdims=True)
        r = pl.reciprocal(l, approx=True)
        r = r * (2.0 - l * r)
        return (e * r).astype(BF16)

    def combine(r, rdst, slot):
        b = b_ref[pl.ds(r, STEP), :]
        g = b * jax.nn.sigmoid(b)
        x = x_ref[pl.ds(r, STEP), :].astype(F32)
        x_ref[pl.ds(rdst, STEP), :] = (x + s_ref[slot] * g).astype(x_ref.dtype)

    def out_copy(r):
        return pltpu.make_async_copy(x_ref.at[pl.ds(r, STEP)], out_hbm.at[pl.ds(r, STEP)], sems.at[SEM_OUT])

    def step(j, c):
        r0 = pl.multiple_of(j * STEP, STEP)
        par = j & 1
        blk = j >> 1
        rb = pl.multiple_of(blk * BLK, BLK)
        rprev = pl.multiple_of(jnp.maximum(r0 - STEP, 0), STEP)
        rdst = pl.multiple_of(jnp.where(j >= 1, r0 - STEP, S), STEP)
        al3 = load_left(a3_ref.at[blk])
        xn = _ln(x_ref[pl.ds(r0, STEP), :].astype(F32))

        parts = []

        def up_products():
            for q in range(FS // 2):
                wt = quad_wt(p_ref, 2 * NQ + par if q == 0 else par * NQ + q - 1, KH)
                for y in _strassen(al3, wt):
                    if y is not None:
                        parts.append(_gelu_left(*y)[0])
                    yield
        ups = up_products()

        def mlp_up(n):
            for _ in range(n):
                next(ups)

        def mlp_down(qs):
            al4 = _cat(parts, 1)
            for q in qs:
                ys = _run(_strassen(al4, quad_wt(r_ref, par * NQ + q, FH)))
                for t in range(2):
                    cols = slice((2 * q + t) * 128, (2 * q + t + 1) * 128)
                    b_ref[pl.ds(rb, BLK), cols] = ys[t] + b_ref[pl.ds(rb, BLK), cols]

        def segment(lhs, build_qkv, build_o, fillers, inter=None):
            qkv = [None] * NP
            prob = [None] * NP
            o = [None] * H
            ph = NP - 3
            ks = ph * 128

            def do_qkv(p):
                y = [[_dot(lhs, wqkv_ref[m * H + 2 * p + hh]) for m in range(3)] for hh in range(2)]
                qkv[p] = [t.astype(BF16) for t in build_qkv(p, y)]

            def do_qk(p):
                prob[p] = softmax_qk(qkv[p][0], qkv[p][1])

            def do_pv(p):
                o2 = jnp.dot(prob[p], qkv[p][2], preferred_element_type=F32)
                o[2 * p], o[2 * p + 1] = build_o(p, o2)

            for p in range(NP):
                do_qkv(p)
                if inter is not None:
                    inter(p)
                if p >= 1:
                    do_qk(p - 1)
                if p >= 3:
                    do_pv(p - 3)
            fillers[0]()
            do_qk(NP - 1)
            do_pv(NP - 3)
            do_pv(NP - 2)
            olo = jnp.concatenate(o[:2 * ph], axis=1)
            acc = [_dot(olo, wo_ref[n, 0:ks, :]) for n in range(ND // 2)]
            do_pv(NP - 1)
            fillers[1]()
            acc += [_dot(olo, wo_ref[n, 0:ks, :]) for n in range(ND // 2, ND)]
            ohi = jnp.concatenate(o[2 * ph:], axis=1)
            res = jnp.concatenate([_dot(ohi, wo_ref[n, ks:, :]) + acc[n] for n in range(ND)], axis=1)
            fillers[2]()
            return res

        qkv_kept = [None] * NP
        o_kept = [None] * H

        def build_qkv_a(p, y):
            qkv_kept[p] = [[y[hh][m][40:48] for m in range(3)] for hh in range(2)]
            return [jnp.concatenate([y[0][m][0:40], y[1][m][0:40]], axis=0) for m in range(3)]

        def build_o_a(p, o2):
            o_kept[2 * p] = o2[32:40]
            o_kept[2 * p + 1] = o2[72:80]
            return o2[0:32].astype(BF16), o2[40:72].astype(BF16)

        def build_qkv_b(p, y):
            return [jnp.concatenate([y[0][m][0:8], qkv_kept[p][0][m], y[0][m][8:32],
                                     y[1][m][0:8], qkv_kept[p][1][m], y[1][m][8:32]], axis=0)
                    for m in range(3)]

        def build_o_b(p, o2):
            return (jnp.concatenate([o2[0:8], o_kept[2 * p], o2[8:40]], axis=0).astype(BF16),
                    jnp.concatenate([o2[40:48], o_kept[2 * p + 1], o2[48:80]], axis=0).astype(BF16))

        def last_down():
            mlp_down(range(2, NQ))
            combine(rprev, rdst, 1 - par)

        nint = 7 * (FS // 2 - 3)
        lhs_a = jnp.concatenate([mem_ref[...], xn[0:40]], axis=0).astype(BF16)
        mlp_up(7)
        sa = segment(lhs_a, build_qkv_a, build_o_a, [lambda: mlp_up(7), lambda: None, lambda: mlp_up(7)])
        mem_ref[...] = sa[0:8]
        s_ref[par, 0:24, :] = sa[8:32]
        lhs_b = jnp.concatenate([sa[0:8], xn[40:64]], axis=0).astype(BF16)
        sb = segment(lhs_b, build_qkv_b, build_o_b,
                     [lambda: mlp_down(range(0, 2)), last_down, lambda: None],
                     inter=lambda p: mlp_up(1) if 1 <= p <= nint else None)
        mem_ref[...] = sb[0:8]
        s_ref[par, 24:64, :] = sb[8:48]

        @pl.when(j >= 1)
        def _():
            out_copy(rprev).start()
        return c
    lax.fori_loop(0, S // STEP, step, 0)
    combine(S - STEP, S - STEP, 1)
    out_copy(S - STEP).start()
    pltpu.make_async_copy(x_ref.at[pl.ds(0, S)], out_hbm, sems.at[SEM_OUT]).wait()


@functools.partial(jax.jit, static_argnames=("A_seg_len",))
def pallas_recurrent_scan__memory_aug_recurrent_mem_tr__mixer_s_mlp__prompt_kernel(
        A_x, A_mem0, A_Wq, A_Wk, A_Wv, A_Wo, A_seg_len, B_x, B_w1, B_w2, B_w3, B_w4):
    del B_x
    B, S, D = A_x.shape
    _, H, DH = A_Wq.shape
    M = A_mem0.shape[1]
    FF = B_w3.shape[1]
    assert (B, S, D, H, DH, M, A_seg_len, FF) == (1, 2048, 1024, 32, 128, 8, 32, 3584)
    nd, nf = D // 128, FF // 128
    kern = functools.partial(_kernel, S=S, D=D, H=H, DH=DH, M=M, SEG=A_seg_len, FF=FF)
    any_spec = pl.BlockSpec(memory_space=pl.ANY)
    out = pl.pallas_call(
        kern,
        out_shape=jax.ShapeDtypeStruct((S, D), A_x.dtype),
        in_specs=[any_spec] * 10,
        out_specs=any_spec,
        scratch_shapes=[
            pltpu.VMEM((S + STEP, D), BF16),
            pltpu.VMEM((3 * H // 2, D, 128), U32),
            pltpu.VMEM((3 * H, D // 2, 128), U32),
            pltpu.VMEM((nd, H * DH // 2, 128), U32),
            pltpu.VMEM((nd, D // 2, 128), U32),
            pltpu.VMEM((3 * nd // 2, 7 * D // 4, 128), U32),
            pltpu.VMEM(((nf - CPRE) // 2, 7 * D // 4, 128), U32),
            pltpu.VMEM((nd, 7 * (nf - CPRE) * 16, 128), U32),
            pltpu.VMEM((nd, S + 16, 128), F32),
            pltpu.VMEM((S, D), F32),
            pltpu.VMEM((S // BLK, 7, HB // 2, D // 2), U32),
            pltpu.VMEM((7, HB // 2, D // 2), U32),
            pltpu.VMEM((2, STEP, D), F32),
            pltpu.VMEM((M, D), BF16),
            pltpu.VMEM((M, D), F32),
            pltpu.SemaphoreType.DMA((4 + nd + 4 + 2 * ((S - RB0) // RB1) + S // RB2,)),
        ],
        compiler_params=pltpu.CompilerParams(vmem_limit_bytes=120 * 1024 * 1024,
                                             disable_bounds_checks=True),
    )(A_x[0], A_mem0[0], A_Wq, A_Wk, A_Wv, A_Wo.reshape(H * DH, D), B_w1, B_w2, B_w3, B_w4)
    return out[None]
```

```python
import functools

import jax
import jax.numpy as jnp
from jax import lax
import jax.experimental.pallas as pl
import jax.experimental.pallas.tpu as pltpu

F32 = jnp.float32
BF16 = jnp.bfloat16
U32 = jnp.uint32
EPS = 1e-5
LOG2E = 1.4426950408889634

HB = 64
BLK = 2 * HB
RB0 = 512
RA = 256
RB1 = 256
RB2 = 512
CPRE = 8
STEP = 64
NPRE = 2
W1G = ((0, 2), (2, 5), (5, 8))
XK = 192
CH = 16


def _ln(x):
    m = jnp.mean(x, axis=-1, keepdims=True)
    xc = x - m
    v = jnp.mean(xc * xc, axis=-1, keepdims=True)
    return xc * lax.rsqrt(v + EPS)


def _gelu(x):
    c = 0.7978845608028654
    return 0.5 * x * (1.0 + jnp.tanh(c * (x + 0.044715 * (x * x * x))))


def _bf(w_u32):
    return pltpu.bitcast(w_u32, BF16)


def _pk(x):
    return pltpu.bitcast(x.astype(BF16), U32)


def _dot(a, w_u32):
    return jnp.dot(a, _bf(w_u32), preferred_element_type=F32)


def _zero_of(y):
    if y.dtype != U32:
        y = pltpu.bitcast(y[0:(8 if y.dtype == F32 else 16), 0:128], U32)
    return (y[0:8, 0:128] >> 31) >> 1


def _after(y, z):
    return jnp.concatenate([y[0:8] + pltpu.bitcast(z, F32), y[8:]], axis=0)


def _left(get, nk):
    rows, zs = [], []
    for r in range(0, HB, CH):
        cols = []
        for t in range(nk):
            a11, a12, a21, a22 = get(r, t), get(r, nk + t), get(HB + r, t), get(HB + r, nk + t)
            p = [y.astype(BF16) for y in (a11 + a22, a21 + a22, a11, a22, a11 + a12, a21 - a11, a12 - a22)]
            zs.append(_zero_of(functools.reduce(jnp.bitwise_or, [pltpu.bitcast(y, U32) for y in p])))
            cols.append(p)
        rows.append(_cat(cols, 1))
    return _cat(rows, 0), zs


def _cat(parts, axis):
    return [jnp.concatenate([p[t] for p in parts], axis=axis) for t in range(7)]


def _right_sums(b11, b21, b12, b22):
    b11, b21, b12, b22 = [_bf(t).astype(F32) for t in (b11, b21, b12, b22)]
    return [_pk(t) for t in (b21 - b11, b12 - b22, b11 + b22, b11 + b12, b21 + b22)]


class _Pace:
    def __init__(self):
        self.items, self.per, self.before = [], 0, []

    def spread(self, items, nslots):
        self.items, self.per, self.credit = list(items), len(items) / nslots, 0.0

    def require(self, zeros, nslots):
        self.before += [None] * (nslots - len(self.before))
        for i, z in enumerate(zeros):
            k = (i + 1) * nslots // len(zeros) - 1
            self.before[k] = z if self.before[k] is None else self.before[k] | z

    def __call__(self, y):
        if self.items:
            self.credit += self.per
            n = min(int(self.credit + 1e-6), len(self.items))
            self.credit -= n
            if n:
                z = _zero_of(y)
                for _ in range(n):
                    self.items.pop(0)(z)
        if self.before:
            z = self.before.pop(0)
            if z is not None:
                y = _after(y, z)
        return y


def _strassen(al, wt, pace=lambda y: y):
    m1 = pace(_dot(al[0], wt(4)))
    yield None
    m4 = pace(_dot(al[3], wt(1)))
    yield None
    m5 = pace(_dot(al[4], wt(3)))
    yield None
    m2 = pace(_dot(al[1], wt(0)))
    yield None
    m3 = pace(_dot(al[2], wt(2)))
    yield None
    c11 = pace(_dot(al[6], wt(6)) + (m1 + m4 - m5))
    yield None
    c22 = pace(_dot(al[5], wt(5)) + (m1 - m2 + m3))
    yield (jnp.concatenate([c11, m2 + m4], axis=0), jnp.concatenate([m3 + m5, c22], axis=0))


def _run(gen):
    for y in gen:
        pass
    return y


def _gelu_left(y0, y1):
    return _left(lambda r, t: _gelu((y0, y1)[t][r:r + CH]), 1)


def _kernel(x_hbm, mem0_hbm, wq_hbm, wk_hbm, wv_hbm, wo_hbm, w1_hbm, w2_hbm, w3_hbm, w4_hbm, out_hbm,
            x_ref, stage, wqkv_ref, wo_ref, w1_ref, q_ref, p_ref, r_ref,
            h_ref, b_ref, a3_ref, pre_ref, s_ref, mem0_ref, mem_ref, sems, *, S, D, H, DH, M, SEG, FF):
    L = M + SEG
    R = 2 * L
    NP = H // 2
    ND = D // 128
    NF = FF // 128
    NQ = ND // 2
    KH = D // 4
    FS = (NF - CPRE) // 2
    FH = FS * 32
    N1 = (S - RB0) // RB1
    N2 = S // RB2
    assert CPRE == ND and FS % 2 == 0
    Q_W2, Q_W3A, Q_W4A = 0, NQ, 2 * NQ
    assert 2 * N1 == 3 * NQ and N2 == NQ == 4 and FS // 2 - 1 == NQ

    SEM_WO, SEM_OUT, SEM_MEM, SEM_P = range(4)
    SEM_W1 = 4
    SEM_X = SEM_W1 + ND
    SEM_Q = SEM_X + 4 + N1
    SEM_G = SEM_Q + N1
    JG = NP // N2

    def tile_copy(src, row0, nrows, col, dst, sem):
        cols = pl.ds(pl.multiple_of(col * 128, 128), 128)
        return pltpu.make_async_copy(src.bitcast(U32).at[pl.ds(row0, nrows), cols], dst, sem)

    def quad_copies(src, row0, kh, col, dst_ref, q, sem, dist=1):
        return [tile_copy(src, row0, 2 * kh, col + t * dist, dst_ref.at[q, pl.ds(2 * kh * t, 2 * kh)], sem)
                for t in range(2)]

    def q_copies(q, sem):
        if q < Q_W3A:
            return quad_copies(w2_hbm, 0, KH, 2 * q, q_ref, q, sem)
        if q < Q_W4A:
            return quad_copies(w3_hbm, 0, KH, q - Q_W3A, q_ref, q, sem, CPRE // 2)
        return quad_copies(w4_hbm, 0, KH, 2 * (q - Q_W4A), q_ref, q, sem)

    def x_copy(lo, n, sem):
        return pltpu.make_async_copy(x_hbm.at[pl.ds(lo, n)], x_ref.at[pl.ds(lo, n)], sem)

    def group(i):
        sem = sems.at[SEM_G + i]
        cps = [pltpu.make_async_copy(w.bitcast(U32).at[:, i * JG + k, :], stage.at[m * NP + i * JG + k], sem)
               for m, w in enumerate((wq_hbm, wk_hbm, wv_hbm)) for k in range(JG)]
        for t in range(2):
            rq = 2 * i + t
            par, pair = rq >> 2, rq & 3
            cps += quad_copies(w3_hbm, 0, KH, CPRE + par * FS + 1 + pair, p_ref, rq, sem, FS // 2)
            row0 = pl.multiple_of(CPRE * 64 + par * 2 * FH, 64)
            cps += quad_copies(w4_hbm, row0, FH, 2 * pair, r_ref, rq, sem)
        return cps

    g_mem = [pltpu.make_async_copy(mem0_hbm, mem0_ref, sems.at[SEM_MEM])]
    X0 = S - N1 * XK
    assert all(X0 + (k + 1) * XK >= min(RB0 + (k + 1) * RB1 + HB, S) for k in range(N1))
    xch = [(0, RA), (RA, RA + HB), (RA + HB, RB0 + HB), (RB0 + HB, X0)]
    xch += [(X0 + k * XK, X0 + (k + 1) * XK) for k in range(N1)]
    g_x = [x_copy(lo, hi - lo, sems.at[SEM_X + i]) for i, (lo, hi) in enumerate(xch)]
    g_w1 = [tile_copy(w1_hbm, 0, 2 * KH, j, w1_ref.at[j], sems.at[SEM_W1 + j]) for j in range(ND)]
    g_q = [q_copies(2 * k, sems.at[SEM_Q + k]) + q_copies(2 * k + 1, sems.at[SEM_Q + k]) for k in range(N1)]
    g_p = [cp for par in range(2)
           for cp in quad_copies(w3_hbm, 0, KH, CPRE + par * FS, p_ref, 2 * NQ + par, sems.at[SEM_P], FS // 2)]
    g_wo = [tile_copy(wo_hbm, 0, H * DH // 2, j, wo_ref.at[j], sems.at[SEM_WO]) for j in range(ND)]

    def start(*gs):
        for g in gs:
            for cp in g:
                cp.start()

    def wait(*gs):
        for g in gs:
            for cp in g:
                cp.wait()

    start(g_x[0:1], g_w1[0:6], g_x[1:2], g_w1[6:], g_x[2:4])
    for k in range(N1):
        start(g_x[4 + k:5 + k], g_q[k])
    start(g_mem, g_p)

    def prep_items(ref, q, kh, r0=0, n=None):
        def item(r, z):
            b = [ref[q, pl.ds(t * kh + r0 + r, 8), :] for t in range(4)]
            for t, y in zip((1, 2, 4, 5, 6), _right_sums(b[0] | z, b[1], b[2], b[3] | z)):
                ref[q, pl.ds(t * kh + r0 + r, 8), :] = y
        return [functools.partial(item, r) for r in range(0, kh if n is None else n, 8)]

    def quad_wt(ref, q, kh):
        return lambda i: ref[q, i * kh:(i + 1) * kh, :]

    def load_left(ref):
        return [_bf(ref[t]) for t in range(7)]

    def store_left(ref, al):
        for t in range(7):
            ref[t] = pltpu.bitcast(al[t], U32)

    h_ref[:, 0:8, :] = jnp.zeros((ND, 8, 128), F32)
    h_ref[:, S + 8:S + 16, :] = jnp.zeros((ND, 8, 128), F32)
    s_ref[...] = jnp.zeros(s_ref.shape, F32)

    def ln2(r):
        xn = _ln(x_ref[pl.ds(r, HB), :].astype(F32))
        b_ref[pl.ds(r, HB), :] = xn
        return _ln(xn).astype(BF16)

    def store_pre(a):
        a32 = pltpu.bitcast(a, U32)
        pre_ref[0] = a32[:, :D // 2]
        pre_ref[1] = a32[:, D // 2:]

    def p1_rows(base, n, a, pace):
        for s in range(n):
            r = base + s * HB
            nxt = r + HB if s + 1 < n else pl.multiple_of(jnp.minimum(r + HB, S - HB), HB)
            a_n = ln2(nxt)
            for j in range(ND):
                h_ref[j, pl.ds(r + 8, HB), :] = pace(_dot(a, w1_ref[j]))
            a = a_n
        store_pre(a)

    NA = RA // HB
    wait(g_x[0:1])
    a0 = [ln2(s * HB) for s in range(NPRE)]
    for gi, (j0, j1) in enumerate(W1G):
        wait(g_w1[j0:j1])
        if gi == len(W1G) - 1:
            wait(g_x[1:2])
            a_n = ln2(RA)
        for s in range(NA):
            if s == len(a0):
                a0.append(ln2(s * HB))
            for j in range(j0, j1):
                h_ref[j, pl.ds(s * HB + 8, HB), :] = _dot(a0[s], w1_ref[j])
    wait(g_x[2:3])
    p1_rows(RA, (RB0 - RA) // HB, a_n, lambda y: y)
    wait(g_x[3:4])

    def p1(k, c):
        base = pl.multiple_of(RB0 + k * RB1, RB1)
        x_copy(pl.multiple_of(X0 + k * XK, HB), XK, sems.at[SEM_X + 4 + k]).wait()
        landed = q_ref.at[pl.ds(2 * k, 2), pl.ds(0, 4 * KH)]
        pltpu.make_async_copy(landed, landed, sems.at[SEM_Q + k]).wait()

        @pl.when((k == 2) | (k == N1 - 1))
        def _():
            start(group(k >> 2))

        pace = _Pace()
        pace.spread(prep_items(q_ref, 2 * k, KH) + prep_items(q_ref, 2 * k + 1, KH), RB1 // HB * ND)
        p1_rows(base, RB1 // HB, _bf(jnp.concatenate([pre_ref[0], pre_ref[1]], axis=1)), pace)
        assert not pace.items
        return c
    lax.fori_loop(0, N1, p1, 0)

    def shifted_left(r0):
        offs = (7, 9, 6, 10)
        return _left(lambda r, t: _gelu(h_ref[t, pl.ds(r0 + r + offs[4 * t // ND], CH), :]), NQ)

    store_left(pre_ref, shifted_left(0)[0])
    wait(g_mem, g_p)
    mem_ref[...] = mem0_ref[...].astype(F32)

    def p2(it, c):
        base = pl.multiple_of(it * RB2, RB2)
        nb = RB2 // BLK
        g = [None] * nb
        u = [None] * nb
        g[0] = load_left(pre_ref)

        masks = {}

        def repack(k, i, z):
            slab = (k // JG) * NP + it * JG + k % JG
            a = stage[slab, pl.ds(i * 16, 8, stride=2), :]
            b = stage[slab, pl.ds(i * 16 + 1, 8, stride=2), :]
            if id(z) not in masks:
                masks[id(z)] = (z, z + U32(0xFFFF), z + U32(0xFFFF0000))
            _, mlo, mhi = masks[id(z)]
            wqkv_ref[2 * slab, i * 8:(i + 1) * 8, :] = (a & mlo) | (b << 16)
            wqkv_ref[2 * slab + 1, i * 8:(i + 1) * 8, :] = (a >> 16) | (b & mhi)

        rp = [functools.partial(repack, k, i) for k in range(3 * JG) for i in range(D // 16)]
        pp = [it_ for t in range(2) for it_ in
              prep_items(p_ref, 2 * it + t, KH) + prep_items(r_ref, 2 * it + t, FH)
              + prep_items(p_ref, 2 * NQ + t, KH, pl.multiple_of(it * (KH // N2), 8), KH // N2)]
        items = []
        while rp or pp:
            items += rp[:5] + pp[:1]
            rp, pp = rp[5:], pp[1:]
        pace = _Pace()
        SL = NQ * 7

        zeros = {}
        carry = {}
        nitems = len(items)

        def make_g(s):
            if s < nb:
                g[s], zeros["g", s] = shifted_left(base + s * BLK)
            else:
                al_n, zeros["g", s] = shifted_left(pl.multiple_of(jnp.minimum(base + RB2, S - BLK), BLK))
                store_left(pre_ref, al_n)

        def mix(s):
            ys = []
            for q in range(NQ):
                ys += _run(_strassen(g[s], quad_wt(q_ref, Q_W2 + q, KH), pace))
            if s == nb - 1:
                wait(group(it))

                @pl.when(it < N2 - 2)
                def _():
                    start(group(it + 2))

                @pl.when(it == N2 - 2)
                def _():
                    start(g_wo)
                pace.spread(items, 1)
            rows = pl.ds(base + s * BLK, BLK)
            x1 = jnp.concatenate(ys, axis=1) + b_ref[rows, :]
            b_ref[rows, :] = x1
            y = [_ln(x1[r:r + CH]) for r in range(0, BLK, CH)]
            al, zeros["a", s] = _left(lambda r, t: y[r // CH][:, t * 128:(t + 1) * 128], NQ)
            store_left(a3_ref.at[it * nb + s], al)

        def up(s):
            al = load_left(a3_ref.at[it * nb + s])
            parts = []
            for q in range(NQ):
                p, carry[0] = _gelu_left(*_run(_strassen(al, quad_wt(q_ref, Q_W3A + q, KH), pace)))
                parts.append(p)
                if q + 1 < NQ:
                    pace.require(carry.pop(0), 7)
            u[s] = _cat(parts, 1)

        def down(s):
            for q in range(NQ):
                ys = _run(_strassen(u[s], quad_wt(q_ref, Q_W4A + q, KH), pace))
                for t in range(2):
                    cols = slice((2 * q + t) * 128, (2 * q + t + 1) * 128)
                    rows = pl.ds(base + s * BLK, BLK)
                    b_ref[rows, cols] = ys[t] + b_ref[rows, cols]

        assert nb == 4
        for s in range(1, nb):
            make_g(s)
        zg = zeros["g", 1] + zeros["g", 2] + zeros["g", 3]
        zeros["g01"], zeros["g12"], zeros["g23"] = zg[:24], zg[24:36], zg[36:]
        plan = [(mix, 0, ["g01"], 0), (mix, 1, [("a", 0), "g12"], 0), (mix, 2, [("a", 1), "g23"], 0),
                (mix, 3, [("a", 2)], 0), (up, 0, [("a", 3)], 0.3), (up, 1, [], 1.0), (down, 0, [], 1.5),
                (up, 2, [], 1.0), (down, 1, [], 1.5), (up, 3, [], 1.0), (down, 2, [], 1.5),
                (down, 3, [("g", 4)], 1.1)]
        wsum = sum(p[3] for p in plan) - plan[-1][3] * 8 / SL
        for fn, s, keys, w in plan:
            for key in keys:
                if key not in zeros:
                    make_g(key[1])
            zs = carry.pop(0, []) + [z for key in keys for z in zeros[key]]
            if zs:
                pace.require(zs, SL - 1 if keys else 7)
            pace.per = nitems * w / wsum / SL
            fn(s)
        assert not pace.items
        return c
    lax.fori_loop(0, N2, p2, 0)
    wait(g_wo)

    row = lax.broadcasted_iota(jnp.int32, (R, R), 0)
    col = lax.broadcasted_iota(jnp.int32, (R, R), 1)
    same_head = (row >= L) == (col >= L)
    rr = jnp.where(row >= L, row - L, row)
    cc = jnp.where(col >= L, col - L, col)
    visible = same_head & ((rr < M) | (rr >= cc))
    scale = DH ** -0.5
    fill = jnp.where(same_head, -1e9 / scale, -jnp.inf).astype(F32)

    def softmax_qk(q2, k2):
        s = lax.dot_general(q2, k2, (((1,), (1,)), ((), ())), preferred_element_type=F32)
        s = jnp.where(visible, s, fill)
        m = jnp.max(s, axis=-1, keepdims=True)
        e = jnp.exp2((s - m) * (scale * LOG2E))
        l = jnp.sum(e, axis=-1, keepdims=True)
        r = pl.reciprocal(l, approx=True)
        r = r * (2.0 - l * r)
        return (e * r).astype(BF16)

    def combine(r, rdst, slot):
        b = b_ref[pl.ds(r, STEP), :]
        g = b * jax.nn.sigmoid(b)
        x = x_ref[pl.ds(r, STEP), :].astype(F32)
        x_ref[pl.ds(rdst, STEP), :] = (x + s_ref[slot] * g).astype(x_ref.dtype)

    def out_copy(r):
        return pltpu.make_async_copy(x_ref.at[pl.ds(r, STEP)], out_hbm.at[pl.ds(r, STEP)], sems.at[SEM_OUT])

    def step(j, c):
        r0 = pl.multiple_of(j * STEP, STEP)
        par = j & 1
        blk = j >> 1
        rb = pl.multiple_of(blk * BLK, BLK)
        rprev = pl.multiple_of(jnp.maximum(r0 - STEP, 0), STEP)
        rdst = pl.multiple_of(jnp.where(j >= 1, r0 - STEP, S), STEP)
        al3 = load_left(a3_ref.at[blk])
        xn = _ln(x_ref[pl.ds(r0, STEP), :].astype(F32))

        parts = []

        def up_products():
            for q in range(FS // 2):
                wt = quad_wt(p_ref, 2 * NQ + par if q == 0 else par * NQ + q - 1, KH)
                for y in _strassen(al3, wt):
                    if y is not None:
                        parts.append(_gelu_left(*y)[0])
                    yield
        ups = up_products()

        def mlp_up(n):
            for _ in range(n):
                next(ups)

        def mlp_down(qs):
            al4 = _cat(parts, 1)
            for q in qs:
                ys = _run(_strassen(al4, quad_wt(r_ref, par * NQ + q, FH)))
                for t in range(2):
                    cols = slice((2 * q + t) * 128, (2 * q + t + 1) * 128)
                    b_ref[pl.ds(rb, BLK), cols] = ys[t] + b_ref[pl.ds(rb, BLK), cols]

        def segment(lhs, build_qkv, build_o, fillers, inter=None):
            qkv = [None] * NP
            prob = [None] * NP
            o = [None] * H
            ph = NP - 3
            ks = ph * 128

            def do_qkv(p):
                y = [[_dot(lhs, wqkv_ref[m * H + 2 * p + hh]) for m in range(3)] for hh in range(2)]
                qkv[p] = [t.astype(BF16) for t in build_qkv(p, y)]

            def do_qk(p):
                prob[p] = softmax_qk(qkv[p][0], qkv[p][1])

            def do_pv(p):
                o2 = jnp.dot(prob[p], qkv[p][2], preferred_element_type=F32)
                o[2 * p], o[2 * p + 1] = build_o(p, o2)

            for p in range(NP):
                do_qkv(p)
                if inter is not None:
                    inter(p)
                if p >= 1:
                    do_qk(p - 1)
                if p >= 3:
                    do_pv(p - 3)
            fillers[0]()
            do_qk(NP - 1)
            do_pv(NP - 3)
            do_pv(NP - 2)
            olo = jnp.concatenate(o[:2 * ph], axis=1)
            acc = [_dot(olo, wo_ref[n, 0:ks, :]) for n in range(ND // 2)]
            do_pv(NP - 1)
            fillers[1]()
            acc += [_dot(olo, wo_ref[n, 0:ks, :]) for n in range(ND // 2, ND)]
            ohi = jnp.concatenate(o[2 * ph:], axis=1)
            res = jnp.concatenate([_dot(ohi, wo_ref[n, ks:, :]) + acc[n] for n in range(ND)], axis=1)
            fillers[2]()
            return res

        qkv_kept = [None] * NP
        o_kept = [None] * H

        def build_qkv_a(p, y):
            qkv_kept[p] = [[y[hh][m][40:48] for m in range(3)] for hh in range(2)]
            return [jnp.concatenate([y[0][m][0:40], y[1][m][0:40]], axis=0) for m in range(3)]

        def build_o_a(p, o2):
            o_kept[2 * p] = o2[32:40]
            o_kept[2 * p + 1] = o2[72:80]
            return o2[0:32].astype(BF16), o2[40:72].astype(BF16)

        def build_qkv_b(p, y):
            return [jnp.concatenate([y[0][m][0:8], qkv_kept[p][0][m], y[0][m][8:32],
                                     y[1][m][0:8], qkv_kept[p][1][m], y[1][m][8:32]], axis=0)
                    for m in range(3)]

        def build_o_b(p, o2):
            return (jnp.concatenate([o2[0:8], o_kept[2 * p], o2[8:40]], axis=0).astype(BF16),
                    jnp.concatenate([o2[40:48], o_kept[2 * p + 1], o2[48:80]], axis=0).astype(BF16))

        def last_down():
            mlp_down(range(2, NQ))
            combine(rprev, rdst, 1 - par)

        nint = 7 * (FS // 2) - 22
        lhs_a = jnp.concatenate([mem_ref[...], xn[0:40]], axis=0).astype(BF16)
        mlp_up(8)
        sa = segment(lhs_a, build_qkv_a, build_o_a, [lambda: mlp_up(7), lambda: None, lambda: mlp_up(7)])
        mem_ref[...] = sa[0:8]
        s_ref[par, 0:24, :] = sa[8:32]
        lhs_b = jnp.concatenate([sa[0:8], xn[40:64]], axis=0).astype(BF16)
        sb = segment(lhs_b, build_qkv_b, build_o_b,
                     [lambda: mlp_down(range(0, 2)), last_down, lambda: None],
                     inter=lambda p: mlp_up(1) if 2 <= p < 2 + nint else None)
        mem_ref[...] = sb[0:8]
        s_ref[par, 24:64, :] = sb[8:48]

        @pl.when(j >= 1)
        def _():
            out_copy(rprev).start()
        return c
    lax.fori_loop(0, S // STEP, step, 0)
    combine(S - STEP, S - STEP, 1)
    out_copy(S - STEP).start()
    pltpu.make_async_copy(x_ref.at[pl.ds(0, S)], out_hbm, sems.at[SEM_OUT]).wait()


@functools.partial(jax.jit, static_argnames=("A_seg_len",))
def pallas_recurrent_scan__memory_aug_recurrent_mem_tr__mixer_s_mlp__prompt_kernel(
        A_x, A_mem0, A_Wq, A_Wk, A_Wv, A_Wo, A_seg_len, B_x, B_w1, B_w2, B_w3, B_w4):
    del B_x
    B, S, D = A_x.shape
    _, H, DH = A_Wq.shape
    M = A_mem0.shape[1]
    FF = B_w3.shape[1]
    assert (B, S, D, H, DH, M, A_seg_len, FF) == (1, 2048, 1024, 32, 128, 8, 32, 3584)
    nd, nf = D // 128, FF // 128
    kern = functools.partial(_kernel, S=S, D=D, H=H, DH=DH, M=M, SEG=A_seg_len, FF=FF)
    any_spec = pl.BlockSpec(memory_space=pl.ANY)
    out = pl.pallas_call(
        kern,
        out_shape=jax.ShapeDtypeStruct((S, D), A_x.dtype),
        in_specs=[any_spec] * 10,
        out_specs=any_spec,
        scratch_shapes=[
            pltpu.VMEM((S + STEP, D), BF16),
            pltpu.VMEM((3 * H // 2, D, 128), U32),
            pltpu.VMEM((3 * H, D // 2, 128), U32),
            pltpu.VMEM((nd, H * DH // 2, 128), U32),
            pltpu.VMEM((nd, D // 2, 128), U32),
            pltpu.VMEM((3 * nd // 2, 7 * D // 4, 128), U32),
            pltpu.VMEM(((nf - CPRE) // 2, 7 * D // 4, 128), U32),
            pltpu.VMEM((nd, 7 * (nf - CPRE) * 16, 128), U32),
            pltpu.VMEM((nd, S + 16, 128), F32),
            pltpu.VMEM((S, D), F32),
            pltpu.VMEM((S // BLK, 7, HB // 2, D // 2), U32),
            pltpu.VMEM((7, HB // 2, D // 2), U32),
            pltpu.VMEM((2, STEP, D), F32),
            pltpu.VMEM((M, D), BF16),
            pltpu.VMEM((M, D), F32),
            pltpu.SemaphoreType.DMA((4 + nd + 4 + 2 * ((S - RB0) // RB1) + S // RB2,)),
        ],
        compiler_params=pltpu.CompilerParams(vmem_limit_bytes=120 * 1024 * 1024,
                                             disable_bounds_checks=True),
    )(A_x[0], A_mem0[0], A_Wq, A_Wk, A_Wv, A_Wo.reshape(H * DH, D), B_w1, B_w2, B_w3, B_w4)
    return out[None]
```

```python
import functools

import jax
import jax.numpy as jnp
from jax import lax
import jax.experimental.pallas as pl
import jax.experimental.pallas.tpu as pltpu

F32 = jnp.float32
BF16 = jnp.bfloat16
U32 = jnp.uint32
EPS = 1e-5
LOG2E = 1.4426950408889634

HB = 64
BLK = 2 * HB
RB0 = 512
RA = 256
RB1 = 384
RB2 = 512
CPRE = 8
STEP = 64
NPRE = 2
W1G = ((0, 2), (2, 5), (5, 8))
XK = 320
CH = 16


def _ln(x):
    m = jnp.mean(x, axis=-1, keepdims=True)
    xc = x - m
    v = jnp.mean(xc * xc, axis=-1, keepdims=True)
    return xc * lax.rsqrt(v + EPS)


def _gelu(x):
    c = 0.7978845608028654
    h = 0.5 * x
    return h + h * jnp.tanh(x * (c + (c * 0.044715) * (x * x)))


def _bf(w_u32):
    return pltpu.bitcast(w_u32, BF16)


def _pk(x):
    return pltpu.bitcast(x.astype(BF16), U32)


def _dot(a, w_u32):
    return jnp.dot(a, _bf(w_u32), preferred_element_type=F32)


def _zero_of(y):
    if y.dtype != U32:
        y = pltpu.bitcast(y[0:(8 if y.dtype == F32 else 16), 0:128], U32)
    return (y[0:8, 0:128] >> 31) >> 1


def _after(y, z):
    return jnp.concatenate([y[0:8] + pltpu.bitcast(z, F32), y[8:]], axis=0)


def _left(get, nk):
    rows, zs = [], []
    for r in range(0, HB, CH):
        cols = []
        for t in range(nk):
            a11, a12, a21, a22 = get(r, t), get(r, nk + t), get(HB + r, t), get(HB + r, nk + t)
            p = [y.astype(BF16) for y in (a11 + a22, a21 + a22, a11, a22, a11 + a12, a21 - a11, a12 - a22)]
            zs.append(_zero_of(functools.reduce(jnp.bitwise_or, [pltpu.bitcast(y, U32) for y in p])))
            cols.append(p)
        rows.append(_cat(cols, 1))
    return _cat(rows, 0), zs


def _cat(parts, axis):
    return [jnp.concatenate([p[t] for p in parts], axis=axis) for t in range(7)]


def _right_sums(b11, b21, b12, b22):
    b11, b21, b12, b22 = [_bf(t).astype(F32) for t in (b11, b21, b12, b22)]
    return [_pk(t) for t in (b21 - b11, b12 - b22, b11 + b22, b11 + b12, b21 + b22)]


class _Pace:
    def __init__(self):
        self.items, self.per, self.before = [], 0, []

    def spread(self, items, nslots):
        self.items, self.per, self.credit = list(items), len(items) / nslots, 0.0

    def require(self, zeros, nslots):
        self.before += [None] * (nslots - len(self.before))
        for i, z in enumerate(zeros):
            k = (i + 1) * nslots // len(zeros) - 1
            self.before[k] = z if self.before[k] is None else self.before[k] | z

    def __call__(self, y):
        if self.items:
            self.credit += self.per
            n = min(int(self.credit + 1e-6), len(self.items))
            self.credit -= n
            if n:
                z = _zero_of(y)
                for _ in range(n):
                    self.items.pop(0)(z)
        if self.before:
            z = self.before.pop(0)
            if z is not None:
                y = _after(y, z)
        return y


def _strassen(al, wt, pace=lambda y: y):
    m1 = pace(_dot(al[0], wt(4)))
    yield None
    m4 = pace(_dot(al[3], wt(1)))
    yield None
    m5 = pace(_dot(al[4], wt(3)))
    yield None
    m2 = pace(_dot(al[1], wt(0)))
    yield None
    m3 = pace(_dot(al[2], wt(2)))
    yield None
    c11 = pace(_dot(al[6], wt(6)) + (m1 + m4 - m5))
    yield None
    c22 = pace(_dot(al[5], wt(5)) + (m1 - m2 + m3))
    yield (jnp.concatenate([c11, m2 + m4], axis=0), jnp.concatenate([m3 + m5, c22], axis=0))


def _run(gen):
    for y in gen:
        pass
    return y


def _gelu_left(y0, y1):
    return _left(lambda r, t: _gelu((y0, y1)[t][r:r + CH]), 1)


def _kernel(x_hbm, mem0_hbm, wq_hbm, wk_hbm, wv_hbm, wo_hbm, w1_hbm, w2_hbm, w3_hbm, w4_hbm, out_hbm,
            x_ref, stage, wqkv_ref, wo_ref, w1_ref, q_ref, p_ref, r_ref,
            h_ref, b_ref, a3_ref, pre1_ref, pre_ref, s_ref, mem0_ref, mem_ref, sems, *, S, D, H, DH, M, SEG, FF):
    L = M + SEG
    R = 2 * L
    NP = H // 2
    ND = D // 128
    NF = FF // 128
    NQ = ND // 2
    KH = D // 4
    FS = (NF - CPRE) // 2
    FH = FS * 32
    N1 = (S - RB0) // RB1
    N2 = S // RB2
    assert CPRE == ND and FS % 2 == 0
    Q_W2, Q_W3A, Q_W4A = 0, NQ, 2 * NQ
    QI = 3 * NQ // N1
    assert QI * N1 == 3 * NQ and N2 == NQ == 4 and FS // 2 - 1 == NQ

    SEM_WO, SEM_OUT, SEM_MEM, SEM_P = range(4)
    SEM_W1 = 4
    SEM_X = SEM_W1 + ND
    SEM_Q = SEM_X + 4 + N1
    SEM_G = SEM_Q + N1
    JG = NP // N2

    def tile_copy(src, row0, nrows, col, dst, sem):
        cols = pl.ds(pl.multiple_of(col * 128, 128), 128)
        return pltpu.make_async_copy(src.bitcast(U32).at[pl.ds(row0, nrows), cols], dst, sem)

    def quad_copies(src, row0, kh, col, dst_ref, q, sem, dist=1):
        return [tile_copy(src, row0, 2 * kh, col + t * dist, dst_ref.at[q, pl.ds(2 * kh * t, 2 * kh)], sem)
                for t in range(2)]

    def q_copies(q, sem):
        if q < Q_W3A:
            return quad_copies(w2_hbm, 0, KH, 2 * q, q_ref, q, sem)
        if q < Q_W4A:
            return quad_copies(w3_hbm, 0, KH, q - Q_W3A, q_ref, q, sem, CPRE // 2)
        return quad_copies(w4_hbm, 0, KH, 2 * (q - Q_W4A), q_ref, q, sem)

    def x_copy(lo, n, sem):
        return pltpu.make_async_copy(x_hbm.at[pl.ds(lo, n)], x_ref.at[pl.ds(lo, n)], sem)

    def group(i):
        sem = sems.at[SEM_G + i]
        cps = [pltpu.make_async_copy(w.bitcast(U32).at[:, i * JG + k, :], stage.at[m * NP + i * JG + k], sem)
               for m, w in enumerate((wq_hbm, wk_hbm, wv_hbm)) for k in range(JG)]
        for t in range(2):
            rq = 2 * i + t
            par, pair = rq >> 2, rq & 3
            cps += quad_copies(w3_hbm, 0, KH, CPRE + par * FS + 1 + pair, p_ref, rq, sem, FS // 2)
            row0 = pl.multiple_of(CPRE * 64 + par * 2 * FH, 64)
            cps += quad_copies(w4_hbm, row0, FH, 2 * pair, r_ref, rq, sem)
        return cps

    g_mem = [pltpu.make_async_copy(mem0_hbm, mem0_ref, sems.at[SEM_MEM])]
    X0 = S - N1 * XK
    assert all(X0 + (k + 1) * XK >= min(RB0 + (k + 1) * RB1 + HB, S) for k in range(N1))
    xch = [(0, RA), (RA, RA + HB), (RA + HB, RB0 + HB), (RB0 + HB, X0)]
    xch += [(X0 + k * XK, X0 + (k + 1) * XK) for k in range(N1)]
    g_x = [x_copy(lo, hi - lo, sems.at[SEM_X + i]) for i, (lo, hi) in enumerate(xch)]
    g_w1 = [tile_copy(w1_hbm, 0, 2 * KH, j, w1_ref.at[j], sems.at[SEM_W1 + j]) for j in range(ND)]
    g_q = [[cp for t in range(QI) for cp in q_copies(QI * k + t, sems.at[SEM_Q + k])] for k in range(N1)]
    g_p = [cp for par in range(2)
           for cp in quad_copies(w3_hbm, 0, KH, CPRE + par * FS, p_ref, 2 * NQ + par, sems.at[SEM_P], FS // 2)]
    g_wo = [tile_copy(wo_hbm, 0, H * DH // 2, j, wo_ref.at[j], sems.at[SEM_WO]) for j in range(ND)]

    def start(*gs):
        for g in gs:
            for cp in g:
                cp.start()

    def wait(*gs):
        for g in gs:
            for cp in g:
                cp.wait()

    start(g_x[0:1], g_w1[0:6], g_x[1:2], g_w1[6:], g_x[2:4])
    for k in range(N1):
        start(g_x[4 + k:5 + k], g_q[k])
    start(g_mem, g_p)

    def prep_items(ref, q, kh, r0=0, n=None):
        def item(r, z):
            b = [ref[q, pl.ds(t * kh + r0 + r, 8), :] for t in range(4)]
            for t, y in zip((1, 2, 4, 5, 6), _right_sums(b[0] | z, b[1], b[2], b[3] | z)):
                ref[q, pl.ds(t * kh + r0 + r, 8), :] = y
        return [functools.partial(item, r) for r in range(0, kh if n is None else n, 8)]

    def quad_wt(ref, q, kh):
        return lambda i: ref[q, i * kh:(i + 1) * kh, :]

    def load_left(ref):
        return [_bf(ref[t]) for t in range(7)]

    def store_left(ref, al):
        for t in range(7):
            ref[t] = pltpu.bitcast(al[t], U32)

    h_ref[:, 0:8, :] = jnp.zeros((ND, 8, 128), F32)
    h_ref[:, S + 8:S + 16, :] = jnp.zeros((ND, 8, 128), F32)
    s_ref[...] = jnp.zeros(s_ref.shape, F32)

    def ln2(r):
        xn = _ln(x_ref[pl.ds(r, HB), :].astype(F32))
        b_ref[pl.ds(r, HB), :] = xn
        return _ln(xn).astype(BF16)

    def shifted_left(r0):
        offs = (7, 9, 6, 10)
        return _left(lambda r, t: _gelu(h_ref[t, pl.ds(r0 + r + offs[4 * t // ND], CH), :]), NQ)

    def p1_rows(base, n, a, pace):
        for s in range(n):
            r = base + s * HB
            nxt = r + HB if s + 1 < n else pl.multiple_of(jnp.minimum(r + HB, S - HB), HB)
            a_n = ln2(nxt)
            for j in range(ND):
                h_ref[j, pl.ds(r + 8, HB), :] = pace(_dot(a, w1_ref[j]))
            a = a_n
        pre1_ref[...] = pltpu.bitcast(a, U32)

    NA = RA // HB
    wait(g_x[0:1])
    a0 = [ln2(s * HB) for s in range(NPRE)]
    for gi, (j0, j1) in enumerate(W1G):
        wait(g_w1[j0:j1])
        if gi == len(W1G) - 1:
            wait(g_x[1:2])
            a_n = ln2(RA)
        for s in range(NA):
            if s == len(a0):
                a0.append(ln2(s * HB))
            for j in range(j0, j1):
                h_ref[j, pl.ds(s * HB + 8, HB), :] = _dot(a0[s], w1_ref[j])
    wait(g_x[2:3])
    al0, zs = shifted_left(0)
    store_left(pre_ref, al0)
    pace = _Pace()
    pace.require(zs, (RB0 - RA) // HB * ND - 2)
    p1_rows(RA, (RB0 - RA) // HB, a_n, pace)
    wait(g_x[3:4])

    def p1(k, c):
        base = pl.multiple_of(RB0 + k * RB1, BLK)
        x_copy(pl.multiple_of(X0 + k * XK, HB), XK, sems.at[SEM_X + 4 + k]).wait()
        landed = q_ref.at[pl.ds(QI * k, QI), pl.ds(0, 4 * KH)]
        pltpu.make_async_copy(landed, landed, sems.at[SEM_Q + k]).wait()

        @pl.when((k & 1) == 1)
        def _():
            start(group(k >> 1))

        pace = _Pace()
        pace.spread([t_ for t in range(QI) for t_ in prep_items(q_ref, QI * k + t, KH)], RB1 // HB * ND)
        p1_rows(base, RB1 // HB, _bf(pre1_ref[...]), pace)
        assert not pace.items
        return c
    lax.fori_loop(0, N1, p1, 0)

    wait(g_mem, g_p)
    mem_ref[...] = mem0_ref[...].astype(F32)

    def p2(it, c):
        base = pl.multiple_of(it * RB2, RB2)
        nb = RB2 // BLK
        g = [None] * nb
        u = [None] * nb
        g[0] = load_left(pre_ref)

        masks = {}

        def repack(k, i, z):
            slab = (k // JG) * NP + it * JG + k % JG
            a = stage[slab, pl.ds(i * 16, 8, stride=2), :]
            b = stage[slab, pl.ds(i * 16 + 1, 8, stride=2), :]
            if id(z) not in masks:
                masks[id(z)] = (z, z + U32(0xFFFF), z + U32(0xFFFF0000))
            _, mlo, mhi = masks[id(z)]
            wqkv_ref[2 * slab, i * 8:(i + 1) * 8, :] = (a & mlo) | (b << 16)
            wqkv_ref[2 * slab + 1, i * 8:(i + 1) * 8, :] = (a >> 16) | (b & mhi)

        rp = [functools.partial(repack, k, i) for k in range(3 * JG) for i in range(D // 16)]
        pp = [it_ for t in range(2) for it_ in
              prep_items(p_ref, 2 * it + t, KH) + prep_items(r_ref, 2 * it + t, FH)
              + prep_items(p_ref, 2 * NQ + t, KH, pl.multiple_of(it * (KH // N2), 8), KH // N2)]
        items = []
        while rp or pp:
            items += rp[:5] + pp[:1]
            rp, pp = rp[5:], pp[1:]
        pace = _Pace()
        SL = NQ * 7

        zeros = {}
        carry = {}
        nitems = len(items)

        def make_g(s):
            if s < nb:
                g[s], zeros["g", s] = shifted_left(base + s * BLK)
            else:
                al_n, zeros["g", s] = shifted_left(pl.multiple_of(jnp.minimum(base + RB2, S - BLK), BLK))
                store_left(pre_ref, al_n)

        def mix(s):
            ys = []
            for q in range(NQ):
                ys += _run(_strassen(g[s], quad_wt(q_ref, Q_W2 + q, KH), pace))
            if s == nb - 1:
                wait(group(it))

                @pl.when(it < N2 - 2)
                def _():
                    start(group(it + 2))

                @pl.when(it == N2 - 2)
                def _():
                    start(g_wo)
                pace.spread(items, 1)
            rows = pl.ds(base + s * BLK, BLK)
            x1 = jnp.concatenate(ys, axis=1) + b_ref[rows, :]
            b_ref[rows, :] = x1
            y = [_ln(x1[r:r + CH]) for r in range(0, BLK, CH)]
            al, zeros["a", s] = _left(lambda r, t: y[r // CH][:, t * 128:(t + 1) * 128], NQ)
            store_left(a3_ref.at[it * nb + s], al)

        def up(s):
            al = load_left(a3_ref.at[it * nb + s])
            parts = []
            for q in range(NQ):
                p, carry[0] = _gelu_left(*_run(_strassen(al, quad_wt(q_ref, Q_W3A + q, KH), pace)))
                parts.append(p)
                if q + 1 < NQ:
                    pace.require(carry.pop(0), 7)
            u[s] = _cat(parts, 1)

        def down(s):
            for q in range(NQ):
                ys = _run(_strassen(u[s], quad_wt(q_ref, Q_W4A + q, KH), pace))
                for t in range(2):
                    cols = slice((2 * q + t) * 128, (2 * q + t + 1) * 128)
                    rows = pl.ds(base + s * BLK, BLK)
                    b_ref[rows, cols] = ys[t] + b_ref[rows, cols]

        assert nb == 4
        for s in range(1, nb):
            make_g(s)
        zg = zeros["g", 1] + zeros["g", 2] + zeros["g", 3]
        zeros["g01"], zeros["g12"], zeros["g23"] = zg[:24], zg[24:36], zg[36:]
        plan = [(mix, 0, ["g01"], 0), (mix, 1, [("a", 0), "g12"], 0), (mix, 2, [("a", 1), "g23"], 0),
                (mix, 3, [("a", 2)], 0), (up, 0, [("a", 3)], 0.3), (up, 1, [], 1.0), (down, 0, [], 1.5),
                (up, 2, [], 1.0), (down, 1, [], 1.5), (up, 3, [], 1.0), (down, 2, [], 1.5),
                (down, 3, [("g", 4)], 1.1)]
        wsum = sum(p[3] for p in plan) - plan[-1][3] * 8 / SL
        for fn, s, keys, w in plan:
            for key in keys:
                if key not in zeros:
                    make_g(key[1])
            zs = carry.pop(0, []) + [z for key in keys for z in zeros[key]]
            if zs:
                pace.require(zs, SL - 1 if keys else 7)
            pace.per = nitems * w / wsum / SL
            fn(s)
        assert not pace.items
        return c
    lax.fori_loop(0, N2, p2, 0)
    wait(g_wo)

    row = lax.broadcasted_iota(jnp.int32, (R, R), 0)
    col = lax.broadcasted_iota(jnp.int32, (R, R), 1)
    same_head = (row >= L) == (col >= L)
    rr = jnp.where(row >= L, row - L, row)
    cc = jnp.where(col >= L, col - L, col)
    visible = same_head & ((rr < M) | (rr >= cc))
    scale = DH ** -0.5
    fill = jnp.where(same_head, -1e9 / scale, -jnp.inf).astype(F32)

    def softmax_qk(q2, k2):
        s = lax.dot_general(q2, k2, (((1,), (1,)), ((), ())), preferred_element_type=F32)
        s = jnp.where(visible, s, fill)
        m = jnp.max(s, axis=-1, keepdims=True)
        e = jnp.exp2((s - m) * (scale * LOG2E))
        l = jnp.sum(e, axis=-1, keepdims=True)
        r = pl.reciprocal(l, approx=True)
        r = r * (2.0 - l * r)
        return (e * r).astype(BF16)

    def combine(r, rdst, slot):
        b = b_ref[pl.ds(r, STEP), :]
        g = b * jax.nn.sigmoid(b)
        x = x_ref[pl.ds(r, STEP), :].astype(F32)
        x_ref[pl.ds(rdst, STEP), :] = (x + s_ref[slot] * g).astype(x_ref.dtype)

    def out_copy(r):
        return pltpu.make_async_copy(x_ref.at[pl.ds(r, STEP)], out_hbm.at[pl.ds(r, STEP)], sems.at[SEM_OUT])

    def step(j, c):
        r0 = pl.multiple_of(j * STEP, STEP)
        par = j & 1
        blk = j >> 1
        rb = pl.multiple_of(blk * BLK, BLK)
        rprev = pl.multiple_of(jnp.maximum(r0 - STEP, 0), STEP)
        rdst = pl.multiple_of(jnp.where(j >= 1, r0 - STEP, S), STEP)
        al3 = load_left(a3_ref.at[blk])
        xn = _ln(x_ref[pl.ds(r0, STEP), :].astype(F32))

        parts = []

        def up_products():
            for q in range(FS // 2):
                wt = quad_wt(p_ref, 2 * NQ + par if q == 0 else par * NQ + q - 1, KH)
                for y in _strassen(al3, wt):
                    if y is not None:
                        parts.append(_gelu_left(*y)[0])
                    yield
        ups = up_products()

        def mlp_up(n):
            for _ in range(n):
                next(ups)

        def mlp_down(qs):
            al4 = _cat(parts, 1)
            for q in qs:
                ys = _run(_strassen(al4, quad_wt(r_ref, par * NQ + q, FH)))
                for t in range(2):
                    cols = slice((2 * q + t) * 128, (2 * q + t + 1) * 128)
                    b_ref[pl.ds(rb, BLK), cols] = ys[t] + b_ref[pl.ds(rb, BLK), cols]

        def segment(lhs, build_qkv, build_o, fillers, inter=None):
            qkv = [None] * NP
            prob = [None] * NP
            o = [None] * H
            ph = NP - 3
            ks = ph * 128

            def do_qkv(p):
                y = [[_dot(lhs, wqkv_ref[m * H + 2 * p + hh]) for m in range(3)] for hh in range(2)]
                qkv[p] = [t.astype(BF16) for t in build_qkv(p, y)]

            def do_qk(p):
                prob[p] = softmax_qk(qkv[p][0], qkv[p][1])

            def do_pv(p):
                o2 = jnp.dot(prob[p], qkv[p][2], preferred_element_type=F32)
                o[2 * p], o[2 * p + 1] = build_o(p, o2)

            for p in range(NP):
                do_qkv(p)
                if inter is not None:
                    inter(p)
                if p >= 1:
                    do_qk(p - 1)
                if p >= 3:
                    do_pv(p - 3)
            fillers[0]()
            do_qk(NP - 1)
            do_pv(NP - 3)
            do_pv(NP - 2)
            olo = jnp.concatenate(o[:2 * ph], axis=1)
            acc = [_dot(olo, wo_ref[n, 0:ks, :]) for n in range(ND // 2)]
            do_pv(NP - 1)
            fillers[1]()
            acc += [_dot(olo, wo_ref[n, 0:ks, :]) for n in range(ND // 2, ND)]
            ohi = jnp.concatenate(o[2 * ph:], axis=1)
            res = jnp.concatenate([_dot(ohi, wo_ref[n, ks:, :]) + acc[n] for n in range(ND)], axis=1)
            fillers[2]()
            return res

        qkv_kept = [None] * NP
        o_kept = [None] * H

        def build_qkv_a(p, y):
            qkv_kept[p] = [[y[hh][m][40:48] for m in range(3)] for hh in range(2)]
            return [jnp.concatenate([y[0][m][0:40], y[1][m][0:40]], axis=0) for m in range(3)]

        def build_o_a(p, o2):
            o_kept[2 * p] = o2[32:40]
            o_kept[2 * p + 1] = o2[72:80]
            return o2[0:32].astype(BF16), o2[40:72].astype(BF16)

        def build_qkv_b(p, y):
            return [jnp.concatenate([y[0][m][0:8], qkv_kept[p][0][m], y[0][m][8:32],
                                     y[1][m][0:8], qkv_kept[p][1][m], y[1][m][8:32]], axis=0)
                    for m in range(3)]

        def build_o_b(p, o2):
            return (jnp.concatenate([o2[0:8], o_kept[2 * p], o2[8:40]], axis=0).astype(BF16),
                    jnp.concatenate([o2[40:48], o_kept[2 * p + 1], o2[48:80]], axis=0).astype(BF16))

        def last_down():
            mlp_down(range(2, NQ))
            combine(rprev, rdst, 1 - par)

        nint = 7 * (FS // 2) - 22
        lhs_a = jnp.concatenate([mem_ref[...], xn[0:40]], axis=0).astype(BF16)
        mlp_up(8)
        sa = segment(lhs_a, build_qkv_a, build_o_a, [lambda: mlp_up(7), lambda: None, lambda: mlp_up(7)])
        mem_ref[...] = sa[0:8]
        s_ref[par, 0:24, :] = sa[8:32]
        lhs_b = jnp.concatenate([sa[0:8], xn[40:64]], axis=0).astype(BF16)
        sb = segment(lhs_b, build_qkv_b, build_o_b,
                     [lambda: mlp_down(range(0, 2)), last_down, lambda: None],
                     inter=lambda p: mlp_up(1) if 2 <= p < 2 + nint else None)
        mem_ref[...] = sb[0:8]
        s_ref[par, 24:64, :] = sb[8:48]

        @pl.when(j >= 1)
        def _():
            out_copy(rprev).start()
        return c
    lax.fori_loop(0, S // STEP, step, 0)
    combine(S - STEP, S - STEP, 1)
    out_copy(S - STEP).start()
    pltpu.make_async_copy(x_ref.at[pl.ds(0, S)], out_hbm, sems.at[SEM_OUT]).wait()


@functools.partial(jax.jit, static_argnames=("A_seg_len",))
def pallas_recurrent_scan__memory_aug_recurrent_mem_tr__mixer_s_mlp__prompt_kernel(
        A_x, A_mem0, A_Wq, A_Wk, A_Wv, A_Wo, A_seg_len, B_x, B_w1, B_w2, B_w3, B_w4):
    del B_x
    B, S, D = A_x.shape
    _, H, DH = A_Wq.shape
    M = A_mem0.shape[1]
    FF = B_w3.shape[1]
    assert (B, S, D, H, DH, M, A_seg_len, FF) == (1, 2048, 1024, 32, 128, 8, 32, 3584)
    nd, nf = D // 128, FF // 128
    kern = functools.partial(_kernel, S=S, D=D, H=H, DH=DH, M=M, SEG=A_seg_len, FF=FF)
    any_spec = pl.BlockSpec(memory_space=pl.ANY)
    out = pl.pallas_call(
        kern,
        out_shape=jax.ShapeDtypeStruct((S, D), A_x.dtype),
        in_specs=[any_spec] * 10,
        out_specs=any_spec,
        scratch_shapes=[
            pltpu.VMEM((S + STEP, D), BF16),
            pltpu.VMEM((3 * H // 2, D, 128), U32),
            pltpu.VMEM((3 * H, D // 2, 128), U32),
            pltpu.VMEM((nd, H * DH // 2, 128), U32),
            pltpu.VMEM((nd, D // 2, 128), U32),
            pltpu.VMEM((3 * nd // 2, 7 * D // 4, 128), U32),
            pltpu.VMEM(((nf - CPRE) // 2, 7 * D // 4, 128), U32),
            pltpu.VMEM((nd, 7 * (nf - CPRE) * 16, 128), U32),
            pltpu.VMEM((nd, S + 16, 128), F32),
            pltpu.VMEM((S, D), F32),
            pltpu.VMEM((S // BLK, 7, HB // 2, D // 2), U32),
            pltpu.VMEM((HB // 2, D), U32),
            pltpu.VMEM((7, HB // 2, D // 2), U32),
            pltpu.VMEM((2, STEP, D), F32),
            pltpu.VMEM((M, D), BF16),
            pltpu.VMEM((M, D), F32),
            pltpu.SemaphoreType.DMA((4 + nd + 4 + 2 * ((S - RB0) // RB1) + S // RB2,)),
        ],
        compiler_params=pltpu.CompilerParams(vmem_limit_bytes=120 * 1024 * 1024,
                                             disable_bounds_checks=True),
    )(A_x[0], A_mem0[0], A_Wq, A_Wk, A_Wv, A_Wo.reshape(H * DH, D), B_w1, B_w2, B_w3, B_w4)
    return out[None]
```

```python
import functools

import jax
import jax.numpy as jnp
from jax import lax
import jax.experimental.pallas as pl
import jax.experimental.pallas.tpu as pltpu

F32 = jnp.float32
BF16 = jnp.bfloat16
U32 = jnp.uint32
EPS = 1e-5
LOG2E = 1.4426950408889634

HB = 64
BLK = 2 * HB
RB0 = 512
RA = 256
RB1 = 384
RB2 = 512
CPRE = 8
STEP = 64
NPRE = 2
W1G = ((0, 2), (2, 5), (5, 8))
XK = 320
CH = 16


def _ln(x):
    m = jnp.mean(x, axis=-1, keepdims=True)
    xc = x - m
    v = jnp.mean(xc * xc, axis=-1, keepdims=True)
    return xc * lax.rsqrt(v + EPS)


def _gelu(x):
    c = 0.7978845608028654
    h = 0.5 * x
    return h + h * jnp.tanh(x * (c + (c * 0.044715) * (x * x)))


def _bf(w_u32):
    return pltpu.bitcast(w_u32, BF16)


def _pk(x):
    return pltpu.bitcast(x.astype(BF16), U32)


def _dot(a, w_u32):
    return jnp.dot(a, _bf(w_u32), preferred_element_type=F32)


def _zero_of(y):
    if y.dtype != U32:
        y = pltpu.bitcast(y[0:(8 if y.dtype == F32 else 16), 0:128], U32)
    return (y[0:8, 0:128] >> 31) >> 1


def _after(y, z):
    return jnp.concatenate([y[0:8] + pltpu.bitcast(z, F32), y[8:]], axis=0)


def _left(get, nk):
    rows, zs = [], []
    for r in range(0, HB, CH):
        cols = []
        for t in range(nk):
            a11, a12, a21, a22 = get(r, t), get(r, nk + t), get(HB + r, t), get(HB + r, nk + t)
            p = [y.astype(BF16) for y in (a11 + a22, a21 + a22, a11, a22, a11 + a12, a21 - a11, a12 - a22)]
            zs.append(_zero_of(functools.reduce(jnp.bitwise_or, [pltpu.bitcast(y, U32) for y in p])))
            cols.append(p)
        rows.append(_cat(cols, 1))
    return _cat(rows, 0), zs


def _cat(parts, axis):
    return [jnp.concatenate([p[t] for p in parts], axis=axis) for t in range(7)]


def _right_sums(b11, b21, b12, b22):
    b11, b21, b12, b22 = [_bf(t).astype(F32) for t in (b11, b21, b12, b22)]
    return [_pk(t) for t in (b21 - b11, b12 - b22, b11 + b22, b11 + b12, b21 + b22)]


class _Pace:
    def __init__(self):
        self.items, self.per, self.before = [], 0, []

    def spread(self, items, nslots):
        self.items, self.per, self.credit = list(items), len(items) / nslots, 0.0

    def require(self, zeros, nslots):
        self.before += [None] * (nslots - len(self.before))
        for i, z in enumerate(zeros):
            k = (i + 1) * nslots // len(zeros) - 1
            self.before[k] = z if self.before[k] is None else self.before[k] | z

    def __call__(self, y):
        if self.items:
            self.credit += self.per
            n = min(int(self.credit + 1e-6), len(self.items))
            self.credit -= n
            if n:
                z = _zero_of(y)
                for _ in range(n):
                    self.items.pop(0)(z)
        if self.before:
            z = self.before.pop(0)
            if z is not None:
                y = _after(y, z)
        return y


def _strassen(al, wt, pace=lambda y: y):
    m1 = pace(_dot(al[0], wt(4)))
    yield None
    m4 = pace(_dot(al[3], wt(1)))
    yield None
    m5 = pace(_dot(al[4], wt(3)))
    yield None
    m2 = pace(_dot(al[1], wt(0)))
    yield None
    m3 = pace(_dot(al[2], wt(2)))
    yield None
    c11 = pace(_dot(al[6], wt(6)) + (m1 + m4 - m5))
    yield None
    c22 = pace(_dot(al[5], wt(5)) + (m1 - m2 + m3))
    yield (jnp.concatenate([c11, m2 + m4], axis=0), jnp.concatenate([m3 + m5, c22], axis=0))


def _run(gen):
    for y in gen:
        pass
    return y


def _gelu_left(y0, y1):
    return _left(lambda r, t: _gelu((y0, y1)[t][r:r + CH]), 1)


def _kernel(x_hbm, mem0_hbm, wq_hbm, wk_hbm, wv_hbm, wo_hbm, w1_hbm, w2_hbm, w3_hbm, w4_hbm, out_hbm,
            x_ref, stage, wqkv_ref, wo_ref, w1_ref, q_ref, p_ref, r_ref,
            h_ref, b_ref, a3_ref, pre1_ref, pre_ref, s_ref, px_ref, e_ref, mem0_ref, mem_ref, sems, *, S, D, H, DH, M, SEG, FF):
    L = M + SEG
    R = 2 * L
    NP = H // 2
    ND = D // 128
    NF = FF // 128
    NQ = ND // 2
    KH = D // 4
    FS = (NF - CPRE) // 2
    FH = FS * 32
    HK = D // 2
    N1 = (S - RB0) // RB1
    N2 = S // RB2
    assert CPRE == ND and FS % 2 == 0
    Q_W2, Q_W3A, Q_W4A = 0, NQ, 2 * NQ
    QI = 3 * NQ // N1
    assert QI * N1 == 3 * NQ and N2 == NQ == 4 and FS // 2 - 1 == NQ

    SEM_WO, SEM_OUT, SEM_MEM, SEM_P = range(4)
    SEM_W1 = 4
    SEM_X = SEM_W1 + ND
    SEM_Q = SEM_X + 4 + N1
    SEM_G = SEM_Q + N1
    JG = NP // N2

    def tile_copy(src, row0, nrows, col, dst, sem):
        cols = pl.ds(pl.multiple_of(col * 128, 128), 128)
        return pltpu.make_async_copy(src.bitcast(U32).at[pl.ds(row0, nrows), cols], dst, sem)

    def quad_copies(src, row0, kh, col, dst_ref, q, sem, dist=1):
        return [tile_copy(src, row0, 2 * kh, col + t * dist, dst_ref.at[q, pl.ds(2 * kh * t, 2 * kh)], sem)
                for t in range(2)]

    def q_copies(q, sem):
        if q < Q_W3A:
            return quad_copies(w2_hbm, 0, KH, 2 * q, q_ref, q, sem)
        if q < Q_W4A:
            return quad_copies(w3_hbm, 0, KH, q - Q_W3A, q_ref, q, sem, CPRE // 2)
        return quad_copies(w4_hbm, 0, KH, 2 * (q - Q_W4A), q_ref, q, sem)

    def x_copy(lo, n, sem):
        return pltpu.make_async_copy(x_hbm.at[pl.ds(lo, n)], x_ref.at[pl.ds(lo, n)], sem)

    def group(i):
        sem = sems.at[SEM_G + i]
        cps = [pltpu.make_async_copy(w.bitcast(U32).at[:, i * JG + k, :], stage.at[m * NP + i * JG + k], sem)
               for m, w in enumerate((wq_hbm, wk_hbm, wv_hbm)) for k in range(JG)]
        for t in range(2):
            rq = 2 * i + t
            par, pair = rq >> 2, rq & 3
            cps += quad_copies(w3_hbm, 0, KH, CPRE + par * FS + 1 + pair, p_ref, rq, sem, FS // 2)
            row0 = pl.multiple_of(CPRE * 64 + par * 2 * FH, 64)
            cps += quad_copies(w4_hbm, row0, FH, 2 * pair, r_ref, rq, sem)
        return cps

    g_mem = [pltpu.make_async_copy(mem0_hbm, mem0_ref, sems.at[SEM_MEM])]
    X0 = S - N1 * XK
    assert all(X0 + (k + 1) * XK >= min(RB0 + (k + 1) * RB1 + HB, S) for k in range(N1))
    xch = [(0, RA), (RA, RA + HB), (RA + HB, RB0 + HB), (RB0 + HB, X0)]
    xch += [(X0 + k * XK, X0 + (k + 1) * XK) for k in range(N1)]
    g_x = [x_copy(lo, hi - lo, sems.at[SEM_X + i]) for i, (lo, hi) in enumerate(xch)]
    g_w1 = [tile_copy(w1_hbm, 0, 2 * KH, j, w1_ref.at[j], sems.at[SEM_W1 + j]) for j in range(ND)]
    g_q = [[cp for t in range(QI) for cp in q_copies(QI * k + t, sems.at[SEM_Q + k])] for k in range(N1)]
    g_p = [cp for par in range(2)
           for cp in quad_copies(w3_hbm, 0, KH, CPRE + par * FS, p_ref, 2 * NQ + par, sems.at[SEM_P], FS // 2)]
    g_wo = [tile_copy(wo_hbm, 0, H * DH // 2, j, wo_ref.at[j], sems.at[SEM_WO]) for j in range(ND)]

    def start(*gs):
        for g in gs:
            for cp in g:
                cp.start()

    def wait(*gs):
        for g in gs:
            for cp in g:
                cp.wait()

    start(g_x[0:1], g_w1[0:6], g_x[1:2], g_w1[6:], g_x[2:4])
    for k in range(N1):
        start(g_x[4 + k:5 + k], g_q[k])
    start(g_mem, g_p)

    def prep_items(ref, q, kh, r0=0, n=None):
        def item(r, z):
            b = [ref[q, pl.ds(t * kh + r0 + r, 8), :] for t in range(4)]
            for t, y in zip((1, 2, 4, 5, 6), _right_sums(b[0] | z, b[1], b[2], b[3] | z)):
                ref[q, pl.ds(t * kh + r0 + r, 8), :] = y
        return [functools.partial(item, r) for r in range(0, kh if n is None else n, 8)]

    def quad_wt(ref, q, kh):
        return lambda i: ref[q, i * kh:(i + 1) * kh, :]

    def load_left(ref):
        return [_bf(ref[t]) for t in range(7)]

    def store_left(ref, al):
        for t in range(7):
            ref[t] = pltpu.bitcast(al[t], U32)

    h_ref[:, 0:8, :] = jnp.zeros((ND, 8, 128), F32)
    h_ref[:, S + 8:S + 16, :] = jnp.zeros((ND, 8, 128), F32)
    s_ref[...] = jnp.zeros(s_ref.shape, F32)

    def ln2(r):
        xn = _ln(x_ref[pl.ds(r, HB), :].astype(F32))
        b_ref[pl.ds(r, HB), :] = xn
        top = jnp.concatenate([xn[g * SEG + 16:g * SEG + 24] for g in range(HB // SEG)], axis=0)
        bot = jnp.concatenate([xn[g * SEG + 24:g * SEG + 32] for g in range(HB // SEG)], axis=0)
        t1, t2, b1, b2 = top[:, :HK], top[:, HK:], bot[:, :HK], bot[:, HK:]
        rows = pl.ds(pl.multiple_of(((r >> 6) & 1) * 8, 8), 8)
        for k, v in enumerate((t1 + b2, b1 - t1, t2 - b2)):
            e_ref[r >> 7, k, rows, :] = _pk(v)
        return _ln(xn).astype(BF16)

    def shifted_left(r0):
        offs = (7, 9, 6, 10)
        return _left(lambda r, t: _gelu(h_ref[t, pl.ds(r0 + r + offs[4 * t // ND], CH), :]), NQ)

    def p1_rows(base, n, a, pace):
        for s in range(n):
            r = base + s * HB
            nxt = r + HB if s + 1 < n else pl.multiple_of(jnp.minimum(r + HB, S - HB), HB)
            a_n = ln2(nxt)
            for j in range(ND):
                h_ref[j, pl.ds(r + 8, HB), :] = pace(_dot(a, w1_ref[j]))
            a = a_n
        pre1_ref[...] = pltpu.bitcast(a, U32)

    NA = RA // HB
    wait(g_x[0:1])
    a0 = [ln2(s * HB) for s in range(NPRE)]
    for gi, (j0, j1) in enumerate(W1G):
        wait(g_w1[j0:j1])
        if gi == len(W1G) - 1:
            wait(g_x[1:2])
            a_n = ln2(RA)
        for s in range(NA):
            if s == len(a0):
                a0.append(ln2(s * HB))
            for j in range(j0, j1):
                h_ref[j, pl.ds(s * HB + 8, HB), :] = _dot(a0[s], w1_ref[j])
    wait(g_x[2:3])
    al0, zs = shifted_left(0)
    store_left(pre_ref, al0)
    pace = _Pace()
    pace.require(zs, (RB0 - RA) // HB * ND - 2)
    p1_rows(RA, (RB0 - RA) // HB, a_n, pace)
    wait(g_x[3:4])

    def p1(k, c):
        base = pl.multiple_of(RB0 + k * RB1, BLK)
        x_copy(pl.multiple_of(X0 + k * XK, HB), XK, sems.at[SEM_X + 4 + k]).wait()
        landed = q_ref.at[pl.ds(QI * k, QI), pl.ds(0, 4 * KH)]
        pltpu.make_async_copy(landed, landed, sems.at[SEM_Q + k]).wait()

        @pl.when((k & 1) == 1)
        def _():
            start(group(k >> 1))

        pace = _Pace()
        pace.spread([t_ for t in range(QI) for t_ in prep_items(q_ref, QI * k + t, KH)], RB1 // HB * ND)
        p1_rows(base, RB1 // HB, _bf(pre1_ref[...]), pace)
        assert not pace.items
        return c
    lax.fori_loop(0, N1, p1, 0)

    wait(g_mem, g_p)
    mem_ref[...] = mem0_ref[...].astype(F32)

    def p2(it, c):
        base = pl.multiple_of(it * RB2, RB2)
        nb = RB2 // BLK
        g = [None] * nb
        u = [None] * nb
        g[0] = load_left(pre_ref)

        def repack(k, i, z):
            slab = (k // JG) * NP + it * JG + k % JG
            ae, ao, be, bo = [stage[slab, pl.ds(o + i * 16, 8, stride=2), :] for o in (0, 1, HK, HK + 1)]
            ae, be = ae | z, be | z
            hi = U32(0xFFFF0000)
            f = lambda y: pltpu.bitcast(y, F32)
            b11, b12 = (ae << 16, ao << 16), (ae & hi, ao & hi)
            b21, b22 = (be << 16, bo << 16), (be & hi, bo & hi)

            def pk(x, y, sign):
                v = [f(p) + f(q) if sign > 0 else f(p) - f(q) for p, q in zip(x, y)]
                return pltpu.bitcast(pltpu.pack_elementwise(v, packed_dtype=BF16), U32)
            r = pl.ds(i * 8, 8)
            r2 = pl.ds(KH + i * 8, 8)
            wqkv_ref[2 * slab, r, :] = (ae & U32(0xFFFF)) | b11[1]
            wqkv_ref[2 * slab, r2, :] = pk(b21, b11, -1)
            wqkv_ref[2 * slab + 1, r, :] = pk(b12, b22, -1)
            wqkv_ref[2 * slab + 1, r2, :] = (be >> 16) | b22[1]
            stage[slab, pl.ds(i * 16, 8), :] = pk(b11, b22, 1)
            stage[slab, pl.ds(i * 16 + 8, 8), :] = pk(b11, b12, 1)
            stage[slab, pl.ds(HK + i * 16, 8), :] = pk(b21, b22, 1)

        rp = [functools.partial(repack, k, i) for k in range(3 * JG) for i in range(KH // 8)]
        pp = [it_ for t in range(2) for it_ in
              prep_items(p_ref, 2 * it + t, KH) + prep_items(r_ref, 2 * it + t, FH)
              + prep_items(p_ref, 2 * NQ + t, KH, pl.multiple_of(it * (KH // N2), 8), KH // N2)]
        items = []
        while rp or pp:
            items += rp[:5] + pp[:2]
            rp, pp = rp[5:], pp[2:]
        pace = _Pace()
        SL = NQ * 7

        zeros = {}
        carry = {}
        nitems = len(items)

        def make_g(s):
            if s < nb:
                g[s], zeros["g", s] = shifted_left(base + s * BLK)
            else:
                al_n, zeros["g", s] = shifted_left(pl.multiple_of(jnp.minimum(base + RB2, S - BLK), BLK))
                store_left(pre_ref, al_n)

        def mix(s):
            ys = []
            for q in range(NQ):
                ys += _run(_strassen(g[s], quad_wt(q_ref, Q_W2 + q, KH), pace))
            if s == nb - 1:
                wait(group(it))

                @pl.when(it < N2 - 2)
                def _():
                    start(group(it + 2))

                @pl.when(it == N2 - 2)
                def _():
                    start(g_wo)
                pace.spread(items, 1)
            rows = pl.ds(base + s * BLK, BLK)
            x1 = jnp.concatenate(ys, axis=1) + b_ref[rows, :]
            b_ref[rows, :] = x1
            y = [_ln(x1[r:r + CH]) for r in range(0, BLK, CH)]
            al, zeros["a", s] = _left(lambda r, t: y[r // CH][:, t * 128:(t + 1) * 128], NQ)
            store_left(a3_ref.at[it * nb + s], al)

        def up(s):
            al = load_left(a3_ref.at[it * nb + s])
            parts = []
            for q in range(NQ):
                p, carry[0] = _gelu_left(*_run(_strassen(al, quad_wt(q_ref, Q_W3A + q, KH), pace)))
                parts.append(p)
                if q + 1 < NQ:
                    pace.require(carry.pop(0), 7)
            u[s] = _cat(parts, 1)

        def down(s):
            for q in range(NQ):
                ys = _run(_strassen(u[s], quad_wt(q_ref, Q_W4A + q, KH), pace))
                for t in range(2):
                    cols = slice((2 * q + t) * 128, (2 * q + t + 1) * 128)
                    rows = pl.ds(base + s * BLK, BLK)
                    b_ref[rows, cols] = ys[t] + b_ref[rows, cols]

        assert nb == 4
        for s in range(1, nb):
            make_g(s)
        zg = zeros["g", 1] + zeros["g", 2] + zeros["g", 3]
        zeros["g01"], zeros["g12"], zeros["g23"] = zg[:24], zg[24:36], zg[36:]
        plan = [(mix, 0, ["g01"], 0), (mix, 1, [("a", 0), "g12"], 0), (mix, 2, [("a", 1), "g23"], 0),
                (mix, 3, [("a", 2)], 0), (up, 0, [("a", 3)], 0.3), (up, 1, [], 0.8), (down, 0, [], 1.6),
                (up, 2, [], 0.8), (down, 1, [], 1.6), (up, 3, [], 0.8), (down, 2, [], 1.6),
                (down, 3, [("g", 4)], 1.0)]
        wsum = sum(p[3] for p in plan) - plan[-1][3] * 2 / SL
        for fn, s, keys, w in plan:
            for key in keys:
                if key not in zeros:
                    make_g(key[1])
            zs = carry.pop(0, []) + [z for key in keys for z in zeros[key]]
            if zs:
                pace.require(zs, SL - 1 if keys else 7)
            pace.per = nitems * w / wsum / SL
            fn(s)
        assert not pace.items
        return c
    lax.fori_loop(0, N2, p2, 0)
    wait(g_wo)

    row = lax.broadcasted_iota(jnp.int32, (R, R), 0)
    col = lax.broadcasted_iota(jnp.int32, (R, R), 1)
    same_head = (row >= L) == (col >= L)
    rr = jnp.where(row >= L, row - L, row)
    cc = jnp.where(col >= L, col - L, col)
    visible = same_head & ((rr < M) | (rr >= cc))
    scale = DH ** -0.5
    fill = jnp.where(same_head, -1e9 / scale, -jnp.inf).astype(F32)

    def softmax_qk(q2, k2):
        s = lax.dot_general(q2, k2, (((1,), (1,)), ((), ())), preferred_element_type=F32)
        s = jnp.where(visible, s, fill)
        m = jnp.max(s, axis=-1, keepdims=True)
        e = jnp.exp2((s - m) * (scale * LOG2E))
        l = jnp.sum(e, axis=-1, keepdims=True)
        r = pl.reciprocal(l, approx=True)
        r = r * (2.0 - l * r)
        return (e * r).astype(BF16)

    def combine(r, rdst, slot):
        b = b_ref[pl.ds(r, STEP), :]
        g = b * jax.nn.sigmoid(b)
        x = x_ref[pl.ds(r, STEP), :].astype(F32)
        x_ref[pl.ds(rdst, STEP), :] = (x + s_ref[slot] * g).astype(x_ref.dtype)

    def out_copy(r):
        return pltpu.make_async_copy(x_ref.at[pl.ds(r, STEP)], out_hbm.at[pl.ds(r, STEP)], sems.at[SEM_OUT])

    def qkv_extra(blk, slab):
        def wt(off):
            return jnp.concatenate([stage[slab, off + 16 * i:off + 16 * i + 8, :] for i in range(KH // 8)], axis=0)
        e = [_bf(e_ref[jnp.minimum(blk, S // BLK - 1), k]) for k in range(3)]
        m1 = _dot(e[0], wt(0))
        px_ref[blk & 1, slab, 1] = _dot(e[1], wt(8)) + m1
        px_ref[blk & 1, slab, 0] = _dot(e[2], wt(HK)) + m1

    for p in range(NP // 2):
        for m in range(3):
            qkv_extra(0, m * NP + p)

    def step(j, c):
        r0 = pl.multiple_of(j * STEP, STEP)
        par = j & 1
        blk = j >> 1
        rb = pl.multiple_of(blk * BLK, BLK)
        rprev = pl.multiple_of(jnp.maximum(r0 - STEP, 0), STEP)
        rdst = pl.multiple_of(jnp.where(j >= 1, r0 - STEP, S), STEP)
        al3 = load_left(a3_ref.at[blk])
        xn = _ln(x_ref[pl.ds(r0, STEP), :].astype(F32))

        parts = []

        def up_products():
            for q in range(FS // 2):
                wt = quad_wt(p_ref, 2 * NQ + par if q == 0 else par * NQ + q - 1, KH)
                for y in _strassen(al3, wt):
                    if y is not None:
                        parts.append(_gelu_left(*y)[0])
                    yield

        def down_products():
            al4 = _cat(parts, 1)
            for q in range(NQ):
                for ys in _strassen(al4, quad_wt(r_ref, par * NQ + q, FH)):
                    if ys is not None:
                        for t in range(2):
                            cols = slice((2 * q + t) * 128, (2 * q + t + 1) * 128)
                            b_ref[pl.ds(rb, BLK), cols] = ys[t] + b_ref[pl.ds(rb, BLK), cols]
                    yield
        ups, downs = up_products(), down_products()

        def run(gen, n):
            for _ in range(n):
                next(gen)

        def segment(sg, mem, build_o, fillers, inter):
            m1, m2 = mem[:, :HK], mem[:, HK:]
            x1, x2 = xn[sg * SEG:(sg + 1) * SEG, :HK], xn[sg * SEG:(sg + 1) * SEG, HK:]
            ms, xs = m1 + m2, x1 + x2
            lhs = [jnp.concatenate(v, axis=0).astype(BF16) for v in (
                [ms, xs[0:16], xs[24:32]], [m2, x2[0:16], x2[24:32]],
                [m1, x1[0:16], x1[16:24]], [ms, xs[0:16], xs[16:24]])]
            prow = pl.ds(pl.multiple_of((par * 2 + sg) * 8, 8), 8)
            qkv = [None] * NP
            prob = [None] * NP
            o = [None] * H
            ph = NP - 3
            ks = ph * 128

            def do_qkv(p):
                res = []
                for m in range(3):
                    w0, w1 = m * H + 2 * p, m * H + 2 * p + 1
                    d11 = _dot(lhs[0], wqkv_ref[w0, 0:KH, :])
                    d4 = _dot(lhs[1], wqkv_ref[w0, KH:, :])
                    d3 = _dot(lhs[2], wqkv_ref[w1, 0:KH, :])
                    d22 = _dot(lhs[3], wqkv_ref[w1, KH:, :])
                    pt = px_ref[blk & 1, m * NP + p, 0, prow, :]
                    pb = px_ref[blk & 1, m * NP + p, 1, prow, :]
                    res.append(jnp.concatenate([
                        d11[0:24] + d4[0:24], pt + (d4[24:32] - d22[24:32]), d11[24:32] + d4[24:32],
                        d3[0:24] + d22[0:24], d3[24:32] + d22[24:32], pb + (d3[24:32] - d11[24:32])],
                        axis=0).astype(BF16))
                qkv[p] = res

            def do_qk(p):
                prob[p] = softmax_qk(qkv[p][0], qkv[p][1])

            def do_pv(p):
                o2 = jnp.dot(prob[p], qkv[p][2], preferred_element_type=F32)
                o[2 * p], o[2 * p + 1] = build_o(p, o2)

            for p in range(NP):
                do_qkv(p)
                inter(p)
                if p >= 1:
                    do_qk(p - 1)
                if p >= 3:
                    do_pv(p - 3)
            fillers[0]()
            do_qk(NP - 1)
            do_pv(NP - 3)
            do_pv(NP - 2)
            olo = jnp.concatenate(o[:2 * ph], axis=1)
            acc = [_dot(olo, wo_ref[n, 0:ks, :]) for n in range(ND // 2)]
            do_pv(NP - 1)
            fillers[1]()
            acc += [_dot(olo, wo_ref[n, 0:ks, :]) for n in range(ND // 2, ND)]
            ohi = jnp.concatenate(o[2 * ph:], axis=1)
            res = jnp.concatenate([_dot(ohi, wo_ref[n, ks:, :]) + acc[n] for n in range(ND)], axis=1)
            fillers[2]()
            return res

        o_kept = [None] * H

        def build_o_a(p, o2):
            o_kept[2 * p] = o2[32:40]
            o_kept[2 * p + 1] = o2[72:80]
            return o2[0:32].astype(BF16), o2[40:72].astype(BF16)

        def build_o_b(p, o2):
            return (jnp.concatenate([o2[0:8], o_kept[2 * p], o2[8:40]], axis=0).astype(BF16),
                    jnp.concatenate([o2[40:48], o_kept[2 * p + 1], o2[48:80]], axis=0).astype(BF16))

        U0, U1, IA, IB, D0 = 7, 6, 1, 2, 7

        def inter_a(p):
            if p < NP // 2:
                for m in range(3):
                    qkv_extra((j + 1) >> 1, m * NP + (1 - par) * (NP // 2) + p)
            if p >= IA:
                run(ups, 1)

        def last_down():
            run(downs, 28 - (NP - IB) - D0)
            combine(rprev, rdst, 1 - par)

        mem = mem_ref[...]
        run(ups, U0)
        sa = segment(0, mem, build_o_a,
                     [lambda: run(ups, U1), lambda: None, lambda: run(ups, 35 - U0 - U1 - (NP - IA))], inter_a)
        mem_ref[...] = sa[0:8]
        s_ref[par, 0:24, :] = sa[8:32]
        sb = segment(1, sa[0:8], build_o_b, [lambda: run(downs, D0), last_down, lambda: None],
                     lambda p: run(downs, 1) if p >= IB else None)
        mem_ref[...] = sb[0:8]
        s_ref[par, 24:64, :] = sb[8:48]

        @pl.when(j >= 1)
        def _():
            out_copy(rprev).start()
        return c
    lax.fori_loop(0, S // STEP, step, 0)
    combine(S - STEP, S - STEP, 1)
    out_copy(S - STEP).start()
    pltpu.make_async_copy(x_ref.at[pl.ds(0, S)], out_hbm, sems.at[SEM_OUT]).wait()


@functools.partial(jax.jit, static_argnames=("A_seg_len",))
def pallas_recurrent_scan__memory_aug_recurrent_mem_tr__mixer_s_mlp__prompt_kernel(
        A_x, A_mem0, A_Wq, A_Wk, A_Wv, A_Wo, A_seg_len, B_x, B_w1, B_w2, B_w3, B_w4):
    del B_x
    B, S, D = A_x.shape
    _, H, DH = A_Wq.shape
    M = A_mem0.shape[1]
    FF = B_w3.shape[1]
    assert (B, S, D, H, DH, M, A_seg_len, FF) == (1, 2048, 1024, 32, 128, 8, 32, 3584)
    nd, nf = D // 128, FF // 128
    kern = functools.partial(_kernel, S=S, D=D, H=H, DH=DH, M=M, SEG=A_seg_len, FF=FF)
    any_spec = pl.BlockSpec(memory_space=pl.ANY)
    out = pl.pallas_call(
        kern,
        out_shape=jax.ShapeDtypeStruct((S, D), A_x.dtype),
        in_specs=[any_spec] * 10,
        out_specs=any_spec,
        scratch_shapes=[
            pltpu.VMEM((S + STEP, D), BF16),
            pltpu.VMEM((3 * H // 2, D, 128), U32),
            pltpu.VMEM((3 * H, D // 2, 128), U32),
            pltpu.VMEM((nd, H * DH // 2, 128), U32),
            pltpu.VMEM((nd, D // 2, 128), U32),
            pltpu.VMEM((3 * nd // 2, 7 * D // 4, 128), U32),
            pltpu.VMEM(((nf - CPRE) // 2, 7 * D // 4, 128), U32),
            pltpu.VMEM((nd, 7 * (nf - CPRE) * 16, 128), U32),
            pltpu.VMEM((nd, S + 16, 128), F32),
            pltpu.VMEM((S, D), F32),
            pltpu.VMEM((S // BLK, 7, HB // 2, D // 2), U32),
            pltpu.VMEM((HB // 2, D), U32),
            pltpu.VMEM((7, HB // 2, D // 2), U32),
            pltpu.VMEM((2, STEP, D), F32),
            pltpu.VMEM((2, 3 * H // 2, 2, 32, 128), F32),
            pltpu.VMEM((S // BLK, 3, 16, D // 2), U32),
            pltpu.VMEM((M, D), BF16),
            pltpu.VMEM((M, D), F32),
            pltpu.SemaphoreType.DMA((4 + nd + 4 + 2 * ((S - RB0) // RB1) + S // RB2,)),
        ],
        compiler_params=pltpu.CompilerParams(vmem_limit_bytes=126 * 1024 * 1024,
                                             disable_bounds_checks=True),
    )(A_x[0], A_mem0[0], A_Wq, A_Wk, A_Wv, A_Wo.reshape(H * DH, D), B_w1, B_w2, B_w3, B_w4)
    return out[None]
```

```python
import functools

import jax
import jax.numpy as jnp
from jax import lax
import jax.experimental.pallas as pl
import jax.experimental.pallas.tpu as pltpu

F32 = jnp.float32
BF16 = jnp.bfloat16
U32 = jnp.uint32
EPS = 1e-5
LOG2E = 1.4426950408889634

HB = 64
BLK = 2 * HB
RB0 = 512
RA = 256
RB1 = 256
RB2 = 512
CPRE = 8
STEP = 64
NPRE = 2
W1G = ((0, 2), (2, 5), (5, 8))
XK = 192
CH = 16


def _ln(x):
    m = jnp.mean(x, axis=-1, keepdims=True)
    xc = x - m
    v = jnp.mean(xc * xc, axis=-1, keepdims=True)
    return xc * lax.rsqrt(v + EPS)


def _gelu(x):
    c = 0.7978845608028654
    h = 0.5 * x
    return h + h * jnp.tanh(x * (c + (c * 0.044715) * (x * x)))


def _bf(w_u32):
    return pltpu.bitcast(w_u32, BF16)


def _pk(x):
    return pltpu.bitcast(x.astype(BF16), U32)


def _dot(a, w_u32):
    return jnp.dot(a, _bf(w_u32), preferred_element_type=F32)


def _zero_of(y):
    if y.dtype != U32:
        y = pltpu.bitcast(y[0:(8 if y.dtype == F32 else 16), 0:128], U32)
    return (y[0:8, 0:128] >> 31) >> 1


def _after(y, z):
    return jnp.concatenate([y[0:8] + pltpu.bitcast(z, F32), y[8:]], axis=0)


def _left(get, nk):
    rows, zs = [], []
    for r in range(0, HB, CH):
        cols = []
        for t in range(nk):
            a11, a12, a21, a22 = get(r, t), get(r, nk + t), get(HB + r, t), get(HB + r, nk + t)
            p = [y.astype(BF16) for y in (a11 + a22, a21 + a22, a11, a22, a11 + a12, a21 - a11, a12 - a22)]
            zs.append(_zero_of(functools.reduce(jnp.bitwise_or, [pltpu.bitcast(y, U32) for y in p])))
            cols.append(p)
        rows.append(_cat(cols, 1))
    return _cat(rows, 0), zs


def _cat(parts, axis):
    return [jnp.concatenate([p[t] for p in parts], axis=axis) for t in range(7)]


def _unpack(w):
    return pltpu.bitcast(w << 16, F32), pltpu.bitcast(w & U32(0xFFFF0000), F32)


def _pack2(x, y, sign):
    v = [p + q if sign > 0 else p - q for p, q in zip(x, y)]
    return pltpu.bitcast(pltpu.pack_elementwise(v, packed_dtype=BF16), U32)


def _right_sums(b11, b21, b12, b22):
    b11, b21, b12, b22 = [_unpack(t) for t in (b11, b21, b12, b22)]
    return [_pack2(b21, b11, -1), _pack2(b12, b22, -1), _pack2(b11, b22, 1), _pack2(b11, b12, 1),
            _pack2(b21, b22, 1)]


class _Pace:
    def __init__(self):
        self.items, self.per, self.before = [], 0, []

    def spread(self, items, nslots):
        self.items, self.per, self.credit = list(items), len(items) / nslots, 0.0

    def require(self, zeros, nslots):
        self.before += [None] * (nslots - len(self.before))
        for i, z in enumerate(zeros):
            k = (i + 1) * nslots // len(zeros) - 1
            self.before[k] = z if self.before[k] is None else self.before[k] | z

    def __call__(self, y):
        if self.items:
            self.credit += self.per
            n = min(int(self.credit + 1e-6), len(self.items))
            self.credit -= n
            if n:
                z = _zero_of(y)
                for _ in range(n):
                    self.items.pop(0)(z)
        if self.before:
            z = self.before.pop(0)
            if z is not None:
                y = _after(y, z)
        return y


def _strassen(al, wt, pace=lambda y: y):
    m1 = pace(_dot(al[0], wt(4)))
    yield None
    m4 = pace(_dot(al[3], wt(1)))
    yield None
    m5 = pace(_dot(al[4], wt(3)))
    yield None
    m2 = pace(_dot(al[1], wt(0)))
    yield None
    m3 = pace(_dot(al[2], wt(2)))
    yield None
    c11 = pace(_dot(al[6], wt(6)) + (m1 + m4 - m5))
    yield None
    c22 = pace(_dot(al[5], wt(5)) + (m1 - m2 + m3))
    yield (jnp.concatenate([c11, m2 + m4], axis=0), jnp.concatenate([m3 + m5, c22], axis=0))


def _run(gen):
    for y in gen:
        pass
    return y


def _gelu_left(y0, y1):
    return _left(lambda r, t: _gelu((y0, y1)[t][r:r + CH]), 1)


def _kernel(x_hbm, mem0_hbm, wq_hbm, wk_hbm, wv_hbm, wo_hbm, w1_hbm, w2_hbm, w3_hbm, w4_hbm, out_hbm,
            x_ref, stage, wqkv_ref, wo_ref, w1_ref, q_ref, p_ref, r_ref,
            h_ref, b_ref, a3_ref, pre1_ref, pre_ref, s_ref, px_ref, e_ref, oe_ref, mem0_ref, mem_ref, sems, *, S, D, H, DH, M, SEG, FF):
    L = M + SEG
    R = 2 * L
    NP = H // 2
    ND = D // 128
    NF = FF // 128
    NQ = ND // 2
    KH = D // 4
    FS = (NF - CPRE) // 2
    FH = FS * 32
    HK = D // 2
    N1 = (S - RB0) // RB1
    N2 = S // RB2
    assert CPRE == ND and FS % 2 == 0
    Q_W2, Q_W3A, Q_W4A = 0, NQ, 2 * NQ
    QI = 3 * NQ // N1
    assert QI * N1 == 3 * NQ and N2 == NQ == 4 and FS // 2 - 1 == NQ

    SEM_OUT, SEM_MEM = range(2)
    SEM_W1 = 2
    SEM_X = SEM_W1 + ND
    SEM_Q = SEM_X + 4 + N1
    SEM_G = SEM_Q + N1
    KQ = KH // N2
    JG = NP // N2

    def tile_copy(src, row0, nrows, col, dst, sem):
        cols = pl.ds(pl.multiple_of(col * 128, 128), 128)
        return pltpu.make_async_copy(src.bitcast(U32).at[pl.ds(row0, nrows), cols], dst, sem)

    def quad_copies(src, row0, kh, col, dst_ref, q, sem, dist=1):
        return [tile_copy(src, row0, 2 * kh, col + t * dist, dst_ref.at[q, pl.ds(2 * kh * t, 2 * kh)], sem)
                for t in range(2)]

    def q_copies(q, sem):
        if q < Q_W3A:
            return quad_copies(w2_hbm, 0, KH, 2 * q, q_ref, q, sem)
        if q < Q_W4A:
            return quad_copies(w3_hbm, 0, KH, q - Q_W3A, q_ref, q, sem, CPRE // 2)
        return quad_copies(w4_hbm, 0, KH, 2 * (q - Q_W4A), q_ref, q, sem)

    def x_copy(lo, n, sem):
        return pltpu.make_async_copy(x_hbm.at[pl.ds(lo, n)], x_ref.at[pl.ds(lo, n)], sem)

    def group(i):
        sem = sems.at[SEM_G + i]
        cps = [pltpu.make_async_copy(w.bitcast(U32).at[:, i * JG + k, :], stage.at[m * NP + i * JG + k], sem)
               for m, w in enumerate((wq_hbm, wk_hbm, wv_hbm)) for k in range(JG)]
        for t in range(2):
            rq = 2 * i + t
            par, pair = rq >> 2, rq & 3
            cps += quad_copies(w3_hbm, 0, KH, CPRE + par * FS + 1 + pair, p_ref, rq, sem, FS // 2)
            row0 = pl.multiple_of(CPRE * 64 + par * 2 * FH, 64)
            cps += quad_copies(w4_hbm, row0, FH, 2 * pair, r_ref, rq, sem)
            cps.append(tile_copy(wo_hbm, 0, H * DH // 2, rq, wo_ref.at[rq], sem))
            for sl in range(4):
                r = pl.multiple_of(i * KQ, KQ)
                cps.append(tile_copy(w3_hbm, (sl % 2) * KH + r, KQ, CPRE + t * FS + (sl // 2) * (FS // 2),
                                     p_ref.at[2 * NQ + t, pl.ds(sl * KH + r, KQ)], sem))
        return cps

    g_mem = [pltpu.make_async_copy(mem0_hbm, mem0_ref, sems.at[SEM_MEM])]
    X0 = S - N1 * XK
    assert all(X0 + (k + 1) * XK >= min(RB0 + (k + 1) * RB1 + HB, S) for k in range(N1))
    xch = [(0, RA), (RA, RA + HB), (RA + HB, RB0 + HB), (RB0 + HB, X0)]
    xch += [(X0 + k * XK, X0 + (k + 1) * XK) for k in range(N1)]
    g_x = [x_copy(lo, hi - lo, sems.at[SEM_X + i]) for i, (lo, hi) in enumerate(xch)]
    g_w1 = [tile_copy(w1_hbm, 0, 2 * KH, j, w1_ref.at[j], sems.at[SEM_W1 + j]) for j in range(ND)]
    g_q = [[cp for t in range(QI) for cp in q_copies(QI * k + t, sems.at[SEM_Q + k])] for k in range(N1)]

    def start(*gs):
        for g in gs:
            for cp in g:
                cp.start()

    def wait(*gs):
        for g in gs:
            for cp in g:
                cp.wait()

    start(g_x[0:1], g_w1[0:6], g_x[1:2], g_w1[6:], g_x[2:4])
    for k in range(N1):
        start(g_x[4 + k:5 + k], g_q[k])
    start(g_mem)

    def prep_items(ref, q, kh, r0=0, n=None):
        def item(r, z):
            b = [ref[q, pl.ds(t * kh + r0 + r, 8), :] for t in range(4)]
            for t, y in zip((1, 2, 4, 5, 6), _right_sums(b[0] | z, b[1], b[2], b[3] | z)):
                ref[q, pl.ds(t * kh + r0 + r, 8), :] = y
        return [functools.partial(item, r) for r in range(0, kh if n is None else n, 8)]

    def wos_rows(q, op, v):
        k = (v // 32) * 3 + op
        return (k // JG) * NP + q * JG + k % JG, pl.ds(HK + 16 * (v % 32) + 8, 8)

    def quad_wt(ref, q, kh):
        return lambda i: ref[q, i * kh:(i + 1) * kh, :]

    def load_left(ref):
        return [_bf(ref[t]) for t in range(7)]

    def store_left(ref, al):
        for t in range(7):
            ref[t] = pltpu.bitcast(al[t], U32)

    h_ref[:, 0:8, :] = jnp.zeros((ND, 8, 128), F32)
    h_ref[:, S + 8:S + 16, :] = jnp.zeros((ND, 8, 128), F32)

    def ln2(r):
        xn = _ln(x_ref[pl.ds(r, HB), :].astype(F32))
        b_ref[pl.ds(r, HB), :] = xn
        top = jnp.concatenate([xn[g * SEG + 16:g * SEG + 24] for g in range(HB // SEG)], axis=0)
        bot = jnp.concatenate([xn[g * SEG + 24:g * SEG + 32] for g in range(HB // SEG)], axis=0)
        t1, t2, b1, b2 = top[:, :HK], top[:, HK:], bot[:, :HK], bot[:, HK:]
        rows = pl.ds(pl.multiple_of(((r >> 6) & 1) * 8, 8), 8)
        for k, v in enumerate((t1 + b2, b1 - t1, t2 - b2)):
            e_ref[r >> 7, k, rows, :] = _pk(v)
        return _ln(xn).astype(BF16)

    def shifted_left(r0):
        offs = (7, 9, 6, 10)
        return _left(lambda r, t: _gelu(h_ref[t, pl.ds(r0 + r + offs[4 * t // ND], CH), :]), NQ)

    def p1_rows(base, n, a, pace):
        for s in range(n):
            r = base + s * HB
            nxt = r + HB if s + 1 < n else pl.multiple_of(jnp.minimum(r + HB, S - HB), HB)
            a_n = ln2(nxt)
            for j in range(ND):
                h_ref[j, pl.ds(r + 8, HB), :] = pace(_dot(a, w1_ref[j]))
            a = a_n
        pre1_ref[...] = pltpu.bitcast(a, U32)

    NA = RA // HB
    wait(g_x[0:1])
    a0 = [ln2(s * HB) for s in range(NPRE)]
    for gi, (j0, j1) in enumerate(W1G):
        wait(g_w1[j0:j1])
        if gi == len(W1G) - 1:
            wait(g_x[1:2])
            a_n = ln2(RA)
        for s in range(NA):
            if s == len(a0):
                a0.append(ln2(s * HB))
            for j in range(j0, j1):
                h_ref[j, pl.ds(s * HB + 8, HB), :] = _dot(a0[s], w1_ref[j])
    wait(g_x[2:3])
    al0, zs = shifted_left(0)
    store_left(pre_ref, al0)
    pace = _Pace()
    pace.require(zs, (RB0 - RA) // HB * ND - 2)
    p1_rows(RA, (RB0 - RA) // HB, a_n, pace)
    wait(g_x[3:4])

    def p1(k, c):
        base = pl.multiple_of(RB0 + k * RB1, BLK)
        x_copy(pl.multiple_of(X0 + k * XK, HB), XK, sems.at[SEM_X + 4 + k]).wait()
        landed = q_ref.at[pl.ds(QI * k, QI), pl.ds(0, 4 * KH)]
        pltpu.make_async_copy(landed, landed, sems.at[SEM_Q + k]).wait()

        @pl.when(k == 1)
        def _():
            start(group(0))

        pace = _Pace()
        pace.spread([t_ for t in range(QI) for t_ in prep_items(q_ref, QI * k + t, KH)], RB1 // HB * ND)
        p1_rows(base, RB1 // HB, _bf(pre1_ref[...]), pace)
        assert not pace.items
        return c
    lax.fori_loop(0, N1, p1, 0)

    wait(g_mem)
    mem_ref[...] = mem0_ref[...].astype(F32)

    def p2(it, c):
        base = pl.multiple_of(it * RB2, RB2)
        nb = RB2 // BLK
        g = [None] * nb
        u = [None] * nb
        g[0] = load_left(pre_ref)

        def repack(k, i, z):
            slab = (k // JG) * NP + it * JG + k % JG
            ae, ao, be, bo = [stage[slab, pl.ds(o + i * 16, 8, stride=2), :] for o in (0, 1, HK, HK + 1)]
            ae, be = ae | z, be | z
            hi = U32(0xFFFF0000)
            f = lambda y: pltpu.bitcast(y, F32)
            b11, b12 = (ae << 16, ao << 16), (ae & hi, ao & hi)
            b21, b22 = (be << 16, bo << 16), (be & hi, bo & hi)

            def pk(x, y, sign):
                v = [f(p) + f(q) if sign > 0 else f(p) - f(q) for p, q in zip(x, y)]
                return pltpu.bitcast(pltpu.pack_elementwise(v, packed_dtype=BF16), U32)
            r = pl.ds(i * 8, 8)
            r2 = pl.ds(KH + i * 8, 8)
            wqkv_ref[2 * slab, r, :] = (ae & U32(0xFFFF)) | b11[1]
            wqkv_ref[2 * slab, r2, :] = pk(b21, b11, -1)
            wqkv_ref[2 * slab + 1, r, :] = pk(b12, b22, -1)
            wqkv_ref[2 * slab + 1, r2, :] = (be >> 16) | b22[1]
            stage[slab, pl.ds(i * 16, 8), :] = pk(b11, b22, 1)
            stage[slab, pl.ds(i * 16 + 8, 8), :] = pk(b11, b12, 1)
            stage[slab, pl.ds(HK + i * 16, 8), :] = pk(b21, b22, 1)

        rp = [functools.partial(repack, k, i) for k in range(3 * JG) for i in range(KH // 8)]
        pp = [it_ for t in range(2) for it_ in
              prep_items(p_ref, 2 * it + t, KH) + prep_items(r_ref, 2 * it + t, FH)
              + prep_items(p_ref, 2 * NQ + t, KH, pl.multiple_of(it * KQ, KQ), KQ)]

        def prep_wo(v, z):
            r1, r2 = pl.ds(128 * (v // 8) + 8 * (v % 8), 8), pl.ds(128 * (v // 8) + 64 + 8 * (v % 8), 8)
            s4, s3, *rest = _right_sums(wo_ref[2 * it, r1, :] | z, wo_ref[2 * it, r2, :],
                                        wo_ref[2 * it + 1, r1, :], wo_ref[2 * it + 1, r2, :] | z)
            wo_ref[2 * it, r2, :] = s4
            wo_ref[2 * it + 1, r1, :] = s3
            for op, y in enumerate(rest):
                slab, rows = wos_rows(it, op, v)
                stage[slab, rows, :] = y

        wp = [functools.partial(prep_wo, v) for v in range(128)]
        items = []
        done = 0
        while rp or pp or wp:
            items += rp[:12] + pp[:4 if rp else 2]
            done += len(rp[:12])
            pp = pp[4 if rp else 2:]
            rp = rp[12:]
            n = min(5, done // 96 * 32 - (128 - len(wp)))
            items += wp[:n]
            wp = wp[n:]
        pace = _Pace()
        SL = NQ * 7

        zeros = {}
        carry = {}
        nitems = len(items)

        def make_g(s):
            if s < nb:
                g[s], zeros["g", s] = shifted_left(base + s * BLK)
            else:
                al_n, zeros["g", s] = shifted_left(pl.multiple_of(jnp.minimum(base + RB2, S - BLK), BLK))
                store_left(pre_ref, al_n)

        def next_weights():
            wait(group(it))

            @pl.when(it < N2 - 1)
            def _():
                start(group(it + 1))
            pace.spread(items, 1)

        def mix(s):
            ys = []
            for q in range(NQ):
                ys += _run(_strassen(g[s], quad_wt(q_ref, Q_W2 + q, KH), pace))
            rows = pl.ds(base + s * BLK, BLK)
            x1 = jnp.concatenate(ys, axis=1) + b_ref[rows, :]
            b_ref[rows, :] = x1
            y = [_ln(x1[r:r + CH]) for r in range(0, BLK, CH)]
            al, zeros["a", s] = _left(lambda r, t: y[r // CH][:, t * 128:(t + 1) * 128], NQ)
            store_left(a3_ref.at[it * nb + s], al)

        def up(s):
            al = load_left(a3_ref.at[it * nb + s])
            parts = []
            for q in range(NQ):
                ys = _run(_strassen(al, quad_wt(q_ref, Q_W3A + q, KH), pace))
                if s == 0 and q == NQ - 1:
                    next_weights()
                p, carry[0] = _gelu_left(*ys)
                parts.append(p)
                if q + 1 < NQ:
                    pace.require(carry.pop(0), 7)
            u[s] = _cat(parts, 1)

        def down(s):
            for q in range(NQ):
                ys = _run(_strassen(u[s], quad_wt(q_ref, Q_W4A + q, KH), pace))
                for t in range(2):
                    cols = slice((2 * q + t) * 128, (2 * q + t + 1) * 128)
                    rows = pl.ds(base + s * BLK, BLK)
                    b_ref[rows, cols] = ys[t] + b_ref[rows, cols]

        assert nb == 4
        for s in range(1, nb):
            make_g(s)
        zg = zeros["g", 1] + zeros["g", 2] + zeros["g", 3]
        zeros["g01"], zeros["g12"], zeros["g23"] = zg[:24], zg[24:36], zg[36:]
        plan = [(mix, 0, ["g01"], 0), (mix, 1, [("a", 0), "g12"], 0), (mix, 2, [("a", 1), "g23"], 0),
                (mix, 3, [("a", 2)], 0), (up, 0, [("a", 3)], 0), (up, 1, [], 0.8), (down, 0, [], 1.6),
                (up, 2, [], 0.8), (down, 1, [], 1.6), (up, 3, [], 0.8), (down, 2, [], 1.6),
                (down, 3, [("g", 4)], 1.0)]
        wsum = sum(p[3] for p in plan) - plan[-1][3] * 2 / SL
        for fn, s, keys, w in plan:
            for key in keys:
                if key not in zeros:
                    make_g(key[1])
            zs = carry.pop(0, []) + [z for key in keys for z in zeros[key]]
            if zs:
                pace.require(zs, SL - 1 if keys else 7)
            pace.per = nitems * w / wsum / SL
            fn(s)
        assert not pace.items
        return c
    lax.fori_loop(0, N2, p2, 0)

    row = lax.broadcasted_iota(jnp.int32, (R, R), 0)
    col = lax.broadcasted_iota(jnp.int32, (R, R), 1)
    same_head = (row >= L) == (col >= L)
    rr = jnp.where(row >= L, row - L, row)
    cc = jnp.where(col >= L, col - L, col)
    visible = same_head & ((rr < M) | (rr >= cc))
    scale = DH ** -0.5
    fill = jnp.where(same_head, -1e9 / scale, -jnp.inf).astype(F32)

    def softmax_qk(q2, k2):
        s = lax.dot_general(q2, k2, (((1,), (1,)), ((), ())), preferred_element_type=F32)
        s = jnp.where(visible, s, fill)
        m = jnp.max(s, axis=-1, keepdims=True)
        e = jnp.exp2((s - m) * (scale * LOG2E))
        l = jnp.sum(e, axis=-1, keepdims=True)
        r = pl.reciprocal(l, approx=True)
        r = r * (2.0 - l * r)
        return (e * r).astype(BF16)

    def combine(r, rdst, slot):
        b = b_ref[pl.ds(r, STEP), :]
        hb = 0.5 * b
        g = hb + hb * jnp.tanh(hb)
        x = x_ref[pl.ds(r, STEP), :].astype(F32)
        x_ref[pl.ds(rdst, STEP), :] = (x + s_ref[slot] * g).astype(x_ref.dtype)

    def out_copy(r):
        return pltpu.make_async_copy(x_ref.at[pl.ds(r, STEP)], out_hbm.at[pl.ds(r, STEP)], sems.at[SEM_OUT])

    def qkv_extra(blk, slab):
        def wt(off):
            return jnp.concatenate([stage[slab, off + 16 * i:off + 16 * i + 8, :] for i in range(KH // 8)], axis=0)
        e = [_bf(e_ref[jnp.minimum(blk, S // BLK - 1), k]) for k in range(3)]
        m1 = _dot(e[0], wt(0))
        px_ref[blk & 1, slab, 1] = _dot(e[1], wt(8)) + m1
        px_ref[blk & 1, slab, 0] = _dot(e[2], wt(HK)) + m1

    def wo_extra(kb, q):
        def wt(op):
            return jnp.concatenate([stage[wos_rows(q, op, v) + (slice(None),)] for v in range(128)], axis=0)
        e = [oe_ref[kb & 1, k].astype(BF16) for k in range(3)]
        m1 = _dot(e[0], wt(0))
        pb = _dot(e[1], wt(1)) + m1
        pt = _dot(e[2], wt(2)) + m1
        c0 = pl.ds(pl.multiple_of(2 * q * 128, 128), 128)
        c1 = pl.ds(pl.multiple_of((2 * q + 1) * 128, 128), 128)
        for g in range(4):
            slot = (2 * kb + g // 2) & 3
            r = (g % 2) * SEG + 16
            s_ref[slot, r:r + 8, c0] = s_ref[slot, r:r + 8, c0] + pt[8 * g:8 * g + 8]
            s_ref[slot, r + 8:r + 16, c1] = s_ref[slot, r + 8:r + 16, c1] + pb[8 * g:8 * g + 8]

    def sweep_lhs(m1, m2, x1, x2):
        ms, xs = m1 + m2, x1 + x2
        return [jnp.concatenate(v, axis=0).astype(BF16) for v in (
            [ms, xs[0:16], xs[24:32]], [m2, x2[0:16], x2[24:32]],
            [m1, x1[0:16], x1[16:24]], [ms, xs[0:16], xs[16:24]])]

    s_ref[1:4] = jnp.zeros((3,) + s_ref.shape[1:], F32)
    oe_ref[1] = jnp.zeros(oe_ref.shape[1:], F32)
    for p in range(NP // 2):
        for m in range(3):
            qkv_extra(0, m * NP + p)

    def step(j, c):
        r0 = pl.multiple_of(j * STEP, STEP)
        par = j & 1
        blk = j >> 1
        rb = pl.multiple_of(blk * BLK, BLK)
        rprev = pl.multiple_of(jnp.maximum(r0 - 3 * STEP, 0), STEP)
        rdst = pl.multiple_of(jnp.where(j >= 3, r0 - 3 * STEP, S), STEP)
        al3 = load_left(a3_ref.at[blk])
        xn = _ln(x_ref[pl.ds(r0, STEP), :].astype(F32))

        parts = []

        def up_products():
            for q in range(FS // 2):
                wt = quad_wt(p_ref, 2 * NQ + par if q == 0 else par * NQ + q - 1, KH)
                for y in _strassen(al3, wt):
                    if y is not None:
                        parts.append(_gelu_left(*y)[0])
                    yield

        def down_products():
            al4 = _cat(parts, 1)
            for q in range(NQ):
                for ys in _strassen(al4, quad_wt(r_ref, par * NQ + q, FH)):
                    if ys is not None:
                        for t in range(2):
                            cols = slice((2 * q + t) * 128, (2 * q + t + 1) * 128)
                            b_ref[pl.ds(rb, BLK), cols] = ys[t] + b_ref[pl.ds(rb, BLK), cols]
                    yield
        ups, downs = up_products(), down_products()

        def run(gen, n):
            for _ in range(n):
                next(gen)

        def segment(sg, mem, fillers, inter):
            xs = xn[sg * SEG:(sg + 1) * SEG]
            lhs = sweep_lhs(mem[:, :HK], mem[:, HK:], xs[:, :HK], xs[:, HK:])
            prow = pl.ds(pl.multiple_of((par * 2 + sg) * 8, 8), 8)
            qkv = [None] * NP
            prob = [None] * NP
            ol = [None] * NP
            ph = NP - 3

            def do_qkv(p):
                res = []
                for m in range(3):
                    w0, w1 = m * H + 2 * p, m * H + 2 * p + 1
                    d11 = _dot(lhs[0], wqkv_ref[w0, 0:KH, :])
                    d4 = _dot(lhs[1], wqkv_ref[w0, KH:, :])
                    d3 = _dot(lhs[2], wqkv_ref[w1, 0:KH, :])
                    d22 = _dot(lhs[3], wqkv_ref[w1, KH:, :])
                    pt = px_ref[blk & 1, m * NP + p, 0, prow, :]
                    pb = px_ref[blk & 1, m * NP + p, 1, prow, :]
                    res.append(jnp.concatenate([
                        d11[0:24] + d4[0:24], pt + (d4[24:32] - d22[24:32]), d11[24:32] + d4[24:32],
                        d3[0:24] + d22[0:24], d3[24:32] + d22[24:32], pb + (d3[24:32] - d11[24:32])],
                        axis=0).astype(BF16))
                qkv[p] = res

            def do_qk(p):
                prob[p] = softmax_qk(qkv[p][0], qkv[p][1])

            def do_pv(p):
                o = jnp.dot(prob[p], qkv[p][2], preferred_element_type=F32)
                o1, o2 = o[0:L], o[L:]
                ol[p] = sweep_lhs(o1[0:8], o2[0:8], o1[8:], o2[8:])
                t1, t2, b1, b2 = o1[24:32], o2[24:32], o1[32:40], o2[32:40]
                for k, v in enumerate((t1 + b2, b1 - t1, t2 - b2)):
                    oe_ref[blk & 1, k, prow, p * 128:(p + 1) * 128] = v

            def wo_part(ps, q, acc=None):
                d = []
                for k in range(4):
                    n, o = 2 * q + k // 2, 64 * (k % 2)
                    y = _dot(jnp.concatenate([ol[p][k] for p in ps], axis=1),
                             jnp.concatenate([wo_ref[n, 128 * p + o:128 * p + o + 64, :] for p in ps], axis=0))
                    d.append(y if acc is None else y + acc[k])
                return d

            for p in range(NP):
                do_qkv(p)
                inter(p)
                if p >= 1:
                    do_qk(p - 1)
                if p >= 3:
                    do_pv(p - 3)
            fillers[0]()
            do_qk(NP - 1)
            do_pv(NP - 3)
            do_pv(NP - 2)
            acc = [wo_part(range(ph), q) for q in range(NQ // 2)]
            do_pv(NP - 1)
            fillers[1]()
            acc += [wo_part(range(ph), q) for q in range(NQ // 2, NQ)]
            cols = []
            for q in range(NQ):
                d11, d4, d3, d22 = wo_part(range(ph, NP), q, acc[q])
                cols += [jnp.concatenate([d11[0:24] + d4[0:24], d4[24:32] - d22[24:32], d11[24:32] + d4[24:32]], axis=0),
                         jnp.concatenate([d3[0:24] + d22[0:24], d3[24:32] + d22[24:32], d3[24:32] - d11[24:32]], axis=0)]
            res = jnp.concatenate(cols, axis=1)
            s_ref[j & 3, sg * SEG:(sg + 1) * SEG, :] = res[8:]
            mem_ref[...] = res[0:8]
            fillers[2]()
            return res[0:8]

        U0, U1, IA, IB, D0 = 8, 6, 1, 2, 7

        def inter_a(p):
            if p < NP // 2:
                for m in range(3):
                    qkv_extra((j + 1) >> 1, m * NP + (1 - par) * (NP // 2) + p)
            if p >= IA:
                run(ups, 1)

        def tail_b0():
            combine(rprev, rdst, (j + 1) & 3)
            run(downs, D0)

        def tail_b2():
            for t in range(2):
                wo_extra((j - 1) >> 1, 2 * (1 - par) + t)

        mem = mem_ref[...]
        run(ups, U0)
        mem = segment(0, mem, [lambda: run(ups, U1), lambda: None, lambda: run(ups, 35 - U0 - U1 - (NP - IA))],
                      inter_a)
        segment(1, mem, [tail_b0, lambda: run(downs, 28 - (NP - IB) - D0), tail_b2],
                lambda p: run(downs, 1) if p >= IB else None)

        @pl.when(j >= 3)
        def _():
            out_copy(rprev).start()
        return c
    nst = S // STEP
    lax.fori_loop(0, nst, step, 0)
    for t in range(2):
        wo_extra(nst // 2 - 1, 2 + t)

    def last(j, c):
        r = pl.multiple_of(j * STEP, STEP)
        combine(r, r, j & 3)
        out_copy(r).start()
        return c
    lax.fori_loop(nst - 3, nst, last, 0)
    pltpu.make_async_copy(x_ref.at[pl.ds(0, S)], out_hbm, sems.at[SEM_OUT]).wait()


@functools.partial(jax.jit, static_argnames=("A_seg_len",))
def pallas_recurrent_scan__memory_aug_recurrent_mem_tr__mixer_s_mlp__prompt_kernel(
        A_x, A_mem0, A_Wq, A_Wk, A_Wv, A_Wo, A_seg_len, B_x, B_w1, B_w2, B_w3, B_w4):
    del B_x
    B, S, D = A_x.shape
    _, H, DH = A_Wq.shape
    M = A_mem0.shape[1]
    FF = B_w3.shape[1]
    assert (B, S, D, H, DH, M, A_seg_len, FF) == (1, 2048, 1024, 32, 128, 8, 32, 3584)
    nd, nf = D // 128, FF // 128
    kern = functools.partial(_kernel, S=S, D=D, H=H, DH=DH, M=M, SEG=A_seg_len, FF=FF)
    any_spec = pl.BlockSpec(memory_space=pl.ANY)
    out = pl.pallas_call(
        kern,
        out_shape=jax.ShapeDtypeStruct((S, D), A_x.dtype),
        in_specs=[any_spec] * 10,
        out_specs=any_spec,
        scratch_shapes=[
            pltpu.VMEM((S + STEP, D), BF16),
            pltpu.VMEM((3 * H // 2, D, 128), U32),
            pltpu.VMEM((3 * H, D // 2, 128), U32),
            pltpu.VMEM((nd, H * DH // 2, 128), U32),
            pltpu.VMEM((nd, D // 2, 128), U32),
            pltpu.VMEM((3 * nd // 2, 7 * D // 4, 128), U32),
            pltpu.VMEM(((nf - CPRE) // 2, 7 * D // 4, 128), U32),
            pltpu.VMEM((nd, 7 * (nf - CPRE) * 16, 128), U32),
            pltpu.VMEM((nd, S + 16, 128), F32),
            pltpu.VMEM((S, D), F32),
            pltpu.VMEM((S // BLK, 7, HB // 2, D // 2), U32),
            pltpu.VMEM((HB // 2, D), U32),
            pltpu.VMEM((7, HB // 2, D // 2), U32),
            pltpu.VMEM((4, STEP, D), F32),
            pltpu.VMEM((2, 3 * H // 2, 2, 32, 128), F32),
            pltpu.VMEM((S // BLK, 3, 16, D // 2), U32),
            pltpu.VMEM((2, 3, 32, H * DH // 2), F32),
            pltpu.VMEM((M, D), BF16),
            pltpu.VMEM((M, D), F32),
            pltpu.SemaphoreType.DMA((2 + nd + 4 + 2 * ((S - RB0) // RB1) + S // RB2,)),
        ],
        compiler_params=pltpu.CompilerParams(vmem_limit_bytes=127 * 1024 * 1024,
                                             disable_bounds_checks=True),
    )(A_x[0], A_mem0[0], A_Wq, A_Wk, A_Wv, A_Wo.reshape(H * DH, D), B_w1, B_w2, B_w3, B_w4)
    return out[None]
```

```python
import functools

import jax
import jax.numpy as jnp
from jax import lax
import jax.experimental.pallas as pl
import jax.experimental.pallas.tpu as pltpu

F32 = jnp.float32
BF16 = jnp.bfloat16
U32 = jnp.uint32
EPS = 1e-5
LOG2E = 1.4426950408889634

HB = 64
BLK = 2 * HB
RB0 = 512
RA = 256
RB1 = 256
RB2 = 512
CPRE = 8
STEP = 64
NPRE = 2
W1G = ((0, 2), (2, 5), (5, 8))
XK = 192
CH = 16


def _ln(x):
    m = jnp.mean(x, axis=-1, keepdims=True)
    xc = x - m
    v = jnp.mean(xc * xc, axis=-1, keepdims=True)
    return xc * lax.rsqrt(v + EPS)


def _gelu(x):
    c = 0.7978845608028654
    h = 0.5 * x
    return h + h * jnp.tanh(x * (c + (c * 0.044715) * (x * x)))


def _bf(w_u32):
    return pltpu.bitcast(w_u32, BF16)


def _pk(x):
    return pltpu.bitcast(x.astype(BF16), U32)


def _dot(a, w_u32):
    return jnp.dot(a, _bf(w_u32), preferred_element_type=F32)


def _zero_of(y):
    if y.dtype != U32:
        y = pltpu.bitcast(y[0:(8 if y.dtype == F32 else 16), 0:128], U32)
    return (y[0:8, 0:128] >> 31) >> 1


def _after(y, z):
    return jnp.concatenate([y[0:8] + pltpu.bitcast(z, F32), y[8:]], axis=0)


def _left(get, nk):
    rows, zs = [], []
    for r in range(0, HB, CH):
        cols = []
        for t in range(nk):
            a11, a12, a21, a22 = get(r, t), get(r, nk + t), get(HB + r, t), get(HB + r, nk + t)
            p = [y.astype(BF16) for y in (a11 + a22, a21 + a22, a11, a22, a11 + a12, a21 - a11, a12 - a22)]
            zs.append(_zero_of(functools.reduce(jnp.bitwise_or, [pltpu.bitcast(y, U32) for y in p])))
            cols.append(p)
        rows.append(_cat(cols, 1))
    return _cat(rows, 0), zs


def _cat(parts, axis):
    return [jnp.concatenate([p[t] for p in parts], axis=axis) for t in range(7)]


def _unpack(w):
    return pltpu.bitcast(w << 16, F32), pltpu.bitcast(w & U32(0xFFFF0000), F32)


def _pack2(x, y, sign):
    v = [p + q if sign > 0 else p - q for p, q in zip(x, y)]
    return pltpu.bitcast(pltpu.pack_elementwise(v, packed_dtype=BF16), U32)


def _right_sums(b11, b21, b12, b22):
    b11, b21, b12, b22 = [_unpack(t) for t in (b11, b21, b12, b22)]
    return [_pack2(b21, b11, -1), _pack2(b12, b22, -1), _pack2(b11, b22, 1), _pack2(b11, b12, 1),
            _pack2(b21, b22, 1)]


class _Pace:
    def __init__(self):
        self.items, self.per, self.before = [], 0, []

    def spread(self, items, nslots):
        self.items, self.per, self.credit = list(items), len(items) / nslots, 0.0

    def require(self, zeros, nslots):
        self.before += [None] * (nslots - len(self.before))
        for i, z in enumerate(zeros):
            k = (i + 1) * nslots // len(zeros) - 1
            self.before[k] = z if self.before[k] is None else self.before[k] | z

    def __call__(self, y):
        if self.items:
            self.credit += self.per
            n = min(int(self.credit + 1e-6), len(self.items))
            self.credit -= n
            if n:
                z = _zero_of(y)
                for _ in range(n):
                    self.items.pop(0)(z)
        if self.before:
            z = self.before.pop(0)
            if z is not None:
                y = _after(y, z)
        return y


def _strassen(al, wt, pace=lambda y: y):
    m1 = pace(_dot(al[0], wt(4)))
    yield None
    m4 = pace(_dot(al[3], wt(1)))
    yield None
    m5 = pace(_dot(al[4], wt(3)))
    yield None
    m2 = pace(_dot(al[1], wt(0)))
    yield None
    m3 = pace(_dot(al[2], wt(2)))
    yield None
    c11 = pace(_dot(al[6], wt(6)) + (m1 + m4 - m5))
    yield None
    c22 = pace(_dot(al[5], wt(5)) + (m1 - m2 + m3))
    yield (jnp.concatenate([c11, m2 + m4], axis=0), jnp.concatenate([m3 + m5, c22], axis=0))


def _run(gen):
    for y in gen:
        pass
    return y


def _gelu_left(y0, y1):
    return _left(lambda r, t: _gelu((y0, y1)[t][r:r + CH]), 1)


def _kernel(x_hbm, mem0_hbm, wq_hbm, wk_hbm, wv_hbm, wo_hbm, w1_hbm, w2_hbm, w3_hbm, w4_hbm, out_hbm,
            x_ref, stage, wqkv_ref, wo_ref, w1_ref, q_ref, p_ref, r_ref,
            h_ref, b_ref, a3_ref, pre1_ref, pre_ref, s_ref, px_ref, e_ref, oe_ref, mem0_ref, mem_ref, sems, *, S, D, H, DH, M, SEG, FF):
    L = M + SEG
    R = 2 * L
    NP = H // 2
    ND = D // 128
    NF = FF // 128
    NQ = ND // 2
    KH = D // 4
    FS = (NF - CPRE) // 2
    FH = FS * 32
    HK = D // 2
    N1 = (S - RB0) // RB1
    N2 = S // RB2
    assert CPRE == ND and FS % 2 == 0
    Q_W2, Q_W3A, Q_W4A = 0, NQ, 2 * NQ
    QI = 3 * NQ // N1
    assert QI * N1 == 3 * NQ and N2 == NQ == 4 and FS // 2 - 1 == NQ

    SEM_OUT, SEM_MEM = range(2)
    SEM_W1 = 2
    SEM_X = SEM_W1 + ND
    SEM_Q = SEM_X + 4 + N1
    SEM_G = SEM_Q + N1
    KQ = KH // N2
    JG = NP // N2

    def tile_copy(src, row0, nrows, col, dst, sem):
        cols = pl.ds(pl.multiple_of(col * 128, 128), 128)
        return pltpu.make_async_copy(src.bitcast(U32).at[pl.ds(row0, nrows), cols], dst, sem)

    def quad_copies(src, row0, kh, col, dst_ref, q, sem, dist=1):
        return [tile_copy(src, row0, 2 * kh, col + t * dist, dst_ref.at[q, pl.ds(2 * kh * t, 2 * kh)], sem)
                for t in range(2)]

    def q_copies(q, sem):
        if q < Q_W3A:
            return quad_copies(w2_hbm, 0, KH, 2 * q, q_ref, q, sem)
        if q < Q_W4A:
            return quad_copies(w3_hbm, 0, KH, q - Q_W3A, q_ref, q, sem, CPRE // 2)
        return quad_copies(w4_hbm, 0, KH, 2 * (q - Q_W4A), q_ref, q, sem)

    def x_copy(lo, n, sem):
        return pltpu.make_async_copy(x_hbm.at[pl.ds(lo, n)], x_ref.at[pl.ds(lo, n)], sem)

    def group(i):
        sem = sems.at[SEM_G + i]
        cps = [pltpu.make_async_copy(w.bitcast(U32).at[:, i * JG + k, :], stage.at[m * NP + i * JG + k], sem)
               for m, w in enumerate((wq_hbm, wk_hbm, wv_hbm)) for k in range(JG)]
        for t in range(2):
            rq = 2 * i + t
            par, pair = rq >> 2, rq & 3
            cps += quad_copies(w3_hbm, 0, KH, CPRE + par * FS + 1 + pair, p_ref, rq, sem, FS // 2)
            row0 = pl.multiple_of(CPRE * 64 + par * 2 * FH, 64)
            cps += quad_copies(w4_hbm, row0, FH, 2 * pair, r_ref, rq, sem)
            cps.append(tile_copy(wo_hbm, 0, H * DH // 2, rq, wo_ref.at[rq], sem))
            for sl in range(4):
                r = pl.multiple_of(i * KQ, KQ)
                cps.append(tile_copy(w3_hbm, (sl % 2) * KH + r, KQ, CPRE + t * FS + (sl // 2) * (FS // 2),
                                     p_ref.at[2 * NQ + t, pl.ds(sl * KH + r, KQ)], sem))
        return cps

    g_mem = [pltpu.make_async_copy(mem0_hbm, mem0_ref, sems.at[SEM_MEM])]
    X0 = S - N1 * XK
    assert all(X0 + (k + 1) * XK >= min(RB0 + (k + 1) * RB1 + HB, S) for k in range(N1))
    xch = [(0, RA), (RA, RA + HB), (RA + HB, RB0 + HB), (RB0 + HB, X0)]
    xch += [(X0 + k * XK, X0 + (k + 1) * XK) for k in range(N1)]
    g_x = [x_copy(lo, hi - lo, sems.at[SEM_X + i]) for i, (lo, hi) in enumerate(xch)]
    g_w1 = [tile_copy(w1_hbm, 0, 2 * KH, j, w1_ref.at[j], sems.at[SEM_W1 + j]) for j in range(ND)]
    g_q = [[cp for t in range(QI) for cp in q_copies(QI * k + t, sems.at[SEM_Q + k])] for k in range(N1)]

    def start(*gs):
        for g in gs:
            for cp in g:
                cp.start()

    def wait(*gs):
        for g in gs:
            for cp in g:
                cp.wait()

    start(g_x[0:1], g_w1[0:6], g_x[1:2], g_w1[6:], g_x[2:4])
    for k in range(N1):
        start(g_x[4 + k:5 + k], g_q[k])
    start(g_mem)

    def prep_items(ref, q, kh, r0=0, n=None):
        def item(r, z):
            b = [ref[q, pl.ds(t * kh + r0 + r, 8), :] for t in range(4)]
            for t, y in zip((1, 2, 4, 5, 6), _right_sums(b[0] | z, b[1], b[2], b[3] | z)):
                ref[q, pl.ds(t * kh + r0 + r, 8), :] = y
        return [functools.partial(item, r) for r in range(0, kh if n is None else n, 8)]

    def wos_rows(q, op, v):
        k = (v // 32) * 3 + op
        return (k // JG) * NP + q * JG + k % JG, pl.ds(HK + 16 * (v % 32) + 8, 8)

    def quad_wt(ref, q, kh):
        return lambda i: ref[q, i * kh:(i + 1) * kh, :]

    def load_left(ref):
        return [_bf(ref[t]) for t in range(7)]

    def store_left(ref, al):
        for t in range(7):
            ref[t] = pltpu.bitcast(al[t], U32)

    h_ref[:, 0:8, :] = jnp.zeros((ND, 8, 128), F32)
    h_ref[:, S + 8:S + 16, :] = jnp.zeros((ND, 8, 128), F32)

    def ln2(r):
        xn = _ln(x_ref[pl.ds(r, HB), :].astype(F32))
        b_ref[pl.ds(r, HB), :] = xn
        top = jnp.concatenate([xn[g * SEG + 16:g * SEG + 24] for g in range(HB // SEG)], axis=0)
        bot = jnp.concatenate([xn[g * SEG + 24:g * SEG + 32] for g in range(HB // SEG)], axis=0)
        t1, t2, b1, b2 = top[:, :HK], top[:, HK:], bot[:, :HK], bot[:, HK:]
        rows = pl.ds(pl.multiple_of(((r >> 6) & 1) * 8, 8), 8)
        for k, v in enumerate((t1 + b2, b1 - t1, t2 - b2)):
            e_ref[r >> 7, k, rows, :] = _pk(v)
        return _ln(xn).astype(BF16)

    def shifted_left(r0):
        offs = (7, 9, 6, 10)
        return _left(lambda r, t: _gelu(h_ref[t, pl.ds(r0 + r + offs[4 * t // ND], CH), :]), NQ)

    def p1_rows(base, n, a, pace):
        for s in range(n):
            r = base + s * HB
            nxt = r + HB if s + 1 < n else pl.multiple_of(jnp.minimum(r + HB, S - HB), HB)
            a_n = ln2(nxt)
            for j in range(ND):
                h_ref[j, pl.ds(r + 8, HB), :] = pace(_dot(a, w1_ref[j]))
            a = a_n
        pre1_ref[...] = pltpu.bitcast(a, U32)

    NA = RA // HB
    wait(g_x[0:1])
    a0 = [ln2(s * HB) for s in range(NPRE)]
    for gi, (j0, j1) in enumerate(W1G):
        wait(g_w1[j0:j1])
        if gi == len(W1G) - 1:
            wait(g_x[1:2])
            a_n = ln2(RA)
        for s in range(NA):
            if s == len(a0):
                a0.append(ln2(s * HB))
            for j in range(j0, j1):
                h_ref[j, pl.ds(s * HB + 8, HB), :] = _dot(a0[s], w1_ref[j])
    wait(g_x[2:3])
    al0, zs = shifted_left(0)
    store_left(pre_ref, al0)
    pace = _Pace()
    pace.require(zs, (RB0 - RA) // HB * ND - 2)
    p1_rows(RA, (RB0 - RA) // HB, a_n, pace)
    wait(g_x[3:4])

    def p1(k, c):
        base = pl.multiple_of(RB0 + k * RB1, BLK)
        x_copy(pl.multiple_of(X0 + k * XK, HB), XK, sems.at[SEM_X + 4 + k]).wait()
        landed = q_ref.at[pl.ds(QI * k, QI), pl.ds(0, 4 * KH)]
        pltpu.make_async_copy(landed, landed, sems.at[SEM_Q + k]).wait()

        @pl.when(k == 1)
        def _():
            start(group(0))

        pace = _Pace()
        pace.spread([t_ for t in range(QI) for t_ in prep_items(q_ref, QI * k + t, KH)], RB1 // HB * ND)
        p1_rows(base, RB1 // HB, _bf(pre1_ref[...]), pace)
        assert not pace.items
        return c
    lax.fori_loop(0, N1, p1, 0)

    wait(g_mem)
    mem_ref[...] = mem0_ref[...].astype(F32)

    def qkv_extra(blk, slab):
        def wt(off):
            return jnp.concatenate([stage[slab, off + 16 * i:off + 16 * i + 8, :] for i in range(KH // 8)], axis=0)
        e = [_bf(e_ref[jnp.minimum(blk, S // BLK - 1), k]) for k in range(3)]
        m1 = _dot(e[0], wt(0))
        px_ref[blk & 1, slab, 1] = _dot(e[1], wt(8)) + m1
        px_ref[blk & 1, slab, 0] = _dot(e[2], wt(HK)) + m1

    def p2(it, c):
        base = pl.multiple_of(it * RB2, RB2)
        nb = RB2 // BLK
        g = [None] * nb
        u = [None] * nb
        g[0] = load_left(pre_ref)

        def repack(k, i, z):
            slab = (k // JG) * NP + it * JG + k % JG
            ae, ao, be, bo = [stage[slab, pl.ds(o + i * 16, 8, stride=2), :] for o in (0, 1, HK, HK + 1)]
            ae, be = ae | z, be | z
            hi = U32(0xFFFF0000)
            f = lambda y: pltpu.bitcast(y, F32)
            b11, b12 = (ae << 16, ao << 16), (ae & hi, ao & hi)
            b21, b22 = (be << 16, bo << 16), (be & hi, bo & hi)

            def pk(x, y, sign):
                v = [f(p) + f(q) if sign > 0 else f(p) - f(q) for p, q in zip(x, y)]
                return pltpu.bitcast(pltpu.pack_elementwise(v, packed_dtype=BF16), U32)
            r = pl.ds(i * 8, 8)
            r2 = pl.ds(KH + i * 8, 8)
            wqkv_ref[2 * slab, r, :] = (ae & U32(0xFFFF)) | b11[1]
            wqkv_ref[2 * slab, r2, :] = pk(b21, b11, -1)
            wqkv_ref[2 * slab + 1, r, :] = pk(b12, b22, -1)
            wqkv_ref[2 * slab + 1, r2, :] = (be >> 16) | b22[1]
            stage[slab, pl.ds(i * 16, 8), :] = pk(b11, b22, 1)
            stage[slab, pl.ds(i * 16 + 8, 8), :] = pk(b11, b12, 1)
            stage[slab, pl.ds(HK + i * 16, 8), :] = pk(b21, b22, 1)

        rp = [functools.partial(repack, k, i) for k in range(3 * JG) for i in range(KH // 8)]
        pp = [it_ for t in range(2) for it_ in
              prep_items(p_ref, 2 * it + t, KH) + prep_items(r_ref, 2 * it + t, FH)
              + prep_items(p_ref, 2 * NQ + t, KH, pl.multiple_of(it * KQ, KQ), KQ)]

        def prep_wo(v, z):
            r1, r2 = pl.ds(128 * (v // 8) + 8 * (v % 8), 8), pl.ds(128 * (v // 8) + 64 + 8 * (v % 8), 8)
            s4, s3, *rest = _right_sums(wo_ref[2 * it, r1, :] | z, wo_ref[2 * it, r2, :],
                                        wo_ref[2 * it + 1, r1, :], wo_ref[2 * it + 1, r2, :] | z)
            wo_ref[2 * it, r2, :] = s4
            wo_ref[2 * it + 1, r1, :] = s3
            for op, y in enumerate(rest):
                slab, rows = wos_rows(it, op, v)
                stage[slab, rows, :] = y

        wp = [functools.partial(prep_wo, v) for v in range(128)]
        items = []
        done = 0
        while rp or pp or wp:
            items += rp[:12] + pp[:4 if rp else 2]
            done += len(rp[:12])
            pp = pp[4 if rp else 2:]
            rp = rp[12:]
            n = min(5, done // 96 * 32 - (128 - len(wp)))
            items += wp[:n]
            wp = wp[n:]
        pace = _Pace()
        SL = NQ * 7

        zeros = {}
        carry = {}
        nitems = len(items)

        def make_g(s):
            if s < nb:
                g[s], zeros["g", s] = shifted_left(base + s * BLK)
            else:
                al_n, zeros["g", s] = shifted_left(pl.multiple_of(jnp.minimum(base + RB2, S - BLK), BLK))
                store_left(pre_ref, al_n)

        def next_weights():
            wait(group(it))

            @pl.when(it < N2 - 1)
            def _():
                start(group(it + 1))
            pace.spread(items, 1)

        def mix(s):
            ys = []
            for q in range(NQ):
                ys += _run(_strassen(g[s], quad_wt(q_ref, Q_W2 + q, KH), pace))
            rows = pl.ds(base + s * BLK, BLK)
            x1 = jnp.concatenate(ys, axis=1) + b_ref[rows, :]
            b_ref[rows, :] = x1
            y = [_ln(x1[r:r + CH]) for r in range(0, BLK, CH)]
            al, zeros["a", s] = _left(lambda r, t: y[r // CH][:, t * 128:(t + 1) * 128], NQ)
            store_left(a3_ref.at[it * nb + s], al)

        def up(s):
            al = load_left(a3_ref.at[it * nb + s])
            parts = []
            for q in range(NQ):
                ys = _run(_strassen(al, quad_wt(q_ref, Q_W3A + q, KH), pace))
                if s == 0 and q == NQ - 1:
                    next_weights()
                p, carry[0] = _gelu_left(*ys)
                parts.append(p)
                if q + 1 < NQ:
                    pace.require(carry.pop(0), 7)
            u[s] = _cat(parts, 1)

        def down(s):
            for q in range(NQ):
                ys = _run(_strassen(u[s], quad_wt(q_ref, Q_W4A + q, KH), pace))
                for t in range(2):
                    cols = slice((2 * q + t) * 128, (2 * q + t + 1) * 128)
                    rows = pl.ds(base + s * BLK, BLK)
                    b_ref[rows, cols] = ys[t] + b_ref[rows, cols]

        assert nb == 4
        for s in range(1, nb):
            make_g(s)
        zg = zeros["g", 1] + zeros["g", 2] + zeros["g", 3]
        zeros["g01"], zeros["g12"], zeros["g23"] = zg[:24], zg[24:36], zg[36:]
        plan = [(mix, 0, ["g01"], 0), (mix, 1, [("a", 0), "g12"], 0), (mix, 2, [("a", 1), "g23"], 0),
                (mix, 3, [("a", 2)], 0), (up, 0, [("a", 3)], 0), (up, 1, [], 0.8), (down, 0, [], 1.6),
                (up, 2, [], 0.8), (down, 1, [], 1.6), (up, 3, [], 0.8), (down, 2, [], 1.6),
                (down, 3, [("g", 4)], 1.0)]
        wsum = sum(p[3] for p in plan) - plan[-1][3] * 6 / SL
        for fn, s, keys, w in plan:
            for key in keys:
                if key not in zeros:
                    make_g(key[1])
            zs = carry.pop(0, []) + [z for key in keys for z in zeros[key]]
            if zs:
                pace.require(zs, SL - 1 if keys else 7)
            pace.per = nitems * w / wsum / SL
            fn(s)
        assert not pace.items
        for k in range(6):
            qkv_extra(0, (k % 3) * NP + 2 * it + k // 3)
        return c
    lax.fori_loop(0, N2, p2, 0)

    row = lax.broadcasted_iota(jnp.int32, (R, R), 0)
    col = lax.broadcasted_iota(jnp.int32, (R, R), 1)
    same_head = (row >= L) == (col >= L)
    rr = jnp.where(row >= L, row - L, row)
    cc = jnp.where(col >= L, col - L, col)
    visible = same_head & ((rr < M) | (rr >= cc))
    scale = DH ** -0.5
    fill = jnp.where(same_head, -1e9 / scale, -jnp.inf).astype(F32)

    def softmax_qk(q2, k2):
        s = lax.dot_general(q2, k2, (((1,), (1,)), ((), ())), preferred_element_type=F32)
        s = jnp.where(visible, s, fill)
        m = jnp.max(s, axis=-1, keepdims=True)
        e = jnp.exp2((s - m) * (scale * LOG2E))
        l = jnp.sum(e, axis=-1, keepdims=True)
        r = pl.reciprocal(l, approx=True)
        r = r * (2.0 - l * r)
        return (e * r).astype(BF16)

    def combine(r, rdst, slot):
        b = b_ref[pl.ds(r, STEP), :]
        hb = 0.5 * b
        g = hb + hb * jnp.tanh(hb)
        x = x_ref[pl.ds(r, STEP), :].astype(F32)
        x_ref[pl.ds(rdst, STEP), :] = (x + s_ref[slot] * g).astype(x_ref.dtype)

    def out_copy(r):
        return pltpu.make_async_copy(x_ref.at[pl.ds(r, STEP)], out_hbm.at[pl.ds(r, STEP)], sems.at[SEM_OUT])

    def wo_extra(kb, q):
        def wt(op):
            return jnp.concatenate([stage[wos_rows(q, op, v) + (slice(None),)] for v in range(128)], axis=0)
        e = [oe_ref[kb & 1, k].astype(BF16) for k in range(3)]
        m1 = _dot(e[0], wt(0))
        pb = _dot(e[1], wt(1)) + m1
        pt = _dot(e[2], wt(2)) + m1
        c0 = pl.ds(pl.multiple_of(2 * q * 128, 128), 128)
        c1 = pl.ds(pl.multiple_of((2 * q + 1) * 128, 128), 128)
        for g in range(4):
            slot = (2 * kb + g // 2) & 3
            r = (g % 2) * SEG + 16
            s_ref[slot, r:r + 8, c0] = s_ref[slot, r:r + 8, c0] + pt[8 * g:8 * g + 8]
            s_ref[slot, r + 8:r + 16, c1] = s_ref[slot, r + 8:r + 16, c1] + pb[8 * g:8 * g + 8]

    def sweep_lhs(m1, m2, x1, x2):
        ms, xs = m1 + m2, x1 + x2
        return [jnp.concatenate(v, axis=0).astype(BF16) for v in (
            [ms, xs[0:16], xs[24:32]], [m2, x2[0:16], x2[24:32]],
            [m1, x1[0:16], x1[16:24]], [ms, xs[0:16], xs[16:24]])]

    s_ref[1:4] = jnp.zeros((3,) + s_ref.shape[1:], F32)
    oe_ref[1] = jnp.zeros(oe_ref.shape[1:], F32)

    def step(j, c):
        r0 = pl.multiple_of(j * STEP, STEP)
        par = j & 1
        blk = j >> 1
        rb = pl.multiple_of(blk * BLK, BLK)
        rprev = pl.multiple_of(jnp.maximum(r0 - 3 * STEP, 0), STEP)
        rdst = pl.multiple_of(jnp.where(j >= 3, r0 - 3 * STEP, S), STEP)
        al3 = load_left(a3_ref.at[blk])
        xn = _ln(x_ref[pl.ds(r0, STEP), :].astype(F32))

        parts = []

        def up_products():
            for q in range(FS // 2):
                wt = quad_wt(p_ref, 2 * NQ + par if q == 0 else par * NQ + q - 1, KH)
                for y in _strassen(al3, wt):
                    if y is not None:
                        parts.append(_gelu_left(*y)[0])
                    yield

        def down_products():
            al4 = _cat(parts, 1)
            for q in range(NQ):
                for ys in _strassen(al4, quad_wt(r_ref, par * NQ + q, FH)):
                    if ys is not None:
                        for t in range(2):
                            cols = slice((2 * q + t) * 128, (2 * q + t + 1) * 128)
                            b_ref[pl.ds(rb, BLK), cols] = ys[t] + b_ref[pl.ds(rb, BLK), cols]
                    yield
        ups, downs = up_products(), down_products()

        def run(gen, n):
            for _ in range(n):
                next(gen)

        def segment(sg, mem, fillers, inter):
            xs = xn[sg * SEG:(sg + 1) * SEG]
            lhs = sweep_lhs(mem[:, :HK], mem[:, HK:], xs[:, :HK], xs[:, HK:])
            prow = pl.ds(pl.multiple_of((par * 2 + sg) * 8, 8), 8)
            qkv = [None] * NP
            prob = [None] * NP
            ol = [None] * NP
            ph = NP - 3

            def do_qkv(p):
                res = []
                for m in range(3):
                    w0, w1 = m * H + 2 * p, m * H + 2 * p + 1
                    d11 = _dot(lhs[0], wqkv_ref[w0, 0:KH, :])
                    d4 = _dot(lhs[1], wqkv_ref[w0, KH:, :])
                    d3 = _dot(lhs[2], wqkv_ref[w1, 0:KH, :])
                    d22 = _dot(lhs[3], wqkv_ref[w1, KH:, :])
                    pt = px_ref[blk & 1, m * NP + p, 0, prow, :]
                    pb = px_ref[blk & 1, m * NP + p, 1, prow, :]
                    res.append(jnp.concatenate([
                        d11[0:24] + d4[0:24], pt + (d4[24:32] - d22[24:32]), d11[24:32] + d4[24:32],
                        d3[0:24] + d22[0:24], d3[24:32] + d22[24:32], pb + (d3[24:32] - d11[24:32])],
                        axis=0).astype(BF16))
                qkv[p] = res

            def do_qk(p):
                prob[p] = softmax_qk(qkv[p][0], qkv[p][1])

            def do_pv(p):
                o = jnp.dot(prob[p], qkv[p][2], preferred_element_type=F32)
                o1, o2 = o[0:L], o[L:]
                ol[p] = sweep_lhs(o1[0:8], o2[0:8], o1[8:], o2[8:])
                t1, t2, b1, b2 = o1[24:32], o2[24:32], o1[32:40], o2[32:40]
                for k, v in enumerate((t1 + b2, b1 - t1, t2 - b2)):
                    oe_ref[blk & 1, k, prow, p * 128:(p + 1) * 128] = v

            def wo_part(ps, q, acc=None):
                d = []
                for k in range(4):
                    n, o = 2 * q + k // 2, 64 * (k % 2)
                    y = _dot(jnp.concatenate([ol[p][k] for p in ps], axis=1),
                             jnp.concatenate([wo_ref[n, 128 * p + o:128 * p + o + 64, :] for p in ps], axis=0))
                    d.append(y if acc is None else y + acc[k])
                return d

            for p in range(NP):
                do_qkv(p)
                inter(p)
                if p >= 1:
                    do_qk(p - 1)
                if p >= 3:
                    do_pv(p - 3)
            fillers[0]()
            do_qk(NP - 1)
            do_pv(NP - 3)
            do_pv(NP - 2)
            acc = [wo_part(range(ph), q) for q in range(NQ // 2)]
            do_pv(NP - 1)
            fillers[1]()
            acc += [wo_part(range(ph), q) for q in range(NQ // 2, NQ)]
            cols = []
            for q in range(NQ):
                d11, d4, d3, d22 = wo_part(range(ph, NP), q, acc[q])
                cols += [jnp.concatenate([d11[0:24] + d4[0:24], d4[24:32] - d22[24:32], d11[24:32] + d4[24:32]], axis=0),
                         jnp.concatenate([d3[0:24] + d22[0:24], d3[24:32] + d22[24:32], d3[24:32] - d11[24:32]], axis=0)]
            res = jnp.concatenate(cols, axis=1)
            s_ref[j & 3, sg * SEG:(sg + 1) * SEG, :] = res[8:]
            mem_ref[...] = res[0:8]
            fillers[2]()
            return res[0:8]

        U0, U1, IA, IB, D0 = 8, 6, 1, 2, 7

        def inter_a(p):
            if p < NP // 2:
                for m in range(3):
                    qkv_extra((j + 1) >> 1, m * NP + (1 - par) * (NP // 2) + p)
            if p >= IA:
                run(ups, 1)

        def tail_b0():
            combine(rprev, rdst, (j + 1) & 3)
            run(downs, D0)

        def tail_b2():
            for t in range(2):
                wo_extra((j - 1) >> 1, 2 * (1 - par) + t)

        mem = mem_ref[...]
        run(ups, U0)
        mem = segment(0, mem, [lambda: run(ups, U1), lambda: None, lambda: run(ups, 35 - U0 - U1 - (NP - IA))],
                      inter_a)
        segment(1, mem, [tail_b0, lambda: run(downs, 28 - (NP - IB) - D0), tail_b2],
                lambda p: run(downs, 1) if p >= IB else None)

        @pl.when(j >= 3)
        def _():
            out_copy(rprev).start()
        return c
    nst = S // STEP
    lax.fori_loop(0, nst, step, 0)
    for t in range(2):
        wo_extra(nst // 2 - 1, 2 + t)

    def last(j, c):
        r = pl.multiple_of(j * STEP, STEP)
        combine(r, r, j & 3)
        out_copy(r).start()
        return c
    lax.fori_loop(nst - 3, nst, last, 0)
    pltpu.make_async_copy(x_ref.at[pl.ds(0, S)], out_hbm, sems.at[SEM_OUT]).wait()


@functools.partial(jax.jit, static_argnames=("A_seg_len",))
def pallas_recurrent_scan__memory_aug_recurrent_mem_tr__mixer_s_mlp__prompt_kernel(
        A_x, A_mem0, A_Wq, A_Wk, A_Wv, A_Wo, A_seg_len, B_x, B_w1, B_w2, B_w3, B_w4):
    del B_x
    B, S, D = A_x.shape
    _, H, DH = A_Wq.shape
    M = A_mem0.shape[1]
    FF = B_w3.shape[1]
    assert (B, S, D, H, DH, M, A_seg_len, FF) == (1, 2048, 1024, 32, 128, 8, 32, 3584)
    nd, nf = D // 128, FF // 128
    kern = functools.partial(_kernel, S=S, D=D, H=H, DH=DH, M=M, SEG=A_seg_len, FF=FF)
    any_spec = pl.BlockSpec(memory_space=pl.ANY)
    out = pl.pallas_call(
        kern,
        out_shape=jax.ShapeDtypeStruct((S, D), A_x.dtype),
        in_specs=[any_spec] * 10,
        out_specs=any_spec,
        scratch_shapes=[
            pltpu.VMEM((S + STEP, D), BF16),
            pltpu.VMEM((3 * H // 2, D, 128), U32),
            pltpu.VMEM((3 * H, D // 2, 128), U32),
            pltpu.VMEM((nd, H * DH // 2, 128), U32),
            pltpu.VMEM((nd, D // 2, 128), U32),
            pltpu.VMEM((3 * nd // 2, 7 * D // 4, 128), U32),
            pltpu.VMEM(((nf - CPRE) // 2, 7 * D // 4, 128), U32),
            pltpu.VMEM((nd, 7 * (nf - CPRE) * 16, 128), U32),
            pltpu.VMEM((nd, S + 16, 128), F32),
            pltpu.VMEM((S, D), F32),
            pltpu.VMEM((S // BLK, 7, HB // 2, D // 2), U32),
            pltpu.VMEM((HB // 2, D), U32),
            pltpu.VMEM((7, HB // 2, D // 2), U32),
            pltpu.VMEM((4, STEP, D), F32),
            pltpu.VMEM((2, 3 * H // 2, 2, 32, 128), F32),
            pltpu.VMEM((S // BLK, 3, 16, D // 2), U32),
            pltpu.VMEM((2, 3, 32, H * DH // 2), F32),
            pltpu.VMEM((M, D), BF16),
            pltpu.VMEM((M, D), F32),
            pltpu.SemaphoreType.DMA((2 + nd + 4 + 2 * ((S - RB0) // RB1) + S // RB2,)),
        ],
        compiler_params=pltpu.CompilerParams(vmem_limit_bytes=127 * 1024 * 1024,
                                             disable_bounds_checks=True),
    )(A_x[0], A_mem0[0], A_Wq, A_Wk, A_Wv, A_Wo.reshape(H * DH, D), B_w1, B_w2, B_w3, B_w4)
    return out[None]
```

```python
import functools

import jax
import jax.numpy as jnp
from jax import lax
import jax.experimental.pallas as pl
import jax.experimental.pallas.tpu as pltpu

F32 = jnp.float32
BF16 = jnp.bfloat16
U32 = jnp.uint32
EPS = 1e-5
LOG2E = 1.4426950408889634

HB = 64
BLK = 2 * HB
RB0 = 512
RA = 256
RB1 = 256
RB2 = 512
CPRE = 8
STEP = 64
NPRE = 2
W1G = ((0, 2), (2, 5), (5, 8))
XK = 192
CH = 16


def _ln(x):
    m = jnp.mean(x, axis=-1, keepdims=True)
    xc = x - m
    v = jnp.mean(xc * xc, axis=-1, keepdims=True)
    return xc * lax.rsqrt(v + EPS)


def _gelu(x):
    c = 0.7978845608028654
    h = 0.5 * x
    return h + h * jnp.tanh(x * (c + (c * 0.044715) * (x * x)))


def _bf(w_u32):
    return pltpu.bitcast(w_u32, BF16)


def _pk(x):
    return pltpu.bitcast(x.astype(BF16), U32)


def _dot(a, w_u32):
    return jnp.dot(a, _bf(w_u32), preferred_element_type=F32)


def _zero_of(y):
    if y.dtype != U32:
        y = pltpu.bitcast(y[0:(8 if y.dtype == F32 else 16), 0:128], U32)
    return (y[0:8, 0:128] >> 31) >> 1


def _after(y, z):
    return jnp.concatenate([y[0:8] + pltpu.bitcast(z, F32), y[8:]], axis=0)


def _left(get, nk):
    rows, zs = [], []
    for r in range(0, HB, CH):
        cols = []
        for t in range(nk):
            a11, a12, a21, a22 = get(r, t), get(r, nk + t), get(HB + r, t), get(HB + r, nk + t)
            p = [y.astype(BF16) for y in (a11 + a22, a21 + a22, a11, a22, a11 + a12, a21 - a11, a12 - a22)]
            zs.append(_zero_of(functools.reduce(jnp.bitwise_or, [pltpu.bitcast(y, U32) for y in p])))
            cols.append(p)
        rows.append(_cat(cols, 1))
    return _cat(rows, 0), zs


def _cat(parts, axis):
    return [jnp.concatenate([p[t] for p in parts], axis=axis) for t in range(7)]


def _unpack(w):
    return pltpu.bitcast(w << 16, F32), pltpu.bitcast(w & U32(0xFFFF0000), F32)


def _pack2(x, y, sign):
    e, o = [pltpu.bitcast(p + q if sign > 0 else p - q, U32) for p, q in zip(x, y)]
    return ((e + U32(0x8000)) >> 16) | ((o + U32(0x7FFF)) & U32(0xFFFF0000))


def _right_sums(b11, b21, b12, b22):
    b11, b21, b12, b22 = [_unpack(t) for t in (b11, b21, b12, b22)]
    return [_pack2(b21, b11, -1), _pack2(b12, b22, -1), _pack2(b11, b22, 1), _pack2(b11, b12, 1),
            _pack2(b21, b22, 1)]


class _Pace:
    def __init__(self):
        self.items, self.per, self.before = [], 0, []

    def spread(self, items, nslots):
        self.items, self.per, self.credit = list(items), len(items) / nslots, 0.0

    def require(self, zeros, nslots):
        self.before += [None] * (nslots - len(self.before))
        for i, z in enumerate(zeros):
            k = (i + 1) * nslots // len(zeros) - 1
            self.before[k] = z if self.before[k] is None else self.before[k] | z

    def __call__(self, y):
        if self.items:
            self.credit += self.per
            n = min(int(self.credit + 1e-6), len(self.items))
            self.credit -= n
            if n:
                z = _zero_of(y)
                for _ in range(n):
                    self.items.pop(0)(z)
        if self.before:
            z = self.before.pop(0)
            if z is not None:
                y = _after(y, z)
        return y


def _strassen(al, wt, pace=lambda y: y):
    m1 = pace(_dot(al[0], wt(4)))
    yield None
    m4 = pace(_dot(al[3], wt(1)))
    yield None
    m5 = pace(_dot(al[4], wt(3)))
    yield None
    m2 = pace(_dot(al[1], wt(0)))
    yield None
    m3 = pace(_dot(al[2], wt(2)))
    yield None
    c11 = pace(_dot(al[6], wt(6)) + (m1 + m4 - m5))
    yield None
    c22 = pace(_dot(al[5], wt(5)) + (m1 - m2 + m3))
    yield (jnp.concatenate([c11, m2 + m4], axis=0), jnp.concatenate([m3 + m5, c22], axis=0))


def _run(gen):
    for y in gen:
        pass
    return y


def _gelu_left(y0, y1):
    return _left(lambda r, t: _gelu((y0, y1)[t][r:r + CH]), 1)


def _kernel(x_hbm, mem0_hbm, wq_hbm, wk_hbm, wv_hbm, wo_hbm, w1_hbm, w2_hbm, w3_hbm, w4_hbm, out_hbm,
            x_ref, stage, wqkv_ref, wo_ref, w1_ref, q_ref, p_ref, r_ref,
            h_ref, b_ref, a3_ref, pre1_ref, pre_ref, s_ref, px_ref, e_ref, oe_ref, mem0_ref, mem_ref, sems, *, S, D, H, DH, M, SEG, FF):
    L = M + SEG
    R = 2 * L
    NP = H // 2
    ND = D // 128
    NF = FF // 128
    NQ = ND // 2
    KH = D // 4
    FS = (NF - CPRE) // 2
    FH = FS * 32
    HK = D // 2
    N1 = (S - RB0) // RB1
    N2 = S // RB2
    assert CPRE == ND and FS % 2 == 0
    Q_W2, Q_W3A, Q_W4A = 0, NQ, 2 * NQ
    QI = 3 * NQ // N1
    assert QI * N1 == 3 * NQ and N2 == NQ == 4 and FS // 2 - 1 == NQ

    SEM_OUT, SEM_MEM = range(2)
    SEM_W1 = 2
    SEM_X = SEM_W1 + ND
    SEM_Q = SEM_X + 4 + N1
    SEM_G = SEM_Q + N1
    KQ = KH // N2
    JG = NP // N2

    def tile_copy(src, row0, nrows, col, dst, sem):
        cols = pl.ds(pl.multiple_of(col * 128, 128), 128)
        return pltpu.make_async_copy(src.bitcast(U32).at[pl.ds(row0, nrows), cols], dst, sem)

    def quad_copies(src, row0, kh, col, dst_ref, q, sem, dist=1):
        return [tile_copy(src, row0, 2 * kh, col + t * dist, dst_ref.at[q, pl.ds(2 * kh * t, 2 * kh)], sem)
                for t in range(2)]

    def q_copies(q, sem):
        if q < Q_W3A:
            return quad_copies(w2_hbm, 0, KH, 2 * q, q_ref, q, sem)
        if q < Q_W4A:
            return quad_copies(w3_hbm, 0, KH, q - Q_W3A, q_ref, q, sem, CPRE // 2)
        return quad_copies(w4_hbm, 0, KH, 2 * (q - Q_W4A), q_ref, q, sem)

    def x_copy(lo, n, sem):
        return pltpu.make_async_copy(x_hbm.at[pl.ds(lo, n)], x_ref.at[pl.ds(lo, n)], sem)

    def group(i):
        sem = sems.at[SEM_G + i]
        cps = [pltpu.make_async_copy(w.bitcast(U32).at[:, i * JG + k, :], stage.at[m * NP + i * JG + k], sem)
               for m, w in enumerate((wq_hbm, wk_hbm, wv_hbm)) for k in range(JG)]
        for t in range(2):
            rq = 2 * i + t
            par, pair = rq >> 2, rq & 3
            cps += quad_copies(w3_hbm, 0, KH, CPRE + par * FS + 1 + pair, p_ref, rq, sem, FS // 2)
            row0 = pl.multiple_of(CPRE * 64 + par * 2 * FH, 64)
            cps += quad_copies(w4_hbm, row0, FH, 2 * pair, r_ref, rq, sem)
            cps.append(tile_copy(wo_hbm, 0, H * DH // 2, rq, wo_ref.at[rq], sem))
            for sl in range(4):
                r = pl.multiple_of(i * KQ, KQ)
                cps.append(tile_copy(w3_hbm, (sl % 2) * KH + r, KQ, CPRE + t * FS + (sl // 2) * (FS // 2),
                                     p_ref.at[2 * NQ + t, pl.ds(sl * KH + r, KQ)], sem))
        return cps

    g_mem = [pltpu.make_async_copy(mem0_hbm, mem0_ref, sems.at[SEM_MEM])]
    X0 = S - N1 * XK
    assert all(X0 + (k + 1) * XK >= min(RB0 + (k + 1) * RB1 + HB, S) for k in range(N1))
    xch = [(0, RA), (RA, RA + HB), (RA + HB, RB0 + HB), (RB0 + HB, X0)]
    xch += [(X0 + k * XK, X0 + (k + 1) * XK) for k in range(N1)]
    g_x = [x_copy(lo, hi - lo, sems.at[SEM_X + i]) for i, (lo, hi) in enumerate(xch)]
    g_w1 = [tile_copy(w1_hbm, 0, 2 * KH, j, w1_ref.at[j], sems.at[SEM_W1 + j]) for j in range(ND)]
    g_q = [[cp for t in range(QI) for cp in q_copies(QI * k + t, sems.at[SEM_Q + k])] for k in range(N1)]

    def start(*gs):
        for g in gs:
            for cp in g:
                cp.start()

    def wait(*gs):
        for g in gs:
            for cp in g:
                cp.wait()

    start(g_x[0:1], g_w1[0:6], g_x[1:2], g_w1[6:], g_x[2:4])
    for k in range(N1):
        start(g_x[4 + k:5 + k], g_q[k])
    start(g_mem)

    def prep_items(ref, q, kh, r0=0, n=None):
        def item(r, z):
            b = [ref[q, pl.ds(t * kh + r0 + r, 8), :] for t in range(4)]
            for t, y in zip((1, 2, 4, 5, 6), _right_sums(b[0] | z, b[1], b[2], b[3] | z)):
                ref[q, pl.ds(t * kh + r0 + r, 8), :] = y
        return [functools.partial(item, r) for r in range(0, kh if n is None else n, 8)]

    def wos_rows(q, op, v):
        k = (v // 32) * 3 + op
        return (k // JG) * NP + q * JG + k % JG, pl.ds(HK + 16 * (v % 32) + 8, 8)

    def quad_wt(ref, q, kh):
        return lambda i: ref[q, i * kh:(i + 1) * kh, :]

    def load_left(ref):
        return [_bf(ref[t]) for t in range(7)]

    def store_left(ref, al):
        for t in range(7):
            ref[t] = pltpu.bitcast(al[t], U32)

    h_ref[:, 0:8, :] = jnp.zeros((ND, 8, 128), F32)
    h_ref[:, S + 8:S + 16, :] = jnp.zeros((ND, 8, 128), F32)

    def ln2(r):
        xn = _ln(x_ref[pl.ds(r, HB), :].astype(F32))
        b_ref[pl.ds(r, HB), :] = xn
        top = jnp.concatenate([xn[g * SEG + 16:g * SEG + 24] for g in range(HB // SEG)], axis=0)
        bot = jnp.concatenate([xn[g * SEG + 24:g * SEG + 32] for g in range(HB // SEG)], axis=0)
        t1, t2, b1, b2 = top[:, :HK], top[:, HK:], bot[:, :HK], bot[:, HK:]
        rows = pl.ds(pl.multiple_of(((r >> 6) & 1) * 8, 8), 8)
        for k, v in enumerate((t1 + b2, b1 - t1, t2 - b2)):
            e_ref[r >> 7, k, rows, :] = _pk(v)
        return _ln(xn).astype(BF16)

    def shifted_left(r0):
        offs = (7, 9, 6, 10)
        return _left(lambda r, t: _gelu(h_ref[t, pl.ds(r0 + r + offs[4 * t // ND], CH), :]), NQ)

    def p1_rows(base, n, a, pace):
        for s in range(n):
            r = base + s * HB
            nxt = r + HB if s + 1 < n else pl.multiple_of(jnp.minimum(r + HB, S - HB), HB)
            a_n = ln2(nxt)
            for j in range(ND):
                h_ref[j, pl.ds(r + 8, HB), :] = pace(_dot(a, w1_ref[j]))
            a = a_n
        pre1_ref[...] = pltpu.bitcast(a, U32)

    NA = RA // HB
    wait(g_x[0:1])
    a0 = [ln2(s * HB) for s in range(NPRE)]
    for gi, (j0, j1) in enumerate(W1G):
        wait(g_w1[j0:j1])
        if gi == len(W1G) - 1:
            wait(g_x[1:2])
            a_n = ln2(RA)
        for s in range(NA):
            if s == len(a0):
                a0.append(ln2(s * HB))
            for j in range(j0, j1):
                h_ref[j, pl.ds(s * HB + 8, HB), :] = _dot(a0[s], w1_ref[j])
    wait(g_x[2:3])
    al0, zs = shifted_left(0)
    store_left(pre_ref, al0)
    pace = _Pace()
    pace.require(zs, (RB0 - RA) // HB * ND - 2)
    p1_rows(RA, (RB0 - RA) // HB, a_n, pace)
    wait(g_x[3:4])

    def p1(k, c):
        base = pl.multiple_of(RB0 + k * RB1, BLK)
        x_copy(pl.multiple_of(X0 + k * XK, HB), XK, sems.at[SEM_X + 4 + k]).wait()
        landed = q_ref.at[pl.ds(QI * k, QI), pl.ds(0, 4 * KH)]
        pltpu.make_async_copy(landed, landed, sems.at[SEM_Q + k]).wait()

        @pl.when(k == 1)
        def _():
            start(group(0))

        pace = _Pace()
        pace.spread([t_ for t in range(QI) for t_ in prep_items(q_ref, QI * k + t, KH)], RB1 // HB * ND)
        p1_rows(base, RB1 // HB, _bf(pre1_ref[...]), pace)
        assert not pace.items
        return c
    lax.fori_loop(0, N1, p1, 0)

    wait(g_mem)
    mem_ref[...] = mem0_ref[...].astype(F32)

    def qkv_extra(blk, slab):
        def wt(off):
            return jnp.concatenate([stage[slab, off + 16 * i:off + 16 * i + 8, :] for i in range(KH // 8)], axis=0)
        e = [_bf(e_ref[jnp.minimum(blk, S // BLK - 1), k]) for k in range(3)]
        m1 = _dot(e[0], wt(0))
        px_ref[blk & 1, slab, 1] = _dot(e[1], wt(8)) + m1
        px_ref[blk & 1, slab, 0] = _dot(e[2], wt(HK)) + m1

    def p2(it, c):
        base = pl.multiple_of(it * RB2, RB2)
        nb = RB2 // BLK
        g = [None] * nb
        u = [None] * nb
        g[0] = load_left(pre_ref)

        def repack(k, i, z):
            slab = (k // JG) * NP + it * JG + k % JG
            ae, ao, be, bo = [stage[slab, pl.ds(o + i * 16, 8, stride=2), :] for o in (0, 1, HK, HK + 1)]
            ae, be = ae | z, be | z
            (b11, b12), (b21, b22) = zip(_unpack(ae), _unpack(ao)), zip(_unpack(be), _unpack(bo))
            r, r2 = pl.ds(i * 8, 8), pl.ds(KH + i * 8, 8)
            wqkv_ref[2 * slab, r, :] = (ae & U32(0xFFFF)) | (ao << 16)
            wqkv_ref[2 * slab, r2, :] = _pack2(b21, b11, -1)
            wqkv_ref[2 * slab + 1, r, :] = _pack2(b12, b22, -1)
            wqkv_ref[2 * slab + 1, r2, :] = (be >> 16) | (bo & U32(0xFFFF0000))
            stage[slab, pl.ds(i * 16, 8), :] = _pack2(b11, b22, 1)
            stage[slab, pl.ds(i * 16 + 8, 8), :] = _pack2(b11, b12, 1)
            stage[slab, pl.ds(HK + i * 16, 8), :] = _pack2(b21, b22, 1)

        rp = [functools.partial(repack, k, i) for k in range(3 * JG) for i in range(KH // 8)]
        pp = [it_ for t in range(2) for it_ in
              prep_items(p_ref, 2 * it + t, KH) + prep_items(r_ref, 2 * it + t, FH)
              + prep_items(p_ref, 2 * NQ + t, KH, pl.multiple_of(it * KQ, KQ), KQ)]

        def prep_wo(v, z):
            r1, r2 = pl.ds(128 * (v // 8) + 8 * (v % 8), 8), pl.ds(128 * (v // 8) + 64 + 8 * (v % 8), 8)
            s4, s3, *rest = _right_sums(wo_ref[2 * it, r1, :] | z, wo_ref[2 * it, r2, :],
                                        wo_ref[2 * it + 1, r1, :], wo_ref[2 * it + 1, r2, :] | z)
            wo_ref[2 * it, r2, :] = s4
            wo_ref[2 * it + 1, r1, :] = s3
            for op, y in enumerate(rest):
                slab, rows = wos_rows(it, op, v)
                stage[slab, rows, :] = y

        wp = [functools.partial(prep_wo, v) for v in range(128)]
        items = []
        done = 0
        while rp or pp or wp:
            items += rp[:12] + pp[:4 if rp else 2]
            done += len(rp[:12])
            pp = pp[4 if rp else 2:]
            rp = rp[12:]
            n = min(5, done // 96 * 32 - (128 - len(wp)))
            items += wp[:n]
            wp = wp[n:]
        pace = _Pace()
        SL = NQ * 7

        zeros = {}
        carry = {}
        nitems = len(items)

        def make_g(s):
            if s < nb:
                g[s], zeros["g", s] = shifted_left(base + s * BLK)
            else:
                al_n, zeros["g", s] = shifted_left(pl.multiple_of(jnp.minimum(base + RB2, S - BLK), BLK))
                store_left(pre_ref, al_n)

        def next_weights():
            wait(group(it))

            @pl.when(it < N2 - 1)
            def _():
                start(group(it + 1))
            pace.spread(items, 1)

        def mix(s):
            ys = []
            for q in range(NQ):
                ys += _run(_strassen(g[s], quad_wt(q_ref, Q_W2 + q, KH), pace))
            rows = pl.ds(base + s * BLK, BLK)
            x1 = jnp.concatenate(ys, axis=1) + b_ref[rows, :]
            b_ref[rows, :] = x1
            y = [_ln(x1[r:r + CH]) for r in range(0, BLK, CH)]
            al, zeros["a", s] = _left(lambda r, t: y[r // CH][:, t * 128:(t + 1) * 128], NQ)
            store_left(a3_ref.at[it * nb + s], al)

        def up(s):
            al = load_left(a3_ref.at[it * nb + s])
            parts = []
            for q in range(NQ):
                ys = _run(_strassen(al, quad_wt(q_ref, Q_W3A + q, KH), pace))
                if s == 0 and q == NQ - 1:
                    next_weights()
                p, carry[0] = _gelu_left(*ys)
                parts.append(p)
                if q + 1 < NQ:
                    pace.require(carry.pop(0), 7)
            u[s] = _cat(parts, 1)

        def down(s):
            for q in range(NQ):
                ys = _run(_strassen(u[s], quad_wt(q_ref, Q_W4A + q, KH), pace))
                for t in range(2):
                    cols = slice((2 * q + t) * 128, (2 * q + t + 1) * 128)
                    rows = pl.ds(base + s * BLK, BLK)
                    b_ref[rows, cols] = ys[t] + b_ref[rows, cols]

        assert nb == 4
        for s in range(1, nb):
            make_g(s)
        zg = zeros["g", 1] + zeros["g", 2] + zeros["g", 3]
        zeros["g01"], zeros["g12"], zeros["g23"] = zg[:24], zg[24:36], zg[36:]
        plan = [(mix, 0, ["g01"], 0), (mix, 1, [("a", 0), "g12"], 0), (mix, 2, [("a", 1), "g23"], 0),
                (mix, 3, [("a", 2)], 0), (up, 0, [("a", 3)], 0), (up, 1, [], 0.8), (down, 0, [], 1.6),
                (up, 2, [], 0.8), (down, 1, [], 1.6), (up, 3, [], 0.8), (down, 2, [], 1.6),
                (down, 3, [("g", 4)], 1.0)]
        wsum = sum(p[3] for p in plan) - plan[-1][3] * 6 / SL
        for fn, s, keys, w in plan:
            for key in keys:
                if key not in zeros:
                    make_g(key[1])
            zs = carry.pop(0, []) + [z for key in keys for z in zeros[key]]
            if zs:
                pace.require(zs, SL - 1 if keys else 7)
            pace.per = nitems * w / wsum / SL
            fn(s)
        assert not pace.items
        for k in range(6):
            qkv_extra(0, (k % 3) * NP + 2 * it + k // 3)
        return c
    lax.fori_loop(0, N2, p2, 0)

    row = lax.broadcasted_iota(jnp.int32, (R, R), 0)
    col = lax.broadcasted_iota(jnp.int32, (R, R), 1)
    same_head = (row >= L) == (col >= L)
    rr = jnp.where(row >= L, row - L, row)
    cc = jnp.where(col >= L, col - L, col)
    visible = same_head & ((rr < M) | (rr >= cc))
    scale = DH ** -0.5
    fill = jnp.where(same_head, -1e9 / scale, -jnp.inf).astype(F32)

    def softmax_qk(q2, k2):
        s = lax.dot_general(q2, k2, (((1,), (1,)), ((), ())), preferred_element_type=F32)
        s = jnp.where(visible, s, fill)
        m = jnp.max(s, axis=-1, keepdims=True)
        e = jnp.exp2((s - m) * (scale * LOG2E))
        l = jnp.sum(e, axis=-1, keepdims=True)
        r = pl.reciprocal(l, approx=True)
        r = r * (2.0 - l * r)
        return (e * r).astype(BF16)

    def combine(r, rdst, slot):
        b = b_ref[pl.ds(r, STEP), :]
        hb = 0.5 * b
        g = hb + hb * jnp.tanh(hb)
        x = x_ref[pl.ds(r, STEP), :].astype(F32)
        x_ref[pl.ds(rdst, STEP), :] = (x + s_ref[slot] * g).astype(x_ref.dtype)

    def out_copy(r):
        return pltpu.make_async_copy(x_ref.at[pl.ds(r, STEP)], out_hbm.at[pl.ds(r, STEP)], sems.at[SEM_OUT])

    def wo_extra(kb, q):
        def wt(op):
            return jnp.concatenate([stage[wos_rows(q, op, v) + (slice(None),)] for v in range(128)], axis=0)
        e = [oe_ref[kb & 1, k].astype(BF16) for k in range(3)]
        m1 = _dot(e[0], wt(0))
        pb = _dot(e[1], wt(1)) + m1
        pt = _dot(e[2], wt(2)) + m1
        c0 = pl.ds(pl.multiple_of(2 * q * 128, 128), 128)
        c1 = pl.ds(pl.multiple_of((2 * q + 1) * 128, 128), 128)
        for g in range(4):
            slot = (2 * kb + g // 2) & 3
            r = (g % 2) * SEG + 16
            s_ref[slot, r:r + 8, c0] = s_ref[slot, r:r + 8, c0] + pt[8 * g:8 * g + 8]
            s_ref[slot, r + 8:r + 16, c1] = s_ref[slot, r + 8:r + 16, c1] + pb[8 * g:8 * g + 8]

    def sweep_lhs(m1, m2, x1, x2):
        ms, xs = m1 + m2, x1 + x2
        return [jnp.concatenate(v, axis=0).astype(BF16) for v in (
            [ms, xs[0:16], xs[24:32]], [m2, x2[0:16], x2[24:32]],
            [m1, x1[0:16], x1[16:24]], [ms, xs[0:16], xs[16:24]])]

    s_ref[1:4] = jnp.zeros((3,) + s_ref.shape[1:], F32)
    oe_ref[1] = jnp.zeros(oe_ref.shape[1:], F32)

    def step(j, c):
        r0 = pl.multiple_of(j * STEP, STEP)
        par = j & 1
        blk = j >> 1
        rb = pl.multiple_of(blk * BLK, BLK)
        rprev = pl.multiple_of(jnp.maximum(r0 - 3 * STEP, 0), STEP)
        rdst = pl.multiple_of(jnp.where(j >= 3, r0 - 3 * STEP, S), STEP)
        al3 = load_left(a3_ref.at[blk])
        xn = _ln(x_ref[pl.ds(r0, STEP), :].astype(F32))

        parts = []

        def up_products():
            for q in range(FS // 2):
                wt = quad_wt(p_ref, 2 * NQ + par if q == 0 else par * NQ + q - 1, KH)
                for y in _strassen(al3, wt):
                    if y is not None:
                        parts.append(_gelu_left(*y)[0])
                    yield

        def down_products():
            al4 = _cat(parts, 1)
            for q in range(NQ):
                for ys in _strassen(al4, quad_wt(r_ref, par * NQ + q, FH)):
                    if ys is not None:
                        for t in range(2):
                            cols = slice((2 * q + t) * 128, (2 * q + t + 1) * 128)
                            b_ref[pl.ds(rb, BLK), cols] = ys[t] + b_ref[pl.ds(rb, BLK), cols]
                    yield
        ups, downs = up_products(), down_products()

        def run(gen, n):
            for _ in range(n):
                next(gen)

        def segment(sg, mem, fillers, inter):
            xs = xn[sg * SEG:(sg + 1) * SEG]
            lhs = sweep_lhs(mem[:, :HK], mem[:, HK:], xs[:, :HK], xs[:, HK:])
            prow = pl.ds(pl.multiple_of((par * 2 + sg) * 8, 8), 8)
            qkv = [None] * NP
            prob = [None] * NP
            ol = [None] * NP
            ph = NP - 3

            def do_qkv(p):
                res = []
                for m in range(3):
                    w0, w1 = m * H + 2 * p, m * H + 2 * p + 1
                    d11 = _dot(lhs[0], wqkv_ref[w0, 0:KH, :])
                    d4 = _dot(lhs[1], wqkv_ref[w0, KH:, :])
                    d3 = _dot(lhs[2], wqkv_ref[w1, 0:KH, :])
                    d22 = _dot(lhs[3], wqkv_ref[w1, KH:, :])
                    pt = px_ref[blk & 1, m * NP + p, 0, prow, :]
                    pb = px_ref[blk & 1, m * NP + p, 1, prow, :]
                    res.append(jnp.concatenate([
                        d11[0:24] + d4[0:24], pt + (d4[24:32] - d22[24:32]), d11[24:32] + d4[24:32],
                        d3[0:24] + d22[0:24], d3[24:32] + d22[24:32], pb + (d3[24:32] - d11[24:32])],
                        axis=0).astype(BF16))
                qkv[p] = res

            def do_qk(p):
                prob[p] = softmax_qk(qkv[p][0], qkv[p][1])

            def do_pv(p):
                o = jnp.dot(prob[p], qkv[p][2], preferred_element_type=F32)
                o1, o2 = o[0:L], o[L:]
                ol[p] = sweep_lhs(o1[0:8], o2[0:8], o1[8:], o2[8:])
                t1, t2, b1, b2 = o1[24:32], o2[24:32], o1[32:40], o2[32:40]
                for k, v in enumerate((t1 + b2, b1 - t1, t2 - b2)):
                    oe_ref[blk & 1, k, prow, p * 128:(p + 1) * 128] = v

            def wo_part(ps, q, acc=None):
                d = []
                for k in range(4):
                    n, o = 2 * q + k // 2, 64 * (k % 2)
                    y = _dot(jnp.concatenate([ol[p][k] for p in ps], axis=1),
                             jnp.concatenate([wo_ref[n, 128 * p + o:128 * p + o + 64, :] for p in ps], axis=0))
                    d.append(y if acc is None else y + acc[k])
                return d

            for p in range(NP):
                do_qkv(p)
                inter(p)
                if p >= 1:
                    do_qk(p - 1)
                if p >= 3:
                    do_pv(p - 3)
            fillers[0]()
            do_qk(NP - 1)
            do_pv(NP - 3)
            do_pv(NP - 2)
            acc = [wo_part(range(ph), q) for q in range(NQ // 2)]
            do_pv(NP - 1)
            fillers[1]()
            acc += [wo_part(range(ph), q) for q in range(NQ // 2, NQ)]
            cols = []
            for q in range(NQ):
                d11, d4, d3, d22 = wo_part(range(ph, NP), q, acc[q])
                cols += [jnp.concatenate([d11[0:24] + d4[0:24], d4[24:32] - d22[24:32], d11[24:32] + d4[24:32]], axis=0),
                         jnp.concatenate([d3[0:24] + d22[0:24], d3[24:32] + d22[24:32], d3[24:32] - d11[24:32]], axis=0)]
            res = jnp.concatenate(cols, axis=1)
            s_ref[j & 3, sg * SEG:(sg + 1) * SEG, :] = res[8:]
            mem_ref[...] = res[0:8]
            fillers[2]()
            return res[0:8]

        U0, U1, IA, IB, D0 = 8, 6, 1, 2, 7

        def inter_a(p):
            if p < NP // 2:
                for m in range(3):
                    qkv_extra((j + 1) >> 1, m * NP + (1 - par) * (NP // 2) + p)
            if p >= IA:
                run(ups, 1)

        def tail_b0():
            combine(rprev, rdst, (j + 1) & 3)
            run(downs, D0)

        def tail_b2():
            for t in range(2):
                wo_extra((j - 1) >> 1, 2 * (1 - par) + t)

        mem = mem_ref[...]
        run(ups, U0)
        mem = segment(0, mem, [lambda: run(ups, U1), lambda: None, lambda: run(ups, 35 - U0 - U1 - (NP - IA))],
                      inter_a)
        segment(1, mem, [tail_b0, lambda: run(downs, 28 - (NP - IB) - D0), tail_b2],
                lambda p: run(downs, 1) if p >= IB else None)

        @pl.when(j >= 3)
        def _():
            out_copy(rprev).start()
        return c
    nst = S // STEP
    lax.fori_loop(0, nst, step, 0)
    for t in range(2):
        wo_extra(nst // 2 - 1, 2 + t)

    def last(j, c):
        r = pl.multiple_of(j * STEP, STEP)
        combine(r, r, j & 3)
        out_copy(r).start()
        return c
    lax.fori_loop(nst - 3, nst, last, 0)
    pltpu.make_async_copy(x_ref.at[pl.ds(0, S)], out_hbm, sems.at[SEM_OUT]).wait()


@functools.partial(jax.jit, static_argnames=("A_seg_len",))
def pallas_recurrent_scan__memory_aug_recurrent_mem_tr__mixer_s_mlp__prompt_kernel(
        A_x, A_mem0, A_Wq, A_Wk, A_Wv, A_Wo, A_seg_len, B_x, B_w1, B_w2, B_w3, B_w4):
    del B_x
    B, S, D = A_x.shape
    _, H, DH = A_Wq.shape
    M = A_mem0.shape[1]
    FF = B_w3.shape[1]
    assert (B, S, D, H, DH, M, A_seg_len, FF) == (1, 2048, 1024, 32, 128, 8, 32, 3584)
    nd, nf = D // 128, FF // 128
    kern = functools.partial(_kernel, S=S, D=D, H=H, DH=DH, M=M, SEG=A_seg_len, FF=FF)
    any_spec = pl.BlockSpec(memory_space=pl.ANY)
    out = pl.pallas_call(
        kern,
        out_shape=jax.ShapeDtypeStruct((S, D), A_x.dtype),
        in_specs=[any_spec] * 10,
        out_specs=any_spec,
        scratch_shapes=[
            pltpu.VMEM((S + STEP, D), BF16),
            pltpu.VMEM((3 * H // 2, D, 128), U32),
            pltpu.VMEM((3 * H, D // 2, 128), U32),
            pltpu.VMEM((nd, H * DH // 2, 128), U32),
            pltpu.VMEM((nd, D // 2, 128), U32),
            pltpu.VMEM((3 * nd // 2, 7 * D // 4, 128), U32),
            pltpu.VMEM(((nf - CPRE) // 2, 7 * D // 4, 128), U32),
            pltpu.VMEM((nd, 7 * (nf - CPRE) * 16, 128), U32),
            pltpu.VMEM((nd, S + 16, 128), F32),
            pltpu.VMEM((S, D), F32),
            pltpu.VMEM((S // BLK, 7, HB // 2, D // 2), U32),
            pltpu.VMEM((HB // 2, D), U32),
            pltpu.VMEM((7, HB // 2, D // 2), U32),
            pltpu.VMEM((4, STEP, D), F32),
            pltpu.VMEM((2, 3 * H // 2, 2, 32, 128), F32),
            pltpu.VMEM((S // BLK, 3, 16, D // 2), U32),
            pltpu.VMEM((2, 3, 32, H * DH // 2), F32),
            pltpu.VMEM((M, D), BF16),
            pltpu.VMEM((M, D), F32),
            pltpu.SemaphoreType.DMA((2 + nd + 4 + 2 * ((S - RB0) // RB1) + S // RB2,)),
        ],
        compiler_params=pltpu.CompilerParams(vmem_limit_bytes=127 * 1024 * 1024,
                                             disable_bounds_checks=True),
    )(A_x[0], A_mem0[0], A_Wq, A_Wk, A_Wv, A_Wo.reshape(H * DH, D), B_w1, B_w2, B_w3, B_w4)
    return out[None]
```

```python
import functools

import jax
import jax.numpy as jnp
from jax import lax
import jax.experimental.pallas as pl
import jax.experimental.pallas.tpu as pltpu

F32 = jnp.float32
BF16 = jnp.bfloat16
U32 = jnp.uint32
EPS = 1e-5
LOG2E = 1.4426950408889634

HB = 64
BLK = 2 * HB
RB0 = 512
RA = 256
RB1 = 256
RB2 = 512
CPRE = 8
STEP = 64
NPRE = 2
W1G = ((0, 2), (2, 5), (5, 8))
XK = 192
CH = 16


def _ln(x):
    m = jnp.mean(x, axis=-1, keepdims=True)
    xc = x - m
    v = jnp.mean(xc * xc, axis=-1, keepdims=True)
    return xc * lax.rsqrt(v + EPS)


def _gelu(x):
    c = 0.7978845608028654
    h = 0.5 * x
    return h + h * jnp.tanh(x * (c + (c * 0.044715) * (x * x)))


def _bf(w_u32):
    return pltpu.bitcast(w_u32, BF16)


def _pk(x):
    return pltpu.bitcast(x.astype(BF16), U32)


def _dot(a, w_u32):
    return jnp.dot(a, _bf(w_u32), preferred_element_type=F32)


def _zero_of(y):
    if y.dtype != U32:
        y = pltpu.bitcast(y[0:(8 if y.dtype == F32 else 16), 0:128], U32)
    return (y[0:8, 0:128] >> 31) >> 1


def _after(y, z):
    return jnp.concatenate([y[0:8] + pltpu.bitcast(z, F32), y[8:]], axis=0)


def _left(get, nk):
    rows, zs = [], []
    for r in range(0, HB, CH):
        cols = []
        for t in range(nk):
            a11, a12, a21, a22 = get(r, t), get(r, nk + t), get(HB + r, t), get(HB + r, nk + t)
            p = [y.astype(BF16) for y in (a11 + a22, a21 + a22, a11, a22, a11 + a12, a21 - a11, a12 - a22)]
            zs.append(_zero_of(functools.reduce(jnp.bitwise_or, [pltpu.bitcast(y, U32) for y in p])))
            cols.append(p)
        rows.append(_cat(cols, 1))
    return _cat(rows, 0), zs


def _cat(parts, axis):
    return [jnp.concatenate([p[t] for p in parts], axis=axis) for t in range(7)]


def _unpack(w):
    return pltpu.bitcast(w << 16, F32), pltpu.bitcast(w & U32(0xFFFF0000), F32)


def _pack2(x, y, sign):
    e, o = [pltpu.bitcast(p + q if sign > 0 else p - q, U32) for p, q in zip(x, y)]
    return ((e + U32(0x8000)) >> 16) | ((o + U32(0x7FFF)) & U32(0xFFFF0000))


def _right_sums(b11, b21, b12, b22):
    b11, b21, b12, b22 = [_unpack(t) for t in (b11, b21, b12, b22)]
    return [_pack2(b21, b11, -1), _pack2(b12, b22, -1), _pack2(b11, b22, 1), _pack2(b11, b12, 1),
            _pack2(b21, b22, 1)]


class _Pace:
    def __init__(self):
        self.items, self.per, self.credit, self.before = [], 0.0, 0.0, []

    def spread(self, items, nslots):
        self.items, self.per = list(items), len(items) / nslots

    def require(self, zeros, nslots):
        for i, z in enumerate(zeros):
            self._gate(max((i + 1) * nslots // len(zeros) - 1, 0), z)

    def _gate(self, k, z):
        self.before += [None] * (k + 1 - len(self.before))
        self.before[k] = z if self.before[k] is None else self.before[k] | z

    def __call__(self, y):
        if self.items:
            self.credit += self.per
            n = min(int(self.credit + 1e-6), len(self.items))
            self.credit -= n
            if n:
                outs = [self.items.pop(0)() for _ in range(n)]
                self._gate(1, _zero_of(functools.reduce(jnp.bitwise_or, outs)))
        if self.before:
            z = self.before.pop(0)
            if z is not None:
                y = _after(y, z)
        return y


def _strassen(al, wt, pace=lambda y: y):
    m1 = pace(_dot(al[0], wt(4)))
    yield None
    m4 = pace(_dot(al[3], wt(1)))
    yield None
    m5 = pace(_dot(al[4], wt(3)))
    yield None
    m2 = pace(_dot(al[1], wt(0)))
    yield None
    m3 = pace(_dot(al[2], wt(2)))
    yield None
    c11 = pace(_dot(al[6], wt(6)) + (m1 + m4 - m5))
    yield None
    c22 = pace(_dot(al[5], wt(5)) + (m1 - m2 + m3))
    yield (jnp.concatenate([c11, m2 + m4], axis=0), jnp.concatenate([m3 + m5, c22], axis=0))


def _run(gen):
    for y in gen:
        pass
    return y


def _gelu_left(y0, y1):
    return _left(lambda r, t: _gelu((y0, y1)[t][r:r + CH]), 1)


def _kernel(x_hbm, mem0_hbm, wq_hbm, wk_hbm, wv_hbm, wo_hbm, w1_hbm, w2_hbm, w3_hbm, w4_hbm, out_hbm,
            x_ref, stage, wqkv_ref, wo_ref, w1_ref, q_ref, p_ref, r_ref,
            h_ref, b_ref, a3_ref, pre1_ref, pre_ref, s_ref, px_ref, e_ref, oe_ref, mem0_ref, mem_ref, sems, *, S, D, H, DH, M, SEG, FF):
    L = M + SEG
    R = 2 * L
    NP = H // 2
    ND = D // 128
    NF = FF // 128
    NQ = ND // 2
    KH = D // 4
    FS = (NF - CPRE) // 2
    FH = FS * 32
    HK = D // 2
    N1 = (S - RB0) // RB1
    N2 = S // RB2
    assert CPRE == ND and FS % 2 == 0
    Q_W2, Q_W3A, Q_W4A = 0, NQ, 2 * NQ
    QI = 3 * NQ // N1
    assert QI * N1 == 3 * NQ and N2 == NQ == 4 and FS // 2 - 1 == NQ

    SEM_OUT, SEM_MEM = range(2)
    SEM_W1 = 2
    SEM_X = SEM_W1 + ND
    SEM_Q = SEM_X + 4 + N1
    SEM_G = SEM_Q + N1
    KQ = KH // N2
    JG = NP // N2

    def tile_copy(src, row0, nrows, col, dst, sem):
        cols = pl.ds(pl.multiple_of(col * 128, 128), 128)
        return pltpu.make_async_copy(src.bitcast(U32).at[pl.ds(row0, nrows), cols], dst, sem)

    def quad_copies(src, row0, kh, col, dst_ref, q, sem, dist=1):
        return [tile_copy(src, row0, 2 * kh, col + t * dist, dst_ref.at[q, pl.ds(2 * kh * t, 2 * kh)], sem)
                for t in range(2)]

    def q_copies(q, sem):
        if q < Q_W3A:
            return quad_copies(w2_hbm, 0, KH, 2 * q, q_ref, q, sem)
        if q < Q_W4A:
            return quad_copies(w3_hbm, 0, KH, q - Q_W3A, q_ref, q, sem, CPRE // 2)
        return quad_copies(w4_hbm, 0, KH, 2 * (q - Q_W4A), q_ref, q, sem)

    def x_copy(lo, n, sem):
        return pltpu.make_async_copy(x_hbm.at[pl.ds(lo, n)], x_ref.at[pl.ds(lo, n)], sem)

    def group(i):
        sem = sems.at[SEM_G + i]
        cps = [pltpu.make_async_copy(w.bitcast(U32).at[:, i * JG + k, :], stage.at[m * NP + i * JG + k], sem)
               for m, w in enumerate((wq_hbm, wk_hbm, wv_hbm)) for k in range(JG)]
        for t in range(2):
            rq = 2 * i + t
            par, pair = rq >> 2, rq & 3
            cps += quad_copies(w3_hbm, 0, KH, CPRE + par * FS + 1 + pair, p_ref, rq, sem, FS // 2)
            row0 = pl.multiple_of(CPRE * 64 + par * 2 * FH, 64)
            cps += quad_copies(w4_hbm, row0, FH, 2 * pair, r_ref, rq, sem)
            cps.append(tile_copy(wo_hbm, 0, H * DH // 2, rq, wo_ref.at[rq], sem))
            for sl in range(4):
                r = pl.multiple_of(i * KQ, KQ)
                cps.append(tile_copy(w3_hbm, (sl % 2) * KH + r, KQ, CPRE + t * FS + (sl // 2) * (FS // 2),
                                     p_ref.at[2 * NQ + t, pl.ds(sl * KH + r, KQ)], sem))
        return cps

    g_mem = [pltpu.make_async_copy(mem0_hbm, mem0_ref, sems.at[SEM_MEM])]
    X0 = S - N1 * XK
    assert all(X0 + (k + 1) * XK >= min(RB0 + (k + 1) * RB1 + HB, S) for k in range(N1))
    xch = [(0, RA), (RA, RA + HB), (RA + HB, RB0 + HB), (RB0 + HB, X0)]
    xch += [(X0 + k * XK, X0 + (k + 1) * XK) for k in range(N1)]
    g_x = [x_copy(lo, hi - lo, sems.at[SEM_X + i]) for i, (lo, hi) in enumerate(xch)]
    g_w1 = [tile_copy(w1_hbm, 0, 2 * KH, j, w1_ref.at[j], sems.at[SEM_W1 + j]) for j in range(ND)]
    g_q = [[cp for t in range(QI) for cp in q_copies(QI * k + t, sems.at[SEM_Q + k])] for k in range(N1)]

    def start(*gs):
        for g in gs:
            for cp in g:
                cp.start()

    def wait(*gs):
        for g in gs:
            for cp in g:
                cp.wait()

    start(g_x[0:1], g_w1[0:6], g_x[1:2], g_w1[6:], g_x[2:4])
    for k in range(N1):
        start(g_x[4 + k:5 + k], g_q[k])
    start(g_mem)

    def prep_items(ref, q, kh, r0=0, n=None):
        def item(r):
            b = [ref[q, pl.ds(t * kh + r0 + r, 8), :] for t in range(4)]
            res = _right_sums(*b)
            for t, y in zip((1, 2, 4, 5, 6), res):
                ref[q, pl.ds(t * kh + r0 + r, 8), :] = y
            return res[-1]
        return [functools.partial(item, r) for r in range(0, kh if n is None else n, 8)]

    def wos_rows(q, op, v):
        k = (v // 32) * 3 + op
        return (k // JG) * NP + q * JG + k % JG, pl.ds(HK + 16 * (v % 32) + 8, 8)

    def quad_wt(ref, q, kh):
        return lambda i: ref[q, i * kh:(i + 1) * kh, :]

    def load_left(ref):
        return [_bf(ref[t]) for t in range(7)]

    def store_left(ref, al):
        for t in range(7):
            ref[t] = pltpu.bitcast(al[t], U32)

    h_ref[:, 0:8, :] = jnp.zeros((ND, 8, 128), F32)
    h_ref[:, S + 8:S + 16, :] = jnp.zeros((ND, 8, 128), F32)

    def ln2(r):
        xn = _ln(x_ref[pl.ds(r, HB), :].astype(F32))
        b_ref[pl.ds(r, HB), :] = xn
        top = jnp.concatenate([xn[g * SEG + 16:g * SEG + 24] for g in range(HB // SEG)], axis=0)
        bot = jnp.concatenate([xn[g * SEG + 24:g * SEG + 32] for g in range(HB // SEG)], axis=0)
        t1, t2, b1, b2 = top[:, :HK], top[:, HK:], bot[:, :HK], bot[:, HK:]
        rows = pl.ds(pl.multiple_of(((r >> 6) & 1) * 8, 8), 8)
        for k, v in enumerate((t1 + b2, b1 - t1, t2 - b2)):
            e_ref[r >> 7, k, rows, :] = _pk(v)
        return _ln(xn).astype(BF16)

    def shifted_left(r0):
        offs = (7, 9, 6, 10)
        return _left(lambda r, t: h_ref[t, pl.ds(r0 + r + offs[4 * t // ND], CH), :], NQ)

    def p1_rows(base, n, a, pace):
        for s in range(n):
            r = base + s * HB
            nxt = r + HB if s + 1 < n else pl.multiple_of(jnp.minimum(r + HB, S - HB), HB)
            a_n = ln2(nxt)
            for j in range(ND):
                h_ref[j, pl.ds(r + 8, HB), :] = _gelu(pace(_dot(a, w1_ref[j])))
            a = a_n
        pre1_ref[...] = pltpu.bitcast(a, U32)

    NA = RA // HB
    wait(g_x[0:1])
    a0 = [ln2(s * HB) for s in range(NPRE)]
    for gi, (j0, j1) in enumerate(W1G):
        wait(g_w1[j0:j1])
        if gi == len(W1G) - 1:
            wait(g_x[1:2])
            a_n = ln2(RA)
        for s in range(NA):
            if s == len(a0):
                a0.append(ln2(s * HB))
            for j in range(j0, j1):
                h_ref[j, pl.ds(s * HB + 8, HB), :] = _gelu(_dot(a0[s], w1_ref[j]))
    wait(g_x[2:3])
    al0, zs = shifted_left(0)
    store_left(pre_ref, al0)
    pace = _Pace()
    pace.require(zs, (RB0 - RA) // HB * ND - 2)
    p1_rows(RA, (RB0 - RA) // HB, a_n, pace)
    wait(g_x[3:4])

    def p1(k, c):
        base = pl.multiple_of(RB0 + k * RB1, BLK)
        x_copy(pl.multiple_of(X0 + k * XK, HB), XK, sems.at[SEM_X + 4 + k]).wait()
        landed = q_ref.at[pl.ds(QI * k, QI), pl.ds(0, 4 * KH)]
        pltpu.make_async_copy(landed, landed, sems.at[SEM_Q + k]).wait()

        @pl.when(k == 1)
        def _():
            start(group(0))

        pace = _Pace()
        pace.spread([t_ for t in range(QI) for t_ in prep_items(q_ref, QI * k + t, KH)], RB1 // HB * ND)
        p1_rows(base, RB1 // HB, _bf(pre1_ref[...]), pace)
        assert not pace.items
        return c
    lax.fori_loop(0, N1, p1, 0)

    wait(g_mem)
    mem_ref[...] = mem0_ref[...].astype(F32)

    def qkv_extra(blk, slab):
        def wt(off):
            return jnp.concatenate([stage[slab, off + 16 * i:off + 16 * i + 8, :] for i in range(KH // 8)], axis=0)
        e = [_bf(e_ref[jnp.minimum(blk, S // BLK - 1), k]) for k in range(3)]
        m1 = _dot(e[0], wt(0))
        px_ref[blk & 1, slab, 1] = _dot(e[1], wt(8)) + m1
        px_ref[blk & 1, slab, 0] = _dot(e[2], wt(HK)) + m1

    def p2(it, c):
        base = pl.multiple_of(it * RB2, RB2)
        nb = RB2 // BLK
        g = [None] * nb
        u = [None] * nb
        g[0] = load_left(pre_ref)

        def repack(k, i):
            slab = (k // JG) * NP + it * JG + k % JG
            ae, ao, be, bo = [stage[slab, pl.ds(o + i * 16, 8, stride=2), :] for o in (0, 1, HK, HK + 1)]
            (b11, b12), (b21, b22) = zip(_unpack(ae), _unpack(ao)), zip(_unpack(be), _unpack(bo))
            r, r2 = pl.ds(i * 8, 8), pl.ds(KH + i * 8, 8)
            res = [_pack2(b21, b11, -1), _pack2(b12, b22, -1), _pack2(b11, b22, 1), _pack2(b11, b12, 1),
                   _pack2(b21, b22, 1)]
            wqkv_ref[2 * slab, r, :] = (ae & U32(0xFFFF)) | (ao << 16)
            wqkv_ref[2 * slab, r2, :] = res[0]
            wqkv_ref[2 * slab + 1, r, :] = res[1]
            wqkv_ref[2 * slab + 1, r2, :] = (be >> 16) | (bo & U32(0xFFFF0000))
            stage[slab, pl.ds(i * 16, 8), :] = res[2]
            stage[slab, pl.ds(i * 16 + 8, 8), :] = res[3]
            stage[slab, pl.ds(HK + i * 16, 8), :] = res[4]
            return res[-1]

        rp = [functools.partial(repack, k, i) for k in range(3 * JG) for i in range(KH // 8)]
        pp = [it_ for t in range(2) for it_ in
              prep_items(p_ref, 2 * it + t, KH) + prep_items(r_ref, 2 * it + t, FH)
              + prep_items(p_ref, 2 * NQ + t, KH, pl.multiple_of(it * KQ, KQ), KQ)]

        def prep_wo(v):
            r1, r2 = pl.ds(128 * (v // 8) + 8 * (v % 8), 8), pl.ds(128 * (v // 8) + 64 + 8 * (v % 8), 8)
            b = [wo_ref[2 * it + t // 2, (r1, r2)[t % 2], :] for t in range(4)]
            s4, s3, *rest = _right_sums(*b)
            wo_ref[2 * it, r2, :] = s4
            wo_ref[2 * it + 1, r1, :] = s3
            for op, y in enumerate(rest):
                slab, rows = wos_rows(it, op, v)
                stage[slab, rows, :] = y
            return rest[-1]

        wp = [functools.partial(prep_wo, v) for v in range(128)]
        items = []
        done = 0
        while rp or pp or wp:
            items += rp[:12] + pp[:4 if rp else 2]
            done += len(rp[:12])
            pp = pp[4 if rp else 2:]
            rp = rp[12:]
            n = min(5, done // 96 * 32 - (128 - len(wp)))
            items += wp[:n]
            wp = wp[n:]
        pace = _Pace()
        SL = NQ * 7

        zeros = {}
        carry = {}
        nitems = len(items)

        def make_g(s):
            if s < nb:
                g[s], zeros["g", s] = shifted_left(base + s * BLK)
            else:
                al_n, zeros["g", s] = shifted_left(pl.multiple_of(jnp.minimum(base + RB2, S - BLK), BLK))
                store_left(pre_ref, al_n)

        def next_weights():
            wait(group(it))

            @pl.when(it < N2 - 1)
            def _():
                start(group(it + 1))
            pace.spread(items, 1)

        def mix(s):
            ys = []
            for q in range(NQ):
                ys += _run(_strassen(g[s], quad_wt(q_ref, Q_W2 + q, KH), pace))
            rows = pl.ds(base + s * BLK, BLK)
            x1 = jnp.concatenate(ys, axis=1) + b_ref[rows, :]
            b_ref[rows, :] = x1
            y = [_ln(x1[r:r + CH]) for r in range(0, BLK, CH)]
            al, zeros["a", s] = _left(lambda r, t: y[r // CH][:, t * 128:(t + 1) * 128], NQ)
            store_left(a3_ref.at[it * nb + s], al)

        def up(s):
            al = load_left(a3_ref.at[it * nb + s])
            parts = []
            for q in range(NQ):
                ys = _run(_strassen(al, quad_wt(q_ref, Q_W3A + q, KH), pace))
                if s == 0 and q == NQ - 1:
                    next_weights()
                p, carry[0] = _gelu_left(*ys)
                parts.append(p)
                if q + 1 < NQ:
                    pace.require(carry.pop(0), 7)
            u[s] = _cat(parts, 1)

        def down(s):
            for q in range(NQ):
                ys = _run(_strassen(u[s], quad_wt(q_ref, Q_W4A + q, KH), pace))
                for t in range(2):
                    cols = slice((2 * q + t) * 128, (2 * q + t + 1) * 128)
                    rows = pl.ds(base + s * BLK, BLK)
                    b_ref[rows, cols] = ys[t] + b_ref[rows, cols]

        assert nb == 4
        for s in range(1, nb):
            make_g(s)
        zg = zeros["g", 1] + zeros["g", 2] + zeros["g", 3]
        zeros["g01"], zeros["g12"], zeros["g23"] = zg[:24], zg[24:36], zg[36:]
        plan = [(mix, 0, ["g01"], 0), (mix, 1, [("a", 0), "g12"], 0), (mix, 2, [("a", 1), "g23"], 0),
                (mix, 3, [("a", 2)], 0), (up, 0, [("a", 3)], 0), (up, 1, [], 0.9), (down, 0, [], 1.6),
                (up, 2, [], 0.9), (down, 1, [], 1.6), (up, 3, [], 0.9), (down, 2, [], 1.6),
                (down, 3, [("g", 4)], 1.5)]
        wsum = sum(p[3] for p in plan) - plan[-1][3] * 2 / SL
        for fn, s, keys, w in plan:
            for key in keys:
                if key not in zeros:
                    make_g(key[1])
            zs = carry.pop(0, []) + [z for key in keys for z in zeros[key]]
            if zs:
                pace.require(zs, SL - 1 if keys else 7)
            pace.per = nitems * w / wsum / SL
            fn(s)
        assert not pace.items
        for k in range(6):
            qkv_extra(0, (k % 3) * NP + 2 * it + k // 3)
        return c
    lax.fori_loop(0, N2, p2, 0)

    row = lax.broadcasted_iota(jnp.int32, (R, R), 0)
    col = lax.broadcasted_iota(jnp.int32, (R, R), 1)
    same_head = (row >= L) == (col >= L)
    rr = jnp.where(row >= L, row - L, row)
    cc = jnp.where(col >= L, col - L, col)
    visible = same_head & ((rr < M) | (rr >= cc))
    scale = DH ** -0.5
    fill = jnp.where(same_head, -1e9 / scale, -jnp.inf).astype(F32)

    def softmax_qk(q2, k2):
        s = lax.dot_general(q2, k2, (((1,), (1,)), ((), ())), preferred_element_type=F32)
        s = jnp.where(visible, s, fill)
        m = jnp.max(s, axis=-1, keepdims=True)
        e = jnp.exp2((s - m) * (scale * LOG2E))
        l = jnp.sum(e, axis=-1, keepdims=True)
        r = pl.reciprocal(l, approx=True)
        r = r * (2.0 - l * r)
        return (e * r).astype(BF16)

    def combine(r, rdst, slot):
        b = b_ref[pl.ds(r, STEP), :]
        hb = 0.5 * b
        g = hb + hb * jnp.tanh(hb)
        x = x_ref[pl.ds(r, STEP), :].astype(F32)
        x_ref[pl.ds(rdst, STEP), :] = (x + s_ref[slot] * g).astype(x_ref.dtype)

    def out_copy(r):
        return pltpu.make_async_copy(x_ref.at[pl.ds(r, STEP)], out_hbm.at[pl.ds(r, STEP)], sems.at[SEM_OUT])

    def wo_extra(kb, q):
        def wt(op):
            return jnp.concatenate([stage[wos_rows(q, op, v) + (slice(None),)] for v in range(128)], axis=0)
        e = [oe_ref[kb & 1, k].astype(BF16) for k in range(3)]
        m1 = _dot(e[0], wt(0))
        pb = _dot(e[1], wt(1)) + m1
        pt = _dot(e[2], wt(2)) + m1
        c0 = pl.ds(pl.multiple_of(2 * q * 128, 128), 128)
        c1 = pl.ds(pl.multiple_of((2 * q + 1) * 128, 128), 128)
        for g in range(4):
            slot = (2 * kb + g // 2) & 3
            r = (g % 2) * SEG + 16
            s_ref[slot, r:r + 8, c0] = s_ref[slot, r:r + 8, c0] + pt[8 * g:8 * g + 8]
            s_ref[slot, r + 8:r + 16, c1] = s_ref[slot, r + 8:r + 16, c1] + pb[8 * g:8 * g + 8]

    def sweep_lhs(m1, m2, x1, x2):
        ms, xs = m1 + m2, x1 + x2
        return [jnp.concatenate(v, axis=0).astype(BF16) for v in (
            [ms, xs[0:16], xs[24:32]], [m2, x2[0:16], x2[24:32]],
            [m1, x1[0:16], x1[16:24]], [ms, xs[0:16], xs[16:24]])]

    s_ref[1:4] = jnp.zeros((3,) + s_ref.shape[1:], F32)
    oe_ref[1] = jnp.zeros(oe_ref.shape[1:], F32)

    def step(j, c):
        r0 = pl.multiple_of(j * STEP, STEP)
        par = j & 1
        blk = j >> 1
        rb = pl.multiple_of(blk * BLK, BLK)
        rprev = pl.multiple_of(jnp.maximum(r0 - 3 * STEP, 0), STEP)
        rdst = pl.multiple_of(jnp.where(j >= 3, r0 - 3 * STEP, S), STEP)
        al3 = load_left(a3_ref.at[blk])
        xn = _ln(x_ref[pl.ds(r0, STEP), :].astype(F32))

        parts = []

        def up_products():
            for q in range(FS // 2):
                wt = quad_wt(p_ref, 2 * NQ + par if q == 0 else par * NQ + q - 1, KH)
                for y in _strassen(al3, wt):
                    if y is not None:
                        parts.append(_gelu_left(*y)[0])
                    yield

        def down_products():
            al4 = _cat(parts, 1)
            for q in range(NQ):
                for ys in _strassen(al4, quad_wt(r_ref, par * NQ + q, FH)):
                    if ys is not None:
                        for t in range(2):
                            cols = slice((2 * q + t) * 128, (2 * q + t + 1) * 128)
                            b_ref[pl.ds(rb, BLK), cols] = ys[t] + b_ref[pl.ds(rb, BLK), cols]
                    yield
        ups, downs = up_products(), down_products()

        def run(gen, n):
            for _ in range(n):
                next(gen)

        def segment(sg, mem, fillers, inter):
            xs = xn[sg * SEG:(sg + 1) * SEG]
            lhs = sweep_lhs(mem[:, :HK], mem[:, HK:], xs[:, :HK], xs[:, HK:])
            prow = pl.ds(pl.multiple_of((par * 2 + sg) * 8, 8), 8)
            qkv = [None] * NP
            prob = [None] * NP
            ol = [None] * NP
            ph = NP - 3

            def do_qkv(p):
                res = []
                for m in range(3):
                    w0, w1 = m * H + 2 * p, m * H + 2 * p + 1
                    d11 = _dot(lhs[0], wqkv_ref[w0, 0:KH, :])
                    d4 = _dot(lhs[1], wqkv_ref[w0, KH:, :])
                    d3 = _dot(lhs[2], wqkv_ref[w1, 0:KH, :])
                    d22 = _dot(lhs[3], wqkv_ref[w1, KH:, :])
                    pt = px_ref[blk & 1, m * NP + p, 0, prow, :]
                    pb = px_ref[blk & 1, m * NP + p, 1, prow, :]
                    res.append(jnp.concatenate([
                        d11[0:24] + d4[0:24], pt + (d4[24:32] - d22[24:32]), d11[24:32] + d4[24:32],
                        d3[0:24] + d22[0:24], d3[24:32] + d22[24:32], pb + (d3[24:32] - d11[24:32])],
                        axis=0).astype(BF16))
                qkv[p] = res

            def do_qk(p):
                prob[p] = softmax_qk(qkv[p][0], qkv[p][1])

            def do_pv(p):
                o = jnp.dot(prob[p], qkv[p][2], preferred_element_type=F32)
                o1, o2 = o[0:L], o[L:]
                ol[p] = sweep_lhs(o1[0:8], o2[0:8], o1[8:], o2[8:])
                t1, t2, b1, b2 = o1[24:32], o2[24:32], o1[32:40], o2[32:40]
                for k, v in enumerate((t1 + b2, b1 - t1, t2 - b2)):
                    oe_ref[blk & 1, k, prow, p * 128:(p + 1) * 128] = v

            def wo_part(ps, q, acc=None):
                d = []
                for k in range(4):
                    n, o = 2 * q + k // 2, 64 * (k % 2)
                    y = _dot(jnp.concatenate([ol[p][k] for p in ps], axis=1),
                             jnp.concatenate([wo_ref[n, 128 * p + o:128 * p + o + 64, :] for p in ps], axis=0))
                    d.append(y if acc is None else y + acc[k])
                return d

            for p in range(NP):
                do_qkv(p)
                inter(p)
                if p >= 1:
                    do_qk(p - 1)
                if p >= 3:
                    do_pv(p - 3)
            fillers[0]()
            do_qk(NP - 1)
            do_pv(NP - 3)
            do_pv(NP - 2)
            acc = [wo_part(range(ph), q) for q in range(NQ // 2)]
            do_pv(NP - 1)
            fillers[1]()
            acc += [wo_part(range(ph), q) for q in range(NQ // 2, NQ)]
            cols = []
            for q in range(NQ):
                d11, d4, d3, d22 = wo_part(range(ph, NP), q, acc[q])
                cols += [jnp.concatenate([d11[0:24] + d4[0:24], d4[24:32] - d22[24:32], d11[24:32] + d4[24:32]], axis=0),
                         jnp.concatenate([d3[0:24] + d22[0:24], d3[24:32] + d22[24:32], d3[24:32] - d11[24:32]], axis=0)]
            res = jnp.concatenate(cols, axis=1)
            s_ref[j & 3, sg * SEG:(sg + 1) * SEG, :] = res[8:]
            mem_ref[...] = res[0:8]
            fillers[2]()
            return res[0:8]

        U0, U1, IA, IB, D0 = 8, 6, 1, 2, 7

        def inter_a(p):
            if p < NP // 2:
                for m in range(3):
                    qkv_extra((j + 1) >> 1, m * NP + (1 - par) * (NP // 2) + p)
            if p >= IA:
                run(ups, 1)

        def tail_b0():
            combine(rprev, rdst, (j + 1) & 3)
            run(downs, D0)

        def tail_b2():
            for t in range(2):
                wo_extra((j - 1) >> 1, 2 * (1 - par) + t)

        mem = mem_ref[...]
        run(ups, U0)
        mem = segment(0, mem, [lambda: run(ups, U1), lambda: None, lambda: run(ups, 35 - U0 - U1 - (NP - IA))],
                      inter_a)
        segment(1, mem, [tail_b0, lambda: run(downs, 28 - (NP - IB) - D0), tail_b2],
                lambda p: run(downs, 1) if p >= IB else None)

        @pl.when(j >= 3)
        def _():
            out_copy(rprev).start()
        return c
    nst = S // STEP
    lax.fori_loop(0, nst, step, 0)
    for t in range(2):
        wo_extra(nst // 2 - 1, 2 + t)

    def last(j, c):
        r = pl.multiple_of(j * STEP, STEP)
        combine(r, r, j & 3)
        out_copy(r).start()
        return c
    lax.fori_loop(nst - 3, nst, last, 0)
    pltpu.make_async_copy(x_ref.at[pl.ds(0, S)], out_hbm, sems.at[SEM_OUT]).wait()


@functools.partial(jax.jit, static_argnames=("A_seg_len",))
def pallas_recurrent_scan__memory_aug_recurrent_mem_tr__mixer_s_mlp__prompt_kernel(
        A_x, A_mem0, A_Wq, A_Wk, A_Wv, A_Wo, A_seg_len, B_x, B_w1, B_w2, B_w3, B_w4):
    del B_x
    B, S, D = A_x.shape
    _, H, DH = A_Wq.shape
    M = A_mem0.shape[1]
    FF = B_w3.shape[1]
    assert (B, S, D, H, DH, M, A_seg_len, FF) == (1, 2048, 1024, 32, 128, 8, 32, 3584)
    nd, nf = D // 128, FF // 128
    kern = functools.partial(_kernel, S=S, D=D, H=H, DH=DH, M=M, SEG=A_seg_len, FF=FF)
    any_spec = pl.BlockSpec(memory_space=pl.ANY)
    out = pl.pallas_call(
        kern,
        out_shape=jax.ShapeDtypeStruct((S, D), A_x.dtype),
        in_specs=[any_spec] * 10,
        out_specs=any_spec,
        scratch_shapes=[
            pltpu.VMEM((S + STEP, D), BF16),
            pltpu.VMEM((3 * H // 2, D, 128), U32),
            pltpu.VMEM((3 * H, D // 2, 128), U32),
            pltpu.VMEM((nd, H * DH // 2, 128), U32),
            pltpu.VMEM((nd, D // 2, 128), U32),
            pltpu.VMEM((3 * nd // 2, 7 * D // 4, 128), U32),
            pltpu.VMEM(((nf - CPRE) // 2, 7 * D // 4, 128), U32),
            pltpu.VMEM((nd, 7 * (nf - CPRE) * 16, 128), U32),
            pltpu.VMEM((nd, S + 16, 128), F32),
            pltpu.VMEM((S, D), F32),
            pltpu.VMEM((S // BLK, 7, HB // 2, D // 2), U32),
            pltpu.VMEM((HB // 2, D), U32),
            pltpu.VMEM((7, HB // 2, D // 2), U32),
            pltpu.VMEM((4, STEP, D), F32),
            pltpu.VMEM((2, 3 * H // 2, 2, 32, 128), F32),
            pltpu.VMEM((S // BLK, 3, 16, D // 2), U32),
            pltpu.VMEM((2, 3, 32, H * DH // 2), F32),
            pltpu.VMEM((M, D), BF16),
            pltpu.VMEM((M, D), F32),
            pltpu.SemaphoreType.DMA((2 + nd + 4 + 2 * ((S - RB0) // RB1) + S // RB2,)),
        ],
        compiler_params=pltpu.CompilerParams(vmem_limit_bytes=127 * 1024 * 1024,
                                             disable_bounds_checks=True),
    )(A_x[0], A_mem0[0], A_Wq, A_Wk, A_Wv, A_Wo.reshape(H * DH, D), B_w1, B_w2, B_w3, B_w4)
    return out[None]
```

```python
import functools

import jax
import jax.numpy as jnp
from jax import lax
import jax.experimental.pallas as pl
import jax.experimental.pallas.tpu as pltpu

F32 = jnp.float32
BF16 = jnp.bfloat16
U32 = jnp.uint32
EPS = 1e-5
LOG2E = 1.4426950408889634

HB = 64
BLK = 2 * HB
RB0 = 512
RA = 256
RB1 = 256
RB2 = 512
CPRE = 8
STEP = 64
NPRE = 2
W1G = ((0, 2), (2, 5), (5, 8))
XK = 192
CH = 16


def _ln(x):
    m = jnp.mean(x, axis=-1, keepdims=True)
    xc = x - m
    v = jnp.mean(xc * xc, axis=-1, keepdims=True)
    return xc * lax.rsqrt(v + EPS)


def _gelu(x):
    c = 0.7978845608028654
    h = 0.5 * x
    return h + h * jnp.tanh(x * (c + (c * 0.044715) * (x * x)))


def _bf(w_u32):
    return pltpu.bitcast(w_u32, BF16)


def _pk(x):
    return pltpu.bitcast(x.astype(BF16), U32)


def _dot(a, w_u32):
    return jnp.dot(a, _bf(w_u32), preferred_element_type=F32)


def _zero_of(y):
    if y.dtype != U32:
        y = pltpu.bitcast(y[0:(8 if y.dtype == F32 else 16), 0:128], U32)
    return (y[0:8, 0:128] >> 31) >> 1


def _after(y, z):
    return jnp.concatenate([y[0:8] + pltpu.bitcast(z, F32), y[8:]], axis=0)


def _left(get, nk):
    rows, zs = [], []
    for r in range(0, HB, CH):
        cols = []
        for t in range(nk):
            a11, a12, a21, a22 = get(r, t), get(r, nk + t), get(HB + r, t), get(HB + r, nk + t)
            p = [y.astype(BF16) for y in (a11 + a22, a21 + a22, a11, a22, a11 + a12, a21 - a11, a12 - a22)]
            zs.append(_zero_of(functools.reduce(jnp.bitwise_or, [pltpu.bitcast(y, U32) for y in p])))
            cols.append(p)
        rows.append(_cat(cols, 1))
    return _cat(rows, 0), zs


def _cat(parts, axis):
    return [jnp.concatenate([p[t] for p in parts], axis=axis) for t in range(7)]


def _unpack(w):
    return pltpu.bitcast(w << 16, F32), pltpu.bitcast(w & U32(0xFFFF0000), F32)


def _pack2(x, y, sign):
    e, o = [pltpu.bitcast(p + q if sign > 0 else p - q, U32) for p, q in zip(x, y)]
    return ((e + U32(0x8000)) >> 16) | ((o + U32(0x7FFF)) & U32(0xFFFF0000))


def _right_sums(b11, b21, b12, b22):
    b11, b21, b12, b22 = [_unpack(t) for t in (b11, b21, b12, b22)]
    return [_pack2(b21, b11, -1), _pack2(b12, b22, -1), _pack2(b11, b22, 1), _pack2(b11, b12, 1),
            _pack2(b21, b22, 1)]


class _Pace:
    def __init__(self):
        self.items, self.per, self.credit, self.before = [], 0.0, 0.0, []

    def spread(self, items, nslots):
        self.items, self.per = list(items), len(items) / nslots

    def require(self, zeros, nslots):
        for i, z in enumerate(zeros):
            self._gate(max((i + 1) * nslots // len(zeros) - 1, 0), z)

    def _gate(self, k, z):
        self.before += [None] * (k + 1 - len(self.before))
        self.before[k] = z if self.before[k] is None else self.before[k] | z

    def __call__(self, y):
        if self.items:
            self.credit += self.per
            n = min(int(self.credit + 1e-6), len(self.items))
            self.credit -= n
            if n:
                outs = [self.items.pop(0)() for _ in range(n)]
                self._gate(1, _zero_of(functools.reduce(jnp.bitwise_or, outs)))
        if self.before:
            z = self.before.pop(0)
            if z is not None:
                y = _after(y, z)
        return y


def _strassen(al, wt, pace=lambda y: y):
    m1 = pace(_dot(al[0], wt(4)))
    yield None
    m4 = pace(_dot(al[3], wt(1)))
    yield None
    m5 = pace(_dot(al[4], wt(3)))
    yield None
    m2 = pace(_dot(al[1], wt(0)))
    yield None
    m3 = pace(_dot(al[2], wt(2)))
    yield None
    c11 = pace(_dot(al[6], wt(6)) + (m1 + m4 - m5))
    yield None
    c22 = pace(_dot(al[5], wt(5)) + (m1 - m2 + m3))
    yield (jnp.concatenate([c11, m2 + m4], axis=0), jnp.concatenate([m3 + m5, c22], axis=0))


def _run(gen):
    for y in gen:
        pass
    return y


def _gelu_left(y0, y1):
    return _left(lambda r, t: _gelu((y0, y1)[t][r:r + CH]), 1)


def _kernel(x_hbm, mem0_hbm, wq_hbm, wk_hbm, wv_hbm, wo_hbm, w1_hbm, w2_hbm, w3_hbm, w4_hbm, out_hbm,
            x_ref, stage, wqkv_ref, wo_ref, w1_ref, q_ref, p_ref, r_ref,
            h_ref, b_ref, a3_ref, pre1_ref, pre_ref, s_ref, px_ref, e_ref, oe_ref, mem0_ref, mem_ref, sems,
            *, S, D, H, DH, M, SEG, FF):
    L = M + SEG
    R = 2 * L
    NP = H // 2
    ND = D // 128
    NF = FF // 128
    NQ = ND // 2
    KH = D // 4
    FS = (NF - CPRE) // 2
    FH = FS * 32
    HK = D // 2
    N1 = (S - RB0) // RB1
    N2 = S // RB2
    assert CPRE == ND and FS % 2 == 0
    Q_W2, Q_W3A, Q_W4A = 0, NQ, 2 * NQ
    QI = 3 * NQ // N1
    assert QI * N1 == 3 * NQ and N2 == NQ == 4 and FS // 2 - 1 == NQ

    SEM_OUT, SEM_MEM = range(2)
    SEM_W1 = 2
    SEM_X = SEM_W1 + ND
    SEM_Q = SEM_X + 4 + N1
    SEM_G = SEM_Q + N1
    KQ = KH // N2
    JG = NP // N2

    def tile_copy(src, row0, nrows, col, dst, sem):
        cols = pl.ds(pl.multiple_of(col * 128, 128), 128)
        return pltpu.make_async_copy(src.bitcast(U32).at[pl.ds(row0, nrows), cols], dst, sem)

    def quad_copies(src, row0, kh, col, dst_ref, q, sem, dist=1):
        return [tile_copy(src, row0, 2 * kh, col + t * dist, dst_ref.at[q, pl.ds(2 * kh * t, 2 * kh)], sem)
                for t in range(2)]

    def q_copies(q, sem):
        if q < Q_W3A:
            return quad_copies(w2_hbm, 0, KH, 2 * q, q_ref, q, sem)
        if q < Q_W4A:
            return quad_copies(w3_hbm, 0, KH, q - Q_W3A, q_ref, q, sem, CPRE // 2)
        return quad_copies(w4_hbm, 0, KH, 2 * (q - Q_W4A), q_ref, q, sem)

    def x_copy(lo, n, sem):
        return pltpu.make_async_copy(x_hbm.at[pl.ds(lo, n)], x_ref.at[pl.ds(lo, n)], sem)

    def group(i):
        sem = sems.at[SEM_G + i]
        cps = [pltpu.make_async_copy(w.bitcast(U32).at[:, i * JG + k, :], stage.at[m * NP + i * JG + k], sem)
               for m, w in enumerate((wq_hbm, wk_hbm, wv_hbm)) for k in range(JG)]
        for t in range(2):
            rq = 2 * i + t
            par, pair = rq >> 2, rq & 3
            cps += quad_copies(w3_hbm, 0, KH, CPRE + par * FS + 1 + pair, p_ref, rq, sem, FS // 2)
            row0 = pl.multiple_of(CPRE * 64 + par * 2 * FH, 64)
            cps += quad_copies(w4_hbm, row0, FH, 2 * pair, r_ref, rq, sem)
            cps.append(tile_copy(wo_hbm, 0, H * DH // 2, rq, wo_ref.at[rq], sem))
            for sl in range(4):
                r = pl.multiple_of(i * KQ, KQ)
                cps.append(tile_copy(w3_hbm, (sl % 2) * KH + r, KQ, CPRE + t * FS + (sl // 2) * (FS // 2),
                                     p_ref.at[2 * NQ + t, pl.ds(sl * KH + r, KQ)], sem))
        return cps

    g_mem = [pltpu.make_async_copy(mem0_hbm, mem0_ref, sems.at[SEM_MEM])]
    X0 = S - N1 * XK
    assert all(X0 + (k + 1) * XK >= min(RB0 + (k + 1) * RB1 + HB, S) for k in range(N1))
    xch = [(0, RA), (RA, RA + HB), (RA + HB, RB0 + HB), (RB0 + HB, X0)]
    xch += [(X0 + k * XK, X0 + (k + 1) * XK) for k in range(N1)]
    g_x = [x_copy(lo, hi - lo, sems.at[SEM_X + i]) for i, (lo, hi) in enumerate(xch)]
    g_w1 = [tile_copy(w1_hbm, 0, 2 * KH, j, w1_ref.at[j], sems.at[SEM_W1 + j]) for j in range(ND)]
    g_q = [[cp for t in range(QI) for cp in q_copies(QI * k + t, sems.at[SEM_Q + k])] for k in range(N1)]

    def start(*gs):
        for g in gs:
            for cp in g:
                cp.start()

    def wait(*gs):
        for g in gs:
            for cp in g:
                cp.wait()

    start(g_x[0:1], g_w1[0:6], g_x[1:2], g_w1[6:], g_x[2:4])
    for k in range(N1):
        start(g_x[4 + k:5 + k], g_q[k])
    start(g_mem)

    def prep_items(ref, q, kh, r0=0, n=None):
        def item(r):
            b = [ref[q, pl.ds(t * kh + r0 + r, 8), :] for t in range(4)]
            res = _right_sums(*b)
            for t, y in zip((1, 2, 4, 5, 6), res):
                ref[q, pl.ds(t * kh + r0 + r, 8), :] = y
            return res[-1]
        return [functools.partial(item, r) for r in range(0, kh if n is None else n, 8)]

    def wos_rows(q, op, v):
        k = (v // 32) * 3 + op
        return (k // JG) * NP + q * JG + k % JG, pl.ds(HK + 16 * (v % 32) + 8, 8)

    def quad_wt(ref, q, kh):
        return lambda i: ref[q, i * kh:(i + 1) * kh, :]

    def load_left(ref):
        return [_bf(ref[t]) for t in range(7)]

    def store_left(ref, al):
        for t in range(7):
            ref[t] = pltpu.bitcast(al[t], U32)

    h_ref[:, 0:8, :] = jnp.zeros((ND, 8, 128), F32)
    h_ref[:, S + 8:S + 16, :] = jnp.zeros((ND, 8, 128), F32)

    def ln2(r):
        xn = _ln(x_ref[pl.ds(r, HB), :].astype(F32))
        b_ref[pl.ds(r, HB), :] = xn
        top = jnp.concatenate([xn[g * SEG + 16:g * SEG + 24] for g in range(HB // SEG)], axis=0)
        bot = jnp.concatenate([xn[g * SEG + 24:g * SEG + 32] for g in range(HB // SEG)], axis=0)
        t1, t2, b1, b2 = top[:, :HK], top[:, HK:], bot[:, :HK], bot[:, HK:]
        rows = pl.ds(pl.multiple_of(((r >> 6) & 1) * 8, 8), 8)
        for k, v in enumerate((t1 + b2, b1 - t1, t2 - b2)):
            e_ref[r >> 7, k, rows, :] = _pk(v)
        return _ln(xn).astype(BF16)

    def shifted_left(r0):
        offs = (7, 9, 6, 10)
        return _left(lambda r, t: h_ref[t, pl.ds(r0 + r + offs[4 * t // ND], CH), :], NQ)

    def p1_rows(base, n, a, pace):
        for s in range(n):
            r = base + s * HB
            nxt = r + HB if s + 1 < n else pl.multiple_of(jnp.minimum(r + HB, S - HB), HB)
            a_n = ln2(nxt)
            for j in range(ND):
                h_ref[j, pl.ds(r + 8, HB), :] = _gelu(pace(_dot(a, w1_ref[j])))
            a = a_n
        pre1_ref[...] = pltpu.bitcast(a, U32)

    NA = RA // HB
    wait(g_x[0:1])
    a0 = [ln2(s * HB) for s in range(NPRE)]
    for gi, (j0, j1) in enumerate(W1G):
        wait(g_w1[j0:j1])
        if gi == len(W1G) - 1:
            wait(g_x[1:2])
            a_n = ln2(RA)
        for s in range(NA):
            if s == len(a0):
                a0.append(ln2(s * HB))
            for j in range(j0, j1):
                h_ref[j, pl.ds(s * HB + 8, HB), :] = _gelu(_dot(a0[s], w1_ref[j]))
    wait(g_x[2:3])
    al0, zs = shifted_left(0)
    store_left(pre_ref, al0)
    pace = _Pace()
    pace.require(zs, (RB0 - RA) // HB * ND - 2)
    p1_rows(RA, (RB0 - RA) // HB, a_n, pace)
    wait(g_x[3:4])

    def p1(k, c):
        base = pl.multiple_of(RB0 + k * RB1, BLK)
        x_copy(pl.multiple_of(X0 + k * XK, HB), XK, sems.at[SEM_X + 4 + k]).wait()
        landed = q_ref.at[pl.ds(QI * k, QI), pl.ds(0, 4 * KH)]
        pltpu.make_async_copy(landed, landed, sems.at[SEM_Q + k]).wait()

        @pl.when(k == 1)
        def _():
            start(group(0))

        pace = _Pace()
        pace.spread([t_ for t in range(QI) for t_ in prep_items(q_ref, QI * k + t, KH)], RB1 // HB * ND)
        p1_rows(base, RB1 // HB, _bf(pre1_ref[...]), pace)
        assert not pace.items
        return c
    lax.fori_loop(0, N1, p1, 0)

    wait(g_mem)
    mem_ref[...] = mem0_ref[...].astype(F32)

    def qkv_extra(blk, slab):
        def wt(off):
            return jnp.concatenate([stage[slab, off + 16 * i:off + 16 * i + 8, :] for i in range(KH // 8)], axis=0)
        e = [_bf(e_ref[jnp.minimum(blk, S // BLK - 1), k]) for k in range(3)]
        m1 = _dot(e[0], wt(0))
        px_ref[blk & 1, slab, 1] = _dot(e[1], wt(8)) + m1
        px_ref[blk & 1, slab, 0] = _dot(e[2], wt(HK)) + m1

    def p2(it, c):
        base = pl.multiple_of(it * RB2, RB2)
        nb = RB2 // BLK
        g = [None] * nb
        u = [None] * nb
        g[0] = load_left(pre_ref)

        def repack(k, i):
            slab = (k // JG) * NP + it * JG + k % JG
            ae, ao, be, bo = [stage[slab, pl.ds(o + i * 16, 8, stride=2), :] for o in (0, 1, HK, HK + 1)]
            (b11, b12), (b21, b22) = zip(_unpack(ae), _unpack(ao)), zip(_unpack(be), _unpack(bo))
            r, r2 = pl.ds(i * 8, 8), pl.ds(KH + i * 8, 8)
            res = [_pack2(b21, b11, -1), _pack2(b12, b22, -1), _pack2(b11, b22, 1), _pack2(b11, b12, 1),
                   _pack2(b21, b22, 1)]
            wqkv_ref[2 * slab, r, :] = (ae & U32(0xFFFF)) | (ao << 16)
            wqkv_ref[2 * slab, r2, :] = res[0]
            wqkv_ref[2 * slab + 1, r, :] = res[1]
            wqkv_ref[2 * slab + 1, r2, :] = (be >> 16) | (bo & U32(0xFFFF0000))
            stage[slab, pl.ds(i * 16, 8), :] = res[2]
            stage[slab, pl.ds(i * 16 + 8, 8), :] = res[3]
            stage[slab, pl.ds(HK + i * 16, 8), :] = res[4]
            return res[-1]

        rp = [functools.partial(repack, k, i) for k in range(3 * JG) for i in range(KH // 8)]
        pp = [it_ for t in range(2) for it_ in
              prep_items(p_ref, 2 * it + t, KH) + prep_items(r_ref, 2 * it + t, FH)
              + prep_items(p_ref, 2 * NQ + t, KH, pl.multiple_of(it * KQ, KQ), KQ)]

        def prep_wo(v):
            r1, r2 = pl.ds(128 * (v // 8) + 8 * (v % 8), 8), pl.ds(128 * (v // 8) + 64 + 8 * (v % 8), 8)
            b = [wo_ref[2 * it + t // 2, (r1, r2)[t % 2], :] for t in range(4)]
            s4, s3, *rest = _right_sums(*b)
            wo_ref[2 * it, r2, :] = s4
            wo_ref[2 * it + 1, r1, :] = s3
            for op, y in enumerate(rest):
                slab, rows = wos_rows(it, op, v)
                stage[slab, rows, :] = y
            return rest[-1]

        wp = [functools.partial(prep_wo, v) for v in range(128)]
        items = []
        done = 0
        while rp or pp or wp:
            items += rp[:12] + pp[:4 if rp else 2]
            done += len(rp[:12])
            pp = pp[4 if rp else 2:]
            rp = rp[12:]
            n = min(5, done // 96 * 32 - (128 - len(wp)))
            items += wp[:n]
            wp = wp[n:]
        pace = _Pace()
        SL = NQ * 7

        zeros = {}
        carry = {}
        nitems = len(items)

        def make_g(s):
            if s < nb:
                g[s], zeros["g", s] = shifted_left(base + s * BLK)
            else:
                al_n, zeros["g", s] = shifted_left(pl.multiple_of(jnp.minimum(base + RB2, S - BLK), BLK))
                store_left(pre_ref, al_n)

        def next_weights():
            wait(group(it))

            @pl.when(it < N2 - 1)
            def _():
                start(group(it + 1))
            pace.spread(items, 1)

        def mix(s):
            ys = []
            for q in range(NQ):
                ys += _run(_strassen(g[s], quad_wt(q_ref, Q_W2 + q, KH), pace))
            rows = pl.ds(base + s * BLK, BLK)
            x1 = jnp.concatenate(ys, axis=1) + b_ref[rows, :]
            b_ref[rows, :] = x1
            y = [_ln(x1[r:r + CH]) for r in range(0, BLK, CH)]
            al, zeros["a", s] = _left(lambda r, t: y[r // CH][:, t * 128:(t + 1) * 128], NQ)
            store_left(a3_ref.at[it * nb + s], al)

        def up(s):
            al = load_left(a3_ref.at[it * nb + s])
            parts = []
            for q in range(NQ):
                ys = _run(_strassen(al, quad_wt(q_ref, Q_W3A + q, KH), pace))
                if s == 0 and q == NQ - 1:
                    next_weights()
                p, carry[0] = _gelu_left(*ys)
                parts.append(p)
                if q + 1 < NQ:
                    pace.require(carry.pop(0), 7)
            u[s] = _cat(parts, 1)

        def down(s):
            for q in range(NQ):
                ys = _run(_strassen(u[s], quad_wt(q_ref, Q_W4A + q, KH), pace))
                for t in range(2):
                    cols = slice((2 * q + t) * 128, (2 * q + t + 1) * 128)
                    rows = pl.ds(base + s * BLK, BLK)
                    b_ref[rows, cols] = ys[t] + b_ref[rows, cols]

        assert nb == 4
        for s in range(1, nb):
            make_g(s)
        zg = zeros["g", 1] + zeros["g", 2] + zeros["g", 3]
        zeros["g01"], zeros["g12"], zeros["g23"] = zg[:24], zg[24:36], zg[36:]
        plan = [(mix, 0, ["g01"], 0), (mix, 1, [("a", 0), "g12"], 0), (mix, 2, [("a", 1), "g23"], 0),
                (mix, 3, [("a", 2), ("g", 4)], 0), (up, 0, [("a", 3)], 0), (up, 1, [], 0.9), (down, 0, [], 1.6),
                (up, 2, [], 0.9), (down, 1, [], 1.6), (up, 3, [], 0.9), (down, 2, [], 1.6), (down, 3, [], 1.6)]
        wsum = sum(p[3] for p in plan) - plan[-1][3] * 2 / SL
        for fn, s, keys, w in plan:
            for key in keys:
                if key not in zeros:
                    make_g(key[1])
            zs = carry.pop(0, []) + [z for key in keys for z in zeros[key]]
            if zs:
                pace.require(zs, SL - 1 if keys else 7)
            pace.per = nitems * w / wsum / SL
            fn(s)
        assert not pace.items
        for k in range(6):
            qkv_extra(0, (k % 3) * NP + 2 * it + k // 3)
        return c
    lax.fori_loop(0, N2, p2, 0)

    row = lax.broadcasted_iota(jnp.int32, (R, R), 0)
    col = lax.broadcasted_iota(jnp.int32, (R, R), 1)
    same_head = (row >= L) == (col >= L)
    rr = jnp.where(row >= L, row - L, row)
    cc = jnp.where(col >= L, col - L, col)
    visible = same_head & ((rr < M) | (rr >= cc))
    scale = DH ** -0.5
    fill = jnp.where(same_head, -1e9 / scale, -jnp.inf).astype(F32)

    def softmax_qk(q2, k2):
        s = lax.dot_general(q2, k2, (((1,), (1,)), ((), ())), preferred_element_type=F32)
        s = jnp.where(visible, s, fill)
        m = jnp.max(s, axis=-1, keepdims=True)
        e = jnp.exp2((s - m) * (scale * LOG2E))
        l = jnp.sum(e, axis=-1, keepdims=True)
        r = pl.reciprocal(l, approx=True)
        r = r * (2.0 - l * r)
        return (e * r).astype(BF16)

    def combine(r, rdst, slot):
        b = b_ref[pl.ds(r, STEP), :]
        hb = 0.5 * b
        g = hb + hb * jnp.tanh(hb)
        x = x_ref[pl.ds(r, STEP), :].astype(F32)
        x_ref[pl.ds(rdst, STEP), :] = (x + s_ref[slot] * g).astype(x_ref.dtype)

    def out_copy(r):
        return pltpu.make_async_copy(x_ref.at[pl.ds(r, STEP)], out_hbm.at[pl.ds(r, STEP)], sems.at[SEM_OUT])

    def wo_extra(kb, q):
        def wt(op):
            return jnp.concatenate([stage[wos_rows(q, op, v) + (slice(None),)] for v in range(128)], axis=0)
        e = [oe_ref[kb & 1, k].astype(BF16) for k in range(3)]
        m1 = _dot(e[0], wt(0))
        pb = _dot(e[1], wt(1)) + m1
        pt = _dot(e[2], wt(2)) + m1
        c0 = pl.ds(pl.multiple_of(2 * q * 128, 128), 128)
        c1 = pl.ds(pl.multiple_of((2 * q + 1) * 128, 128), 128)
        for g in range(4):
            slot = (2 * kb + g // 2) & 3
            r = (g % 2) * SEG + 16
            s_ref[slot, r:r + 8, c0] = s_ref[slot, r:r + 8, c0] + pt[8 * g:8 * g + 8]
            s_ref[slot, r + 8:r + 16, c1] = s_ref[slot, r + 8:r + 16, c1] + pb[8 * g:8 * g + 8]

    def sweep_lhs(m1, m2, x1, x2):
        ms, xs = m1 + m2, x1 + x2
        return [jnp.concatenate(v, axis=0).astype(BF16) for v in (
            [ms, xs[0:16], xs[24:32]], [m2, x2[0:16], x2[24:32]],
            [m1, x1[0:16], x1[16:24]], [ms, xs[0:16], xs[16:24]])]

    s_ref[1:4] = jnp.zeros((3,) + s_ref.shape[1:], F32)
    oe_ref[1] = jnp.zeros(oe_ref.shape[1:], F32)

    def step(j, c):
        r0 = pl.multiple_of(j * STEP, STEP)
        par = j & 1
        blk = j >> 1
        rb = pl.multiple_of(blk * BLK, BLK)
        rprev = pl.multiple_of(jnp.maximum(r0 - 3 * STEP, 0), STEP)
        rdst = pl.multiple_of(jnp.where(j >= 3, r0 - 3 * STEP, S), STEP)
        al3 = load_left(a3_ref.at[blk])
        xn = _ln(x_ref[pl.ds(r0, STEP), :].astype(F32))

        parts = []

        def up_products():
            for q in range(FS // 2):
                wt = quad_wt(p_ref, 2 * NQ + par if q == 0 else par * NQ + q - 1, KH)
                for y in _strassen(al3, wt):
                    if y is not None:
                        parts.append(_gelu_left(*y)[0])
                    yield

        def down_products():
            al4 = _cat(parts, 1)
            for q in range(NQ):
                for ys in _strassen(al4, quad_wt(r_ref, par * NQ + q, FH)):
                    if ys is not None:
                        for t in range(2):
                            cols = slice((2 * q + t) * 128, (2 * q + t + 1) * 128)
                            b_ref[pl.ds(rb, BLK), cols] = ys[t] + b_ref[pl.ds(rb, BLK), cols]
                    yield
        ups, downs = up_products(), down_products()

        def run(gen, n):
            for _ in range(n):
                next(gen)

        def segment(sg, mem, fillers, inter):
            xs = xn[sg * SEG:(sg + 1) * SEG]
            lhs = sweep_lhs(mem[:, :HK], mem[:, HK:], xs[:, :HK], xs[:, HK:])
            prow = pl.ds(pl.multiple_of((par * 2 + sg) * 8, 8), 8)
            qkv = [None] * NP
            prob = [None] * NP
            ol = [None] * NP
            ph = NP - 3

            def do_qkv(p):
                res = []
                for m in range(3):
                    w0, w1 = m * H + 2 * p, m * H + 2 * p + 1
                    d11 = _dot(lhs[0], wqkv_ref[w0, 0:KH, :])
                    d4 = _dot(lhs[1], wqkv_ref[w0, KH:, :])
                    d3 = _dot(lhs[2], wqkv_ref[w1, 0:KH, :])
                    d22 = _dot(lhs[3], wqkv_ref[w1, KH:, :])
                    pt = px_ref[blk & 1, m * NP + p, 0, prow, :]
                    pb = px_ref[blk & 1, m * NP + p, 1, prow, :]
                    res.append(jnp.concatenate([
                        d11[0:24] + d4[0:24], pt + (d4[24:32] - d22[24:32]), d11[24:32] + d4[24:32],
                        d3[0:24] + d22[0:24], d3[24:32] + d22[24:32], pb + (d3[24:32] - d11[24:32])],
                        axis=0).astype(BF16))
                qkv[p] = res

            def do_qk(p):
                prob[p] = softmax_qk(qkv[p][0], qkv[p][1])

            def do_pv(p):
                o = jnp.dot(prob[p], qkv[p][2], preferred_element_type=F32)
                o1, o2 = o[0:L], o[L:]
                ol[p] = sweep_lhs(o1[0:8], o2[0:8], o1[8:], o2[8:])
                t1, t2, b1, b2 = o1[24:32], o2[24:32], o1[32:40], o2[32:40]
                for k, v in enumerate((t1 + b2, b1 - t1, t2 - b2)):
                    oe_ref[blk & 1, k, prow, p * 128:(p + 1) * 128] = v

            def wo_part(ps, q, acc=None):
                d = []
                for k in range(4):
                    n, o = 2 * q + k // 2, 64 * (k % 2)
                    y = _dot(jnp.concatenate([ol[p][k] for p in ps], axis=1),
                             jnp.concatenate([wo_ref[n, 128 * p + o:128 * p + o + 64, :] for p in ps], axis=0))
                    d.append(y if acc is None else y + acc[k])
                return d

            for p in range(NP):
                do_qkv(p)
                inter(p)
                if p >= 1:
                    do_qk(p - 1)
                if p >= 3:
                    do_pv(p - 3)
            fillers[0]()
            do_qk(NP - 1)
            do_pv(NP - 3)
            do_pv(NP - 2)
            acc = [wo_part(range(ph), q) for q in range(NQ // 2)]
            do_pv(NP - 1)
            fillers[1]()
            acc += [wo_part(range(ph), q) for q in range(NQ // 2, NQ)]
            cols = []
            for q in range(NQ):
                d11, d4, d3, d22 = wo_part(range(ph, NP), q, acc[q])
                cols += [jnp.concatenate([d11[0:24] + d4[0:24], d4[24:32] - d22[24:32], d11[24:32] + d4[24:32]], axis=0),
                         jnp.concatenate([d3[0:24] + d22[0:24], d3[24:32] + d22[24:32], d3[24:32] - d11[24:32]], axis=0)]
            res = jnp.concatenate(cols, axis=1)
            s_ref[j & 3, sg * SEG:(sg + 1) * SEG, :] = res[8:]
            mem_ref[...] = res[0:8]
            fillers[2]()
            return res[0:8]

        U0, U1, IA, IB, D0 = 8, 6, 1, 2, 7

        def inter_a(p):
            if p < NP // 2:
                for m in range(3):
                    qkv_extra((j + 1) >> 1, m * NP + (1 - par) * (NP // 2) + p)
            if p >= IA:
                run(ups, 1)

        def tail_b0():
            combine(rprev, rdst, (j + 1) & 3)
            run(downs, D0)

        def tail_b2():
            for t in range(2):
                wo_extra((j - 1) >> 1, 2 * (1 - par) + t)

        mem = mem_ref[...]
        run(ups, U0)
        mem = segment(0, mem, [lambda: run(ups, U1), lambda: None, lambda: run(ups, 35 - U0 - U1 - (NP - IA))],
                      inter_a)
        segment(1, mem, [tail_b0, lambda: run(downs, 28 - (NP - IB) - D0), tail_b2],
                lambda p: run(downs, 1) if p >= IB else None)

        @pl.when(j >= 3)
        def _():
            out_copy(rprev).start()
        return c
    nst = S // STEP
    lax.fori_loop(0, nst, step, 0)
    for t in range(2):
        wo_extra(nst // 2 - 1, 2 + t)

    def last(j, c):
        r = pl.multiple_of(j * STEP, STEP)
        combine(r, r, j & 3)
        out_copy(r).start()
        return c
    lax.fori_loop(nst - 3, nst, last, 0)
    pltpu.make_async_copy(x_ref.at[pl.ds(0, S)], out_hbm, sems.at[SEM_OUT]).wait()


@functools.partial(jax.jit, static_argnames=("A_seg_len",))
def pallas_recurrent_scan__memory_aug_recurrent_mem_tr__mixer_s_mlp__prompt_kernel(
        A_x, A_mem0, A_Wq, A_Wk, A_Wv, A_Wo, A_seg_len, B_x, B_w1, B_w2, B_w3, B_w4):
    del B_x
    B, S, D = A_x.shape
    _, H, DH = A_Wq.shape
    M = A_mem0.shape[1]
    FF = B_w3.shape[1]
    assert (B, S, D, H, DH, M, A_seg_len, FF) == (1, 2048, 1024, 32, 128, 8, 32, 3584)
    nd, nf = D // 128, FF // 128
    kern = functools.partial(_kernel, S=S, D=D, H=H, DH=DH, M=M, SEG=A_seg_len, FF=FF)
    any_spec = pl.BlockSpec(memory_space=pl.ANY)
    out = pl.pallas_call(
        kern,
        out_shape=jax.ShapeDtypeStruct((S, D), A_x.dtype),
        in_specs=[any_spec] * 10,
        out_specs=any_spec,
        scratch_shapes=[
            pltpu.VMEM((S + STEP, D), BF16),
            pltpu.VMEM((3 * H // 2, D, 128), U32),
            pltpu.VMEM((3 * H, D // 2, 128), U32),
            pltpu.VMEM((nd, H * DH // 2, 128), U32),
            pltpu.VMEM((nd, D // 2, 128), U32),
            pltpu.VMEM((3 * nd // 2, 7 * D // 4, 128), U32),
            pltpu.VMEM(((nf - CPRE) // 2, 7 * D // 4, 128), U32),
            pltpu.VMEM((nd, 7 * (nf - CPRE) * 16, 128), U32),
            pltpu.VMEM((nd, S + 16, 128), F32),
            pltpu.VMEM((S, D), F32),
            pltpu.VMEM((S // BLK, 7, HB // 2, D // 2), U32),
            pltpu.VMEM((HB // 2, D), U32),
            pltpu.VMEM((7, HB // 2, D // 2), U32),
            pltpu.VMEM((4, STEP, D), F32),
            pltpu.VMEM((2, 3 * H // 2, 2, 32, 128), F32),
            pltpu.VMEM((S // BLK, 3, 16, D // 2), U32),
            pltpu.VMEM((2, 3, 32, H * DH // 2), F32),
            pltpu.VMEM((M, D), BF16),
            pltpu.VMEM((M, D), F32),
            pltpu.SemaphoreType.DMA((2 + nd + 4 + 2 * ((S - RB0) // RB1) + S // RB2,)),
        ],
        compiler_params=pltpu.CompilerParams(vmem_limit_bytes=127 * 1024 * 1024,
                                             disable_bounds_checks=True),
    )(A_x[0], A_mem0[0], A_Wq, A_Wk, A_Wv, A_Wo.reshape(H * DH, D), B_w1, B_w2, B_w3, B_w4)
    return out[None]
```
